```python
import jax
import jax.numpy as jnp

def _softmax(x, axis=-1):
    return jax.nn.softmax(x, axis=axis)
def _gelu(x):
    return jax.nn.gelu(x, approximate=True)
def _silu(x):
    return jax.nn.silu(x)
def _sigmoid(x):
    return jax.nn.sigmoid(x)
def _layernorm(x, axis=-1, eps=1e-5):
    m = jnp.mean(x, axis=axis, keepdims=True)
    v = jnp.var(x, axis=axis, keepdims=True)
    return (x - m) / jnp.sqrt(v + eps)
def _scatter_add(tgt, idx, src, axis=0):
    return tgt.at[idx].add(src)
def _segment_sum(src, seg, n):
    return jax.ops.segment_sum(src, seg, n)
class _Rng:
    def __init__(self, key):
        self._k = key
    def _next(self):
        self._k, sub = jax.random.split(self._k)
        return sub
    def normal(self, shape):
        return jax.random.normal(self._next(), shape, dtype=jnp.bfloat16)
    def randint(self, lo, hi, shape):
        return jax.random.randint(self._next(), shape, lo, hi, dtype=jnp.int32)
    def uniform(self, shape, lo=0.0, hi=1.0):
        return jax.random.uniform(self._next(), shape, jnp.bfloat16, lo, hi)
    def permutation(self, n):
        return jax.random.permutation(self._next(), n)


kernel_name = 'interleave_layers__sliding_local_dilated__softmax_full_mha__prompt'

def setup_inputs():
    _rng = _Rng(jax.random.key(int.from_bytes(__import__("os").urandom(4), "little")))
    _w = (lambda a: (lambda t: t.astype(jnp.bfloat16) if jnp.issubdtype(t.dtype, jnp.floating) else t)(jnp.asarray(a)))
    def _A_setup():
        B, S, D = 1, 2048, 1024
        return {
            "x": _w((lambda *s: _rng.normal(s) * 0.05)(B, S, D)),
            "wqkv": _w((lambda *s: _rng.normal(s) * 0.05)(D, 3 * D)),
            "wo": _w((lambda *s: _rng.normal(s) * 0.05)(D, D)),
        }
    _A_in = _A_setup()

    def _B_setup():
        B, S, D = 1, 2048, 1024
        return {
            "x": _w((lambda *s: _rng.normal(s) * 0.05)(B, S, D)),
            "wqkv": _w((lambda *s: _rng.normal(s) * 0.05)(D, 3 * D)),
            "wo": _w((lambda *s: _rng.normal(s) * 0.05)(D, D)),
        }
    _B_in = _B_setup()

    return {
        "A_x": _A_in["x"],
        "A_wqkv": _A_in["wqkv"],
        "A_wo": _A_in["wo"],
        "B_x": _B_in["x"],
        "B_wqkv": _B_in["wqkv"],
        "B_wo": _B_in["wo"],
    }

def reference(A_x, A_wqkv, A_wo, B_x, B_wqkv, B_wo):
    def _A_ref(x, wqkv, wo):
        B, S, D = x.shape
        H = 32; Dh = D // H
        W, dil = 8, 2
        qkv = (lambda x, *d: x.transpose(*d))((x @ wqkv).reshape(B, S, 3, H, Dh), 2, 0, 3, 1, 4)
        q, k, v = qkv[0], qkv[1], qkv[2]
        scale = Dh ** -0.5
        pos = jnp.arange(S)
        off = jnp.arange(W) * dil
        idx = pos[:, None] - off[None, :]
        mask = idx >= 0
        idx_c = jnp.where(mask, idx, 0).reshape(-1)
        kg = k[:, :, idx_c, :].reshape(B, H, S, W, Dh)
        vg = v[:, :, idx_c, :].reshape(B, H, S, W, Dh)
        logits = jnp.einsum("bhsd,bhswd->bhsw", q, kg) * scale
        logits = jnp.where(mask[None, None, :, :], logits, -1e9)
        attn = _softmax(logits, axis=-1)
        o = jnp.einsum("bhsw,bhswd->bhsd", attn, vg)
        return (lambda x, *d: x.transpose(*d))(o, 0, 2, 1, 3).reshape(B, S, D) @ wo

    def _B_ref(x, wqkv, wo):
        B, S, D = x.shape
        H = 32; Dh = D // H
        qkv = (lambda x, *d: x.transpose(*d))((x @ wqkv).reshape(B, S, 3, H, Dh), 2, 0, 3, 1, 4)
        q, k, v = qkv[0], qkv[1], qkv[2]
        scale = Dh ** -0.5
        scores = jnp.einsum("bhqd,bhkd->bhqk", q, k) * scale
        p = _softmax(scores, axis=-1)
        o = jnp.einsum("bhqk,bhkd->bhqd", p, v)
        return (lambda x, *d: x.transpose(*d))(o, 0, 2, 1, 3).reshape(B, S, D) @ wo

    x = A_x
    x = x + _A_ref(_layernorm(x, axis=-1), A_wqkv, A_wo)
    x = x + _B_ref(_layernorm(x, axis=-1), B_wqkv, B_wo)
    x = x + _A_ref(_layernorm(x, axis=-1), A_wqkv, A_wo)
    x = x + _B_ref(_layernorm(x, axis=-1), B_wqkv, B_wo)
    return x
```

```python
import functools
import math

import jax
import jax.numpy as jnp
from jax import lax
import jax.experimental.pallas as pl
import jax.experimental.pallas.tpu as pltpu

F32 = jnp.float32
BF16 = jnp.bfloat16

S = 2048
D = 1024
H = 32
DH = D // H
NT = D // 128
WIN, DIL = 8, 2
HALO = 16
EPS = 1e-5
NEG = -1e9
QSCALE = DH ** -0.5 * math.log2(math.e)

R = 256
NR = S // R
BQ = 256
CK = 128
QB = 2
NQ = S // BQ
assert BQ == R


def _dot(a, b):
    return jnp.dot(a, b, preferred_element_type=F32)


def _layernorm(x):
    m = jnp.mean(x, axis=-1, keepdims=True)
    xc = x - m
    v = jnp.mean(xc * xc, axis=-1, keepdims=True)
    return xc * lax.rsqrt(v + EPS)


def _tile(t):
    return slice(t * 128, (t + 1) * 128)


def _permute_heads(tiles):
    shape = tiles[0].shape
    lane = lax.broadcasted_iota(jnp.int32, shape, 1)
    tiles = list(tiles)
    for b in (1, 2, 4):
        swap = ((lane >> 2) & b) != 0
        tiles = [jnp.where(swap, tiles[i ^ b], tiles[i]) for i in range(NT)]
    e, j, hl = lane >> 5, (lane >> 2) & 7, lane & 3
    return [jnp.take_along_axis(tiles[i], hl * 32 + (j ^ i) * 4 + e, axis=1) for i in range(NT)]


def _permute_heads_bf16(w):
    w32 = pltpu.bitcast(w, jnp.int32)
    out = _permute_heads([w32[:, _tile(t)] for t in range(NT)])
    return pltpu.bitcast(jnp.concatenate(out, axis=1), BF16)


def _kernel(x_hbm, awqkv_hbm, awo_hbm, bwqkv_hbm, bwo_hbm, out_hbm,
            io_ref, x_ref, xn_ref, awqkv_ref, awo_raw_ref, awo_ref, bwqkv_ref, bwo_ref,
            qa_ref, ka_ref, va_ref, pa_ref, oa_ref,
            qt_ref, k_ref, vt_ref, ot_ref, s_ref, m_ref, sems, out_sems):
    x_cp = pltpu.make_async_copy(x_hbm, io_ref, sems.at[0])
    aw_cp = [pltpu.make_async_copy(awqkv_hbm.at[:, pl.ds(p * D, D)],
                                   awqkv_ref.at[:, pl.ds(p * D, D)], sems.at[1 + p])
             for p in range(3)]
    awo_cp = pltpu.make_async_copy(awo_hbm, awo_raw_ref, sems.at[4])
    bw_cp = pltpu.make_async_copy(bwqkv_hbm, bwqkv_ref, sems.at[5])
    bwo_cp = pltpu.make_async_copy(bwo_hbm, bwo_ref, sems.at[6])
    x_cp.start()
    for cp in aw_cp:
        cp.start()

    def rows(i, n=R):
        return pl.ds(pl.multiple_of(i * n, n), n)

    ka_ref[:, R:, :] = jnp.zeros((NT, HALO, 128), F32)
    va_ref[:, R:, :] = jnp.zeros((NT, HALO, 128), F32)

    x_cp.wait()
    awo_cp.start()

    @pl.loop(0, NR)
    def _(i):
        x_ref[rows(i), :] = io_ref[rows(i), :].astype(F32)

    for p in range(3):
        aw_cp[p].wait()

        @pl.loop(0, D // 256)
        def _(i):
            blk = (rows(i, 256), pl.ds(p * D, D))
            awqkv_ref[blk] = _permute_heads_bf16(awqkv_ref[blk])

    bw_cp.start()
    bwo_cp.start()
    awo_cp.wait()

    for t in range(NT):
        awo_ref[:, _tile(t)] = _permute_heads_bf16(awo_raw_ref[:, _tile(t)].T).T

    def local_qkv_attn(i):
        xn = xn_ref[...]
        nxt = jnp.minimum(i + 1, NR - 1)
        for t in range(NT):
            ka_ref[t, :HALO, :] = ka_ref[t, R:, :]
        k = _dot(xn, awqkv_ref[:, D:2 * D])
        for t in range(NT):
            ka_ref[t, HALO:, :] = k[:, _tile(t)]
        q = _dot(xn, awqkv_ref[:, :D])
        for t in range(NT):
            qa_ref[t] = q[:, _tile(t)]
        G = 16
        for r in range(0, R, G):
            logits = [None] * WIN
            for t in range(NT):
                qv = qa_ref[t, r:r + G, :]
                for w in range(WIN):
                    lo = HALO + r - DIL * w
                    prod = qv * ka_ref[t, lo:lo + G, :]
                    logits[w] = prod if t == 0 else logits[w] + prod
            for w in range(WIN):
                a = logits[w]
                a = a + pltpu.roll(a, 64, 1)
                a = (a + pltpu.roll(a, 32, 1)) * QSCALE
                if r < DIL * w:
                    pos = i * R + r + lax.broadcasted_iota(jnp.int32, (G, 128), 0)
                    a = jnp.where(pos >= DIL * w, a, NEG * math.log2(math.e))
                logits[w] = a
            mx = functools.reduce(jnp.maximum, logits)
            e = [jnp.exp2(a - mx) for a in logits]
            inv = 1.0 / functools.reduce(jnp.add, e)
            for w in range(WIN):
                pa_ref[w, r:r + G, :] = e[w] * inv
        for t in range(NT):
            v = _dot(xn, awqkv_ref[:, 2 * D + t * 128:2 * D + (t + 1) * 128])
            va_ref[t, :HALO, :] = jnp.where(i == 0, jnp.broadcast_to(v[0:1], (HALO, 128)),
                                            va_ref[t, R:, :])
            va_ref[t, HALO:, :] = v
            acc = None
            for w in range(WIN):
                lo = HALO - DIL * w
                prod = pa_ref[w] * va_ref[t, lo:lo + R, :]
                acc = prod if w == 0 else acc + prod
            oa_ref[rows(i), _tile(t)] = acc.astype(BF16)
        xn_ref[...] = _layernorm(x_ref[rows(nxt), :]).astype(BF16)

    def local_out_full_qkv(i):
        SUB = 128
        for r in range(0, R, SUB):
            rr = pl.ds(pl.multiple_of(i * R + r, SUB), SUB)
            x = x_ref[rr, :] + _dot(oa_ref[rr, :], awo_ref[...])
            x_ref[rr, :] = x
            xn_ref[r:r + SUB, :] = _layernorm(x).astype(BF16)
        xn = xn_ref[...]
        q = _dot(xn, bwqkv_ref[:, :D]) * QSCALE
        for t in range(NT):
            qt_ref[t, i] = q[:, _tile(t)].T.astype(BF16)
        v = _dot(xn, bwqkv_ref[:, 2 * D:])
        for t in range(NT):
            vt_ref[t, i] = v[:, _tile(t)].T.astype(BF16)
        k = _dot(xn, bwqkv_ref[:, D:2 * D])
        for t in range(NT):
            k_ref[t, rows(i), :] = k[:, _tile(t)].astype(BF16)

    def attn_unit(u, j, nxt, cur, tail=False):
        hs = slice(j * DH, (j + 1) * DH)
        if cur is not None:
            m = jnp.broadcast_to(jnp.max(m_ref[u], axis=0, keepdims=True), (16, BQ))
        l = acc = m_acc = None
        for c in range(S // CK):
            ks = slice(c * CK, (c + 1) * CK)

            def scores():
                parts = [qt_ref[nxt[0], nxt[1], hs, :]]
                if j > 0:
                    parts.insert(0, jnp.zeros((DH * j, BQ), BF16))
                if j < 3:
                    parts.append(jnp.zeros((DH * (3 - j), BQ), BF16))
                return _dot(k_ref[nxt[0], ks, :], jnp.concatenate(parts, axis=0))

            late = tail and c == S // CK - 1
            if nxt is not None and not late:
                s = scores()
            if cur is not None:
                slabs = {}
                for r in reversed(range(CK // 16)):
                    p = jnp.exp2(s_ref[u, c * CK + r * 16:c * CK + (r + 1) * 16, :] - m)
                    ls = p[0:8] + p[8:16]
                    l = ls if l is None else l + ls
                    slabs[r] = p
                p = jnp.concatenate([slabs[r] for r in range(CK // 16)], axis=0).astype(BF16)
                off = c * CK % R
                a = _dot(vt_ref[cur[0], c * CK // R, hs, off:off + CK], p)
                acc = a if acc is None else acc + a
            if nxt is not None:
                if late:
                    s = scores()
                s_ref[u, ks, :] = s
                mx = jnp.max(s.reshape(CK // 8, 8, BQ), axis=0)
                m_acc = mx if m_acc is None else jnp.maximum(m_acc, mx)
        if nxt is not None:
            m_ref[u] = m_acc
        if cur is not None:
            inv = 1.0 / jnp.sum(l, axis=0, keepdims=True)
            ot_ref[cur[0], cur[1], hs, :] = (acc * inv).astype(BF16)

    def full_attention():
        nqb = NQ // QB
        n_it = NT * nqb

        @pl.loop(0, QB)
        def _(b):
            for j in range(4):
                attn_unit(b * 4 + j, j, (0, b), None)

        @pl.loop(0, n_it - 1)
        def _(i):
            g, q = i // nqb, (i % nqb) * QB
            g2, q2 = (i + 1) // nqb, ((i + 1) % nqb) * QB
            for b in range(QB):
                for j in range(4):
                    attn_unit(b * 4 + j, j, (g2, q2 + b), (g, q + b),
                              tail=(b == QB - 1 and j == 3))

        @pl.loop(0, QB)
        def _(b):
            for j in range(4):
                attn_unit(b * 4 + j, j, None, (NT - 1, NQ - QB + b))

    def out_copy(i):
        return pltpu.make_async_copy(io_ref.at[rows(i)], out_hbm.at[rows(i)], out_sems.at[i])

    @pl.loop(0, 2)
    def _(rep):
        xn_ref[...] = _layernorm(x_ref[0:R, :]).astype(BF16)
        pl.loop(0, NR)(local_qkv_attn)

        @pl.when(rep == 0)
        def _():
            bw_cp.wait()
            bwo_cp.wait()

        pl.loop(0, NR)(local_out_full_qkv)
        full_attention()

        for t in range(NT):
            xn_ref[:, _tile(t)] = ot_ref[t, 0].T

        @pl.loop(0, NR)
        def _(i):
            x = x_ref[rows(i), :] + _dot(xn_ref[...], bwo_ref[...])
            x_ref[rows(i), :] = x
            io_ref[rows(i), :] = x.astype(BF16)
            nxt = jnp.minimum(i + 1, NR - 1)
            for t in range(NT):
                xn_ref[:, _tile(t)] = ot_ref[t, nxt].T

            @pl.when(rep == 1)
            def _():
                out_copy(i).start()

    for i in range(NR):
        out_copy(i).wait()


@jax.jit
def pallas_interleave_layers__sliding_local_dilated__softmax_full_mha__prompt_kernel(
    A_x: jax.Array,
    A_wqkv: jax.Array,
    A_wo: jax.Array,
    B_x: jax.Array,
    B_wqkv: jax.Array,
    B_wo: jax.Array,
):
    del B_x
    vmem = pltpu.VMEM
    out = pl.pallas_call(
        _kernel,
        out_shape=jax.ShapeDtypeStruct((S, D), BF16),
        in_specs=[pl.BlockSpec(memory_space=pl.ANY)] * 5,
        out_specs=pl.BlockSpec(memory_space=pl.ANY),
        scratch_shapes=[
            vmem((S, D), BF16),
            vmem((S, D), F32),
            vmem((R, D), BF16),
            vmem((D, 3 * D), BF16),
            vmem((D, D), BF16),
            vmem((D, D), BF16),
            vmem((D, 3 * D), BF16),
            vmem((D, D), BF16),
            vmem((NT, R, 128), F32),
            vmem((NT, HALO + R, 128), F32),
            vmem((NT, HALO + R, 128), F32),
            vmem((WIN, R, 128), F32),
            vmem((S, D), BF16),
            vmem((NT, NQ, 128, BQ), BF16),
            vmem((NT, S, 128), BF16),
            vmem((NT, NR, 128, R), BF16),
            vmem((NT, NQ, 128, BQ), BF16),
            vmem((4 * QB, S, BQ), F32),
            vmem((4 * QB, 8, BQ), F32),
            pltpu.SemaphoreType.DMA((7,)),
            pltpu.SemaphoreType.DMA((NR,)),
        ],
        compiler_params=pltpu.CompilerParams(vmem_limit_bytes=110 * 2 ** 20),
        name="interleave_layers",
    )(A_x.reshape(S, D), A_wqkv, A_wo, B_wqkv, B_wo)
    return out.reshape(A_x.shape)
```

```python
import functools
import math

import jax
import jax.numpy as jnp
from jax import lax
import jax.experimental.pallas as pl
import jax.experimental.pallas.tpu as pltpu

F32 = jnp.float32
BF16 = jnp.bfloat16
I32 = jnp.int32

S = 2048
D = 1024
H = 32
DH = D // H
NT = D // 128
NP = NT // 2
WIN, DIL = 8, 2
HALO = 16
EPS = 1e-5
NEG = -1e9
LOG2E = math.log2(math.e)
QSCALE = DH ** -0.5 * LOG2E

R = 256
HR = R // 2
NR = S // R
BQ = 256
CK = 128
QB = 2
NQ = S // BQ
assert BQ == R
SLACK = 2
EARLY = 1
PAD = 8
NBW = 6
NMIX = 0


def _dot(a, b):
    return jnp.dot(a, b, preferred_element_type=F32)


def _pack(x):
    return pltpu.bitcast(x.astype(BF16), I32)


def _unpack(x):
    return pltpu.bitcast(x, BF16)


def _tile(t):
    return slice(t * 128, (t + 1) * 128)


def _lhs_terms(a11, a12, a21, a22):
    return [a21 + a22, a22, a11 + a22, a21 - a11, a12 - a22, a11 + a12, a11]


def _rhs_terms(b11, b12, b21, b22):
    return [b11, b21 - b11, b11 + b22, b11 + b12, b21 + b22, b22, b12 - b22]


def _tasks(reads, fn, *args):
    return [(reads, functools.partial(fn, *args[:-1], a)) for a in args[-1]]


class _Projector:
    def __init__(self, lhs, z):
        self.lhs, self.z = lhs, z
        self.results, self.deadlines, self.plan = [], {}, {}

    def spread(self, tasks, first, last):
        for n, task in enumerate(tasks):
            step, sub = divmod(int(8 * (first + n * (last - first) / len(tasks))), 8)
            self.plan.setdefault(step, []).append((sub, *task))

    def not_before_now(self, ref, sub):
        if len(self.results) > EARLY:
            spare = (0,) * (len(ref.shape) - 2) + (slice(ref.shape[-2] - PAD, None), slice(128))
            ref[spare] = self.results[-1 - EARLY][16 * sub:16 * sub + PAD].astype(ref.dtype)

    def due(self, ref, n, sub=0):
        if ref is not None:
            value = ref[(self.z,) + (0,) * (len(ref.shape) - 3)
                        + (slice(32 // ref.dtype.itemsize), slice(128))]
            self.deadlines.setdefault(len(self.results) + n, []).append((sub, pltpu.bitcast(value, I32)))

    def product(self, s, rhs):
        lhs = self.lhs(s)
        waits = self.deadlines.pop(len(self.results), ())
        if waits:
            head = [lhs[r:r + 8, :128] for r in range(0, lhs.shape[0], 8)]
            for sub, value in waits:
                head[sub] = jnp.where(self.z > 0, value, head[sub])
            lhs = jnp.concatenate([jnp.concatenate(head, axis=0), lhs[:, 128:]], axis=1)
        out = _dot(_unpack(lhs), _unpack(rhs))
        tasks = self.plan.pop(len(self.results), ())
        self.results.append(out)
        for sub, reads, task in sorted(tasks, key=lambda t: t[0]):
            for ref in reads:
                self.not_before_now(ref, sub)
            self.due(task(), SLACK, sub)
        return out

    def strassen(self, w_ref, col_pair, emit, emit_delay=2):
        def product(s):
            return self.product(s, w_ref[col_pair, :, s].reshape(D // 4, 128))

        x = product(0)
        y = product(1)
        self.due(emit(1, 0, x + y), emit_delay)
        m = product(2)
        x, y = m - x, y + m
        x = x + product(3)
        y = y + product(4)
        m = product(5)
        self.due(emit(0, 0, y - m), emit_delay)
        y = product(6)
        emit(1, 1, x + y)
        self.due(emit(0, 1, m + y), emit_delay)


def _permute_heads(tiles):
    dtype = tiles[0].dtype
    tiles = [pltpu.bitcast(t, I32) for t in tiles]
    lane = lax.broadcasted_iota(I32, tiles[0].shape, 1)
    for b in (1, 2, 4):
        swap = ((lane >> 2) & b) != 0
        tiles = [jnp.where(swap, tiles[i ^ b], tiles[i]) for i in range(NT)]
    e, j, hl = lane >> 5, (lane >> 2) & 7, lane & 3
    tiles = [jnp.take_along_axis(tiles[i], hl * 32 + (j ^ i) * 4 + e, axis=1) for i in range(NT)]
    return [pltpu.bitcast(t, dtype) for t in tiles]


def _kernel(x_hbm, awqkv_hbm, awo_hbm, bwqkv_hbm, bwo_hbm, out_hbm,
            x_ref, lhs_ref, nxt_ref, mean_ref, rstd_ref,
            wa_ref, wao_ref, wb_ref, wbo_ref, awqkv_ref, awo_ref, bwqkv_ref, bwo_ref,
            qa_refs, ka_refs, va_refs, pa_refs, prob_ref, oa_ref, flip_refs, tmp_ref,
            qt_ref, k_ref, vt_ref, ot_ref, s_ref, m_ref,
            x_sems, aw_sems, awo_sems, bw_sems, bwo_sem):
    def rows(i, n=R, off=0, size=None, align=None):
        return pl.ds(pl.multiple_of(i * n + off, align or size or n), size or n)

    def x_copy(i):
        return pltpu.make_async_copy(x_hbm.at[rows(i)], x_ref.at[rows(i)], x_sems.at[i])

    def out_copy(i):
        return pltpu.make_async_copy(x_ref.at[rows(i)], out_hbm.at[rows(i)], x_sems.at[i])

    def aw_copy(i):
        return pltpu.make_async_copy(awqkv_hbm.at[rows(i % NP, 256), rows(i // NP, D)],
                                     awqkv_ref.at[i], aw_sems.at[i])

    def awo_copy(i):
        return pltpu.make_async_copy(awo_hbm.at[:, rows(i, 256)], awo_ref.at[i, :D], awo_sems.at[i])

    def bw_copy(i):
        return pltpu.make_async_copy(bwqkv_hbm.at[rows(i // 2, 256), rows(i % 2, 3 * D // 2)],
                                     bwqkv_ref.at[i, :256], bw_sems.at[i])

    bwo_copy = pltpu.make_async_copy(bwo_hbm, bwo_ref.at[:D], bwo_sem)

    def put_weights(w_ref, col_pair, row_pair, r, b11, b12, b21, b22):
        terms = _rhs_terms(*(b.astype(F32) for b in (b11, b12, b21, b22)))
        for s, term in enumerate(terms):
            w_ref[col_pair, row_pair, s, r // 2:(r + b11.shape[0]) // 2, :] = _pack(term)

    G = 16

    def weight_tasks(w_ref, col_pair, row_pair, src, load):
        def task(r):
            lo, hi = load(r), load(128 + r)
            put_weights(w_ref, col_pair, row_pair, r,
                        lo[:, :128], lo[:, 128:], hi[:, :128], hi[:, 128:])
            return w_ref
        return _tasks([src], task, range(0, 128, G))

    def norm_tasks(i, dst, z):
        views = [x_ref.at[rows(i + n * z)] for n in range(3)]

        def mean_task(r):
            x = views[0][r:r + G, :].astype(F32)
            mean_ref[0, r:r + G, :] = jnp.broadcast_to(
                jnp.mean(x, axis=-1, keepdims=True), (G, 128))
            return mean_ref

        def rstd_task(r):
            x = views[1][r:r + G, :].astype(F32)
            mean = mean_ref[z, r:r + G, :]
            sq = functools.reduce(
                jnp.add, [jnp.square(x[:, _tile(t)] - mean) for t in range(NT)])
            var = jnp.sum(sq, axis=-1, keepdims=True) * (1.0 / D)
            rstd_ref[0, r:r + G, :] = lax.rsqrt(jnp.broadcast_to(var, (G, 128)) + EPS)
            return rstd_ref

        def terms_task(r, p):
            blocks = []
            for h in (0, HR):
                mean, rstd = mean_ref[z, h + r:h + r + G, :], rstd_ref[z, h + r:h + r + G, :]
                x = views[2][h + r:h + r + G, p * 256:(p + 1) * 256].astype(F32)
                blocks += [(x[:, :128] - mean) * rstd, (x[:, 128:] - mean) * rstd]
            for s, term in enumerate(_lhs_terms(*blocks)):
                dst[0, s, r // 2:(r + G) // 2, _tile(p)] = _pack(term)
            return dst

        return (_tasks([x_ref], mean_task, range(0, R, G)),
                _tasks([x_ref], rstd_task, range(0, R, G)),
                [t for r in range(0, HR, G) for t in _tasks([x_ref], terms_task, r, range(NP))])

    def advance_tasks(proj, width):
        def task(s):
            lhs_ref[0, s, :, :width] = nxt_ref[proj.z, s, :HR // 2, :width]
        return _tasks([nxt_ref], task, range(7))

    def run(*stages):
        for stage in stages:
            for _, task in stage:
                task()

    x_copy(0).start()
    for i in range(3 * NP):
        aw_copy(i).start()
    x_copy(1).start()
    awo_copy(0).start()
    bw_copy(0).start()
    for p in range(NP):
        ka_refs[p][:, R:R + HALO, :] = jnp.zeros((2, HALO, 128), F32)
        va_refs[p][:, :HALO, :] = jnp.zeros((2, HALO, 128), F32)

    @pl.loop(0, 3 * NP)
    def _(i):
        aw_copy(i).wait()
        t = _permute_heads([awqkv_ref[i, :, _tile(c)] for c in range(NT)])
        for p in range(NP):
            put_weights(wa_ref, i // NP * NP + p, i % NP, 0, t[2 * p][:128], t[2 * p + 1][:128],
                        t[2 * p][128:], t[2 * p + 1][128:])

    for i in range(1, NR):
        if i + 1 < NR:
            x_copy(i + 1).start()
        if i < NP:
            awo_copy(i).start()
        bw_copy(i).start()
    bwo_copy.start()
    x_copy(0).wait()

    def mix_tasks(i, z, p, store):
        prob = prob_ref.at[i + z * (p + 1)]
        v = va_refs[p].at[:, rows(i + z, R, 0, HALO + R, 8)]

        def mix_task(r):
            o = [None, None]
            for w in range(WIN):
                a = prob[w, r:r + 8, :]
                for c in (0, 1):
                    prod = a * v[c, HALO + r - DIL * w:HALO + r - DIL * w + 8, :]
                    o[c] = prod if w == 0 else o[c] + prod
            for c in (0, 1):
                qa_refs[p][c, r:r + 8, :] = o[c]
            return qa_refs[p]

        def terms_task(r):
            blocks = [qa_refs[p][z + c, h + r:h + r + G, :] for h in (0, HR) for c in (0, 1)]
            for s, term in enumerate(_lhs_terms(*blocks)):
                ref = store(s, slice(r // 2, (r + G) // 2), _pack(term))
            return ref

        return (_tasks([va_refs[p], prob_ref], mix_task, range(0, R, 8))
                + _tasks([qa_refs[p]], terms_task, range(0, HR, G)))

    def bw_tasks(i, blocks):
        def block(c):
            return weight_tasks(wb_ref, i % 2 * 6 + c, i // 2, bwqkv_ref,
                                lambda r: bwqkv_ref[i, r:r + G, c * 256:(c + 1) * 256])
        return [t for c in blocks for t in block(c)]

    def local_qkv_attention(rep, i):
        @pl.when(rep == 0)
        def _():
            pl.when(i + 1 < NR)(lambda: x_copy(i + 1).wait())
            pl.when(i < NP)(lambda: awo_copy(i).wait())
            bw_copy(i).wait()

        z = i >> 20
        proj = _Projector(lambda s: lhs_ref[0, s], z)
        norm = norm_tasks(jnp.minimum(i + 1, NR - 1), nxt_ref, z)

        def flip_task(r):
            flip_refs[0][0, :256, _tile(r)] = awo_ref[i % NP, _tile(r), :].T
            return flip_refs[0]

        def permute_task(r):
            t = _permute_heads([flip_refs[0][z, r:r + 2 * G, _tile(c)] for c in range(NT)])
            flip_refs[1][0, r:r + 2 * G, :] = jnp.concatenate(t, axis=1)
            return flip_refs[1]

        def unflip_task(r):
            tmp_ref[0, _tile(r), :] = flip_refs[1][z, :256, _tile(r)].T
            return tmp_ref

        def awo_tasks(p):
            return weight_tasks(wao_ref, i % NP, p, tmp_ref,
                                lambda r: tmp_ref[z, p * 256 + r:p * 256 + r + G, :])

        def logits_task(p, r):
            q = [qa_refs[p][z + c, r:r + 8, :] for c in (0, 1)]
            for w in range(WIN):
                win = slice(HALO + r - DIL * w, HALO + r - DIL * w + 8)
                a = q[0] * ka_refs[p][z, win, :] + q[1] * ka_refs[p][z + 1, win, :]
                if p > 0:
                    a = a + pa_refs[p - 1][z, w, r:r + 8, :]
                if p == NP - 1:
                    a = a + pltpu.roll(a, 64, 1)
                pa_refs[p][0, w, r:r + 8, :] = a
            return pa_refs[p]

        def fold_task(r):
            for w in range(WIN):
                a = pa_refs[NP - 1][z, w, r:r + 8, :]
                a = (a + pltpu.roll(a, 32, 1)) * QSCALE
                if r < DIL * w:
                    pos = i * R + r + lax.broadcasted_iota(I32, (8, 128), 0)
                    a = jnp.where(pos >= DIL * w, a, NEG * LOG2E)
                pa_refs[0][0, w, r:r + 8, :] = a
            return pa_refs[0]

        def softmax_task(r):
            logits = [pa_refs[0][z, w, r:r + 8, :] for w in range(WIN)]
            mx = functools.reduce(jnp.maximum, logits)
            e = [jnp.exp2(a - mx) for a in logits]
            inv = 1.0 / functools.reduce(jnp.add, e)
            for w in range(WIN):
                prob_ref[i, w, r:r + 8, :] = e[w] * inv
            return prob_ref

        def logits_tasks(p):
            return _tasks([qa_refs[p], ka_refs[p], *pa_refs[max(p - 1, 0):p]],
                          logits_task, p, range(0, R, 8))

        def keys(p):
            def emit(h, c, val):
                ka_refs[p][c, HALO + h * HR:HALO + (h + 1) * HR, :] = val
                return ka_refs[p]
            ka_refs[p][:, :HALO, :] = ka_refs[p][:, R:R + HALO, :]
            proj.strassen(wa_ref, NP + p, emit)

        def queries(p):
            def emit(h, c, val):
                qa_refs[p][c, h * HR:(h + 1) * HR, :] = val
                return qa_refs[p]
            proj.strassen(wa_ref, p, emit)

        def values(p):
            def emit(h, c, val):
                if h == 0:
                    va_refs[p][c, :HALO, :] = jnp.where(
                        i == 0, jnp.broadcast_to(val[0:1], (HALO, 128)), va_refs[p][c, :HALO, :])
                va_refs[p][c, rows(i, R, HALO + h * HR, HR, 8), :] = val
                return va_refs[p]
            proj.strassen(wa_ref, 2 * NP + p, emit)

        def early_mix(p):
            def store(s, rs, val):
                oa_ref[i, s, rs, _tile(p)] = val
                return oa_ref
            return mix_tasks(i, z, p, store)

        proj.spread(norm[0], 0, 5)
        proj.spread(norm[1], 6, 15)
        proj.spread(_tasks([awo_ref], flip_task, range(NT)), 2, 10)
        proj.spread(_tasks([flip_refs[0]], permute_task, range(0, 256, 2 * G)), 13, 29)
        proj.spread(_tasks([flip_refs[1]], unflip_task, range(NT)), 31, 39)
        for p in range(NP):
            proj.spread(logits_tasks(p), 14 * p + 15, 14 * p + 23)
        proj.spread(norm[2][:16], 23, 29)
        proj.spread(norm[2][16:], 37, 43)
        proj.spread([t for p in range(NP) for t in awo_tasks(p)], 51, 57)
        proj.spread(_tasks([pa_refs[NP - 1]], fold_task, range(0, R, 8)), 65, 72)
        proj.spread(_tasks([pa_refs[0]], softmax_task, range(0, R, 8)), 69, 77)
        proj.spread(bw_tasks(i, range(NBW)), 2, 50)
        for p in range(NMIX):
            proj.spread(early_mix(p), 76 + 8 * p / NMIX, 76 + 8 * (p + 1) / NMIX)
        proj.spread(advance_tasks(proj, D // 2), 77, 84)
        for p in range(NP):
            keys(p)
            queries(p)
        for p in range(NP):
            values(p)

    def late_mix(i, z, p, dst):
        def store(s, rs, val):
            dst[0, s, rs, _tile(p - NMIX)] = val
            return dst
        return mix_tasks(i, z, p, store)

    def local_output(i):
        z = i >> 20
        proj = _Projector(
            lambda s: jnp.concatenate([oa_ref[i, s], lhs_ref[0, s, :, :(NP - NMIX) * 128]][0 if NMIX else 1:], axis=1), z)
        nxt = jnp.minimum(i + 1, NR - 1)

        proj.spread([t for p in range(NMIX, NP) for t in late_mix(nxt, z, p, nxt_ref)], 0, 21)
        proj.spread(bw_tasks(i, range(NBW, 6)), 2, 28)
        proj.spread(advance_tasks(proj, (NP - NMIX) * 128), 21, 28)
        add_projection(i, proj, wao_ref)

    def add_projection(i, proj, w_ref):
        for p in range(NP):
            def emit(h, c, val, p=p):
                blk = (rows(i, R, h * HR, HR), _tile(2 * p + c))
                x_ref[blk] = (x_ref[blk].astype(F32) + val).astype(BF16)
            proj.strassen(w_ref, p, emit)

    def full_qkv(i):
        z = i >> 20
        proj = _Projector(lambda s: lhs_ref[0, s], z)
        norm = norm_tasks(jnp.minimum(i + 1, NR - 1), nxt_ref, z)

        def bwo_tasks(c):
            return weight_tasks(
                wbo_ref, i % 2 * 2 + c, i // 2, bwo_ref,
                lambda r: bwo_ref[rows(i // 2, 256, r, G), rows(i % 2 * 2 + c, 256)])

        proj.spread(norm[0], 0, 7)
        proj.spread(norm[1], 8, 22)
        proj.spread(bwo_tasks(0) + bwo_tasks(1), 22, 38)
        proj.spread(norm[2], 57, 73)
        proj.spread(advance_tasks(proj, D // 2), 77, 84)
        for p in range(NP):
            def emit(h, c, val, p=p):
                qt_ref[2 * p + c, i, :, h * HR:(h + 1) * HR] = _pack((val * QSCALE).T)
                return qt_ref
            proj.strassen(wb_ref, p, emit, 4)
        for p in range(NP):
            def emit(h, c, val, p=p):
                vt_ref[2 * p + c, i, :, h * HR:(h + 1) * HR] = _pack(val.T)
                return vt_ref
            proj.strassen(wb_ref, 2 * NP + p, emit, 4)
        for p in range(NP):
            def emit(h, c, val, p=p):
                k_ref[2 * p + c, rows(i, R // 2, h * HR // 2, HR // 2), :] = _pack(val)
                return k_ref
            proj.strassen(wb_ref, NP + p, emit)

    def attn_unit(u, j, nxt, cur, tail=False):
        hs = slice(j * DH // 2, (j + 1) * DH // 2)
        if cur is not None:
            m = jnp.broadcast_to(jnp.max(m_ref[u], axis=0, keepdims=True), (16, BQ))
        l = acc = m_acc = None
        for c in range(S // CK):
            def scores():
                parts = [qt_ref[nxt[0], nxt[1], hs, :]]
                if j > 0:
                    parts.insert(0, jnp.zeros((DH // 2 * j, BQ), I32))
                if j < 3:
                    parts.append(jnp.zeros((DH // 2 * (3 - j), BQ), I32))
                return _dot(_unpack(k_ref[nxt[0], c * CK // 2:(c + 1) * CK // 2, :]),
                            _unpack(jnp.concatenate(parts, axis=0)))

            late = tail and c == S // CK - 1
            if nxt is not None and not late:
                s = scores()
            if cur is not None:
                slabs = {}
                for r in reversed(range(CK // 16)):
                    p = jnp.exp2(s_ref[u, c * CK + r * 16:c * CK + (r + 1) * 16, :] - m)
                    ls = p[0:8] + p[8:16]
                    l = ls if l is None else l + ls
                    slabs[r] = p
                p = jnp.concatenate([slabs[r] for r in range(CK // 16)], axis=0).astype(BF16)
                off = c * CK % R
                a = _dot(_unpack(vt_ref[cur[0], c * CK // R, hs, off:off + CK]), p)
                acc = a if acc is None else acc + a
            if nxt is not None:
                if late:
                    s = scores()
                s_ref[u, c * CK:(c + 1) * CK, :] = s
                mx = jnp.max(s.reshape(CK // 8, 8, BQ), axis=0)
                m_acc = mx if m_acc is None else jnp.maximum(m_acc, mx)
        if nxt is not None:
            m_ref[u] = m_acc
        if cur is not None:
            inv = 1.0 / jnp.sum(l, axis=0, keepdims=True)
            ot_ref[cur[0], cur[1], j * DH:(j + 1) * DH, :] = acc * inv

    def full_attention():
        nqb = NQ // QB
        n_it = NT * nqb

        @pl.loop(0, QB)
        def _(b):
            for j in range(4):
                attn_unit(b * 4 + j, j, (0, b), None)

        @pl.loop(0, n_it - 1)
        def _(i):
            g, q = i // nqb, (i % nqb) * QB
            g2, q2 = (i + 1) // nqb, ((i + 1) % nqb) * QB
            for b in range(QB):
                for j in range(4):
                    attn_unit(b * 4 + j, j, (g2, q2 + b), (g, q + b),
                              tail=(b == QB - 1 and j == 3))

        @pl.loop(0, QB)
        def _(b):
            for j in range(4):
                attn_unit(b * 4 + j, j, None, (NT - 1, NQ - QB + b))

    def attn_out_tasks(i, dst):
        def task(p, s):
            term = _lhs_terms(ot_ref[2 * p, i, :, :HR], ot_ref[2 * p + 1, i, :, :HR],
                              ot_ref[2 * p, i, :, HR:], ot_ref[2 * p + 1, i, :, HR:])[s]
            dst[0, s, :HR // 2, _tile(p)] = _pack(term.T)
            return dst
        return [t for p in range(NP) for t in _tasks([], task, p, range(7))]

    @pl.loop(0, 2)
    def _(rep):
        run(*norm_tasks(0, lhs_ref, rep >> 20))
        pl.loop(0, NR)(functools.partial(local_qkv_attention, rep))

        @pl.when(rep == 0)
        def _():
            bwo_copy.wait()

        run(*[late_mix(0, rep >> 20, p, lhs_ref) for p in range(NMIX, NP)])
        pl.loop(0, NR)(local_output)
        run(*norm_tasks(0, lhs_ref, rep >> 20))
        pl.loop(0, NR)(full_qkv)
        full_attention()
        run(attn_out_tasks(0, lhs_ref))

        @pl.loop(0, NR)
        def _(i):
            tasks = attn_out_tasks(jnp.minimum(i + 1, NR - 1), nxt_ref)
            proj = _Projector(lambda s: lhs_ref[0, s], i >> 20)
            proj.spread(tasks, 0, 19)
            proj.spread(advance_tasks(proj, D // 2), 21, 28)
            add_projection(i, proj, wbo_ref)
            pl.when(rep == 1)(lambda: out_copy(i).start())

    for i in range(NR):
        out_copy(i).wait()


@jax.jit
def pallas_interleave_layers__sliding_local_dilated__softmax_full_mha__prompt_kernel(
    A_x: jax.Array,
    A_wqkv: jax.Array,
    A_wo: jax.Array,
    B_x: jax.Array,
    B_wqkv: jax.Array,
    B_wo: jax.Array,
):
    del B_x
    vmem = pltpu.VMEM
    dma = pltpu.SemaphoreType.DMA
    out = pl.pallas_call(
        _kernel,
        out_shape=jax.ShapeDtypeStruct((S, D), BF16),
        in_specs=[pl.BlockSpec(memory_space=pl.ANY)] * 5,
        out_specs=pl.BlockSpec(memory_space=pl.ANY),
        scratch_shapes=[
            vmem((S + 2 * PAD, D), BF16),
            vmem((1, 7, HR // 2, D // 2), I32),
            vmem((1, 7, HR // 2 + PAD, D // 2), I32),
            vmem((1, R, 128), F32),
            vmem((1, R, 128), F32),
            vmem((3 * NP, NP, 7, 64, 128), I32),
            vmem((NP, NP, 7, 64, 128), I32),
            vmem((3 * NP, NP, 7, 64, 128), I32),
            vmem((NP, NP, 7, 64, 128), I32),
            vmem((3 * NP, 256, D), BF16),
            vmem((NP, D + 2 * PAD, 256), BF16),
            vmem((NR, 256 + 2 * PAD, 3 * D // 2), BF16),
            vmem((D + 2 * PAD, D), BF16),
            [vmem((2, R + PAD, 128), F32)] * NP,
            [vmem((2, HALO + R + PAD, 128), F32)] * NP,
            [vmem((2, HALO + S + PAD, 128), F32)] * NP,
            [vmem((1, WIN, R + PAD, 128), F32)] * NP,
            vmem((NR, WIN, R + PAD, 128), F32),
            vmem((NR, 7, HR // 2, max(NMIX, 1) * 128), I32),
            [vmem((1, 256 + 2 * PAD, D), BF16)] * 2,
            vmem((1, D + 2 * PAD, 256), BF16),
            vmem((NT, NQ, 64, BQ), I32),
            vmem((NT, S // 2, 128), I32),
            vmem((NT, NR, 64, R), I32),
            vmem((NT, NQ, 128, BQ), F32),
            vmem((4 * QB, S, BQ), F32),
            vmem((4 * QB, 8, BQ), F32),
            dma((NR,)), dma((3 * NP,)), dma((NP,)), dma((NR,)), dma(()),
        ],
        compiler_params=pltpu.CompilerParams(vmem_limit_bytes=120 * 2 ** 20),
        name="interleave_layers",
    )(A_x.reshape(S, D), A_wqkv, A_wo, B_wqkv, B_wo)
    return out.reshape(A_x.shape)
```

```python
import functools
import math

import jax
import jax.numpy as jnp
from jax import lax
import jax.experimental.pallas as pl
import jax.experimental.pallas.tpu as pltpu

F32 = jnp.float32
BF16 = jnp.bfloat16
I32 = jnp.int32

S = 2048
D = 1024
H = 32
DH = D // H
NT = D // 128
NP = NT // 2
WIN, DIL = 8, 2
HALO = 16
EPS = 1e-5
NEG = -1e9
LOG2E = math.log2(math.e)
QSCALE = DH ** -0.5 * LOG2E

R = 256
NR = S // R
CK = 128
QB = 2
G = 16
PAD = 8
SLACK = 16
EARLY = 8

LHS_TERMS = (((1, 1, 0), (1, 1, 1)), ((1, 1, 1),), ((1, 0, 0), (1, 1, 1)), ((1, 1, 0), (-1, 0, 0)),
             ((1, 0, 1), (-1, 1, 1)), ((1, 0, 0), (1, 0, 1)), ((1, 0, 0),))
RHS_TERMS = (((1, 0, 0),), ((1, 1, 0), (-1, 0, 0)), ((1, 0, 0), (1, 1, 1)), ((1, 0, 0), (1, 0, 1)),
             ((1, 1, 0), (1, 1, 1)), ((1, 1, 1),), ((1, 0, 1), (-1, 1, 1)))


def _term(spec, block):
    out = block(*spec[0][1:])
    for sign, r, c in spec[1:]:
        out = out + block(r, c) if sign > 0 else out - block(r, c)
    return out


def _nested_terms(specs, outer, block):
    inner = {(r, c): _term(specs[outer], lambda a, b: block(2 * a + r, 2 * b + c))
             for r in (0, 1) for c in (0, 1)}
    return [_term(spec, lambda r, c: inner[r, c]) for spec in specs]


def _combine(s, m, x, y, emit):
    if s == 0:
        return m, None
    if s == 1:
        emit(1, 0, x() + m)
        return None, m
    if s == 2:
        return m - x(), y() + m
    if s == 3:
        return x() + m, None
    if s == 4:
        return None, y() + m
    if s == 5:
        emit(0, 0, y() - m)
        return None, m
    emit(1, 1, x() + m)
    emit(0, 1, y() + m)
    return None, None


def _strassen(product, emit):
    x = y = None
    for s in range(7):
        new_x, new_y = _combine(s, product(s), lambda: x, lambda: y, emit)
        x = x if new_x is None else new_x
        y = y if new_y is None else new_y


def _dot(a, b):
    return jnp.dot(a, b, preferred_element_type=F32)


def _pack(x):
    return pltpu.bitcast(x.astype(BF16), I32)


def _unpack(x):
    return pltpu.bitcast(x, BF16)


def _tile(t, n=128):
    return slice(t * n, (t + 1) * n)


def _tasks(reads, fn, *args):
    return [(reads, functools.partial(fn, *args[:-1], a)) for a in args[-1]]


def _run(tasks):
    for _, task in tasks:
        task()


class _Projector:
    def __init__(self, z):
        self.z = z
        self.results, self.deadlines, self.plan = [], {}, {}

    def spread(self, tasks, first, last):
        for n, task in enumerate(tasks):
            at = int(8 * (first + n * (last - first) / len(tasks)))
            self.plan.setdefault(at, []).append(task)

    def due(self, ref, at):
        if ref is not None:
            value = ref[(0,) * (len(ref.shape) - 2)
                        + (slice(32 // ref.dtype.itemsize), slice(128))]
            self.deadlines.setdefault(at, []).append(pltpu.bitcast(value, I32))

    def product(self, lhs, rhs):
        now = range(len(self.results), len(self.results) + lhs.shape[0] // 8)
        head = [lhs[_tile(n, 8), :128] for n in range(len(now))]
        for n, at in enumerate(now):
            for value in self.deadlines.pop(at, ()):
                head[n] = jnp.where(self.z > 0, value, head[n])
        lhs = jnp.concatenate([jnp.concatenate(head, axis=0), lhs[:, 128:]], axis=1)
        out = _dot(_unpack(lhs), _unpack(rhs))
        self.results += [(out, n * G) for n in range(len(now))]
        for at in now:
            for reads, task in self.plan.pop(at, ()):
                for ref in reads if at >= EARLY else ():
                    earlier, r = self.results[at - EARLY]
                    spare = slice(ref.shape[-2] - PAD, None)
                    ref[(self.z,) + (0,) * (len(ref.shape) - 3) + (spare, slice(128))] = (
                        earlier[r:r + PAD, :128].astype(ref.dtype))
                self.due(task(), at + 8 + SLACK)
        return out

    def paced(self, emit):
        return lambda *args: self.due(emit(*args), len(self.results) + 16)

    def one_level(self, lhs_ref, w_ref, emit):
        _strassen(lambda s: self.product(lhs_ref[s], w_ref[:, s].reshape(D // 4, 128)),
                  self.paced(emit))

    def two_levels(self, lhs_ref, w_ref, sum_refs, emit):
        emit = self.paced(emit)
        for s in range(7):
            def fold(r, c, m):
                new = _combine(s, m, lambda: sum_refs[r][c][0], lambda: sum_refs[r][c][1],
                               lambda a, b, val: emit(2 * a + r, 2 * b + c, val))
                for n, val in enumerate(new):
                    if val is not None:
                        sum_refs[r][c][self.z + n] = val
                return sum_refs[r][c]

            _strassen(lambda t: self.product(lhs_ref[7 * s + t],
                                             w_ref[:, 7 * s + t].reshape(D // 8, 256)),
                      self.paced(fold))


def _permute_heads(tiles):
    dtype = tiles[0].dtype
    tiles = [pltpu.bitcast(t, I32) for t in tiles]
    lane = lax.broadcasted_iota(I32, tiles[0].shape, 1)
    for b in (1, 2, 4):
        swap = ((lane >> 2) & b) != 0
        tiles = [jnp.where(swap, tiles[i ^ b], tiles[i]) for i in range(NT)]
    e, j, hl = lane >> 5, (lane >> 2) & 7, lane & 3
    tiles = [jnp.take_along_axis(tiles[i], hl * 32 + (j ^ i) * 4 + e, axis=1) for i in range(NT)]
    return [pltpu.bitcast(t, dtype) for t in tiles]


def _rows(i, n=R, off=0, size=None, align=None):
    return pl.ds(pl.multiple_of(i * n + off, align or size or n), size or n)


def _kernel(x_hbm, awqkv_hbm, awo_hbm, bwqkv_hbm, bwo_hbm, out_hbm,
            x_ref, chunk_ref, left_ref, mean_ref, rstd_ref, piece_ref,
            wa_ref, wao_ref, wb_ref, wbo_ref, awo_ref, bwqkv_ref, bwo_ref,
            x_sems, aw_sems, awo_sems, bw_sems, bwo_sem):
    def x_copy(i):
        return pltpu.make_async_copy(x_hbm.at[_rows(i)], x_ref.at[_rows(i)], x_sems.at[i])

    def out_copy(i):
        return pltpu.make_async_copy(x_ref.at[_rows(i)], out_hbm.at[_rows(i)], x_sems.at[i])

    def awo_copy(i):
        return pltpu.make_async_copy(
            awo_hbm.at[:, _rows(i, 256)], awo_ref.at[i, :D], awo_sems.at[i])

    def bw_copy(i):
        return pltpu.make_async_copy(
            bwqkv_hbm.at[:, _rows(i, 32)], bwqkv_ref.at[i], bw_sems.at[i])

    bwo_copy = pltpu.make_async_copy(bwo_hbm, bwo_ref, bwo_sem)

    def put_weights(w_ref, r, block):
        for s, spec in enumerate(RHS_TERMS):
            term = _pack(_term(spec, lambda a, b: block(a, b).astype(F32)))
            w_ref[s, r // 2:r // 2 + term.shape[0], :] = term

    def nested_weight_tasks(w_ref, dst, z, src):
        def fetch(a):
            piece_ref[z, a, :32, :] = src(a)
            return piece_ref

        def task(s, r, c):
            terms = _nested_terms(RHS_TERMS, s, lambda a, b: piece_ref[
                0, a, r:r + G, _tile(2 * b + c)].astype(F32))
            for t, term in enumerate(terms):
                dst[7 * s + t, r // 2:(r + G) // 2, _tile(c)] = _pack(term)
            return w_ref
        return _tasks([], fetch, range(4)) + [
            t for s in range(7) for r in (0, G) for t in _tasks([piece_ref], task, s, r, (0, 1))]

    def norm_tasks(i, z):
        def mean_task(r):
            x = x_ref[_rows(i, R, r, G), :]
            chunk_ref[z, r:r + G, :] = x
            mean_ref[z, r:r + G, :] = jnp.broadcast_to(
                jnp.mean(x.astype(F32), axis=-1, keepdims=True), (G, 128))
            return mean_ref

        def rstd_task(r):
            x = chunk_ref[0, r:r + G, :].astype(F32)
            mean = mean_ref[0, r:r + G, :]
            sq = functools.reduce(
                jnp.add, [jnp.square(x[:, _tile(t)] - mean) for t in range(NT)])
            var = jnp.sum(sq, axis=-1, keepdims=True) * (1.0 / D)
            rstd_ref[z, r:r + G, :] = lax.rsqrt(jnp.broadcast_to(var, (G, 128)) + EPS)
            return rstd_ref

        def scale_task(r):
            x = chunk_ref[0, r:r + G, :].astype(F32)
            mean, rstd = mean_ref[0, r:r + G, :], rstd_ref[0, r:r + G, :]
            for t in range(NT):
                left_ref[z, t, r:r + G, :] = (x[:, _tile(t)] - mean) * rstd
            return left_ref

        return [_tasks([chunk_ref], task, range(0, R, G))
                for task in (mean_task, rstd_task, scale_task)]

    def left_tasks(lhs_ref):
        def task(s, r):
            lhs_ref[s, r // 2:(r + G) // 2, :] = _pack(jnp.concatenate([
                _term(LHS_TERMS[s], lambda a, b: left_ref[
                    0, 2 * p + b, a * 128 + r:a * 128 + r + G, :]) for p in range(NP)], axis=1))
        return [t for s in range(7) for t in _tasks([left_ref], task, s, range(0, 128, G))]

    def nested_left_tasks(lhs_ref):
        def task(s, r, c):
            terms = _nested_terms(LHS_TERMS, s, lambda a, b: left_ref[
                0, 2 * b + c, a * 64 + r:a * 64 + r + G, :])
            for t, term in enumerate(terms):
                lhs_ref[7 * s + t, r // 2:(r + G) // 2, _tile(c)] = _pack(term)
        return [t for s in range(7) for r in range(0, 64, G)
                for t in _tasks([left_ref], task, s, r, (0, 1))]

    def add_to_stream(i, r, cols, val):
        blk = (_rows(i, R, r, val.shape[0]), cols)
        x_ref[blk] = (x_ref[blk].astype(F32) + val).astype(BF16)

    def start_up(awqkv_ref):
        def aw_copy(i):
            return pltpu.make_async_copy(awqkv_hbm.at[_rows(i % NP, 256), _rows(i // NP, D)],
                                         awqkv_ref.at[i], aw_sems.at[i])

        x_copy(0).start()
        for i in range(3 * NP):
            aw_copy(i).start()
        x_copy(1).start()
        awo_copy(0).start()
        bw_copy(0).start()

        @pl.loop(0, 3 * NP)
        def _(i):
            aw_copy(i).wait()
            t = _permute_heads([awqkv_ref[i, :, _tile(c)] for c in range(NT)])
            for p in range(NP):
                put_weights(wa_ref.at[i // NP * NP + p, i % NP], 0,
                            lambda a, b: t[2 * p + b][_tile(a)])

        for i in range(1, NR):
            if i + 1 < NR:
                x_copy(i + 1).start()
            if i < NP:
                awo_copy(i).start()
            bw_copy(i).start()
        bwo_copy.start()
        x_copy(0).wait()

    def local_layer(rep, lhs_ref, q_refs, k_refs, v_ref, sum_refs, prob_ref, held_ref, flip_refs):
        def qkv_softmax(i):
            @pl.when(rep == 0)
            def _():
                pl.when(i + 1 < NR)(lambda: x_copy(i + 1).wait())
                pl.when(i < NP)(lambda: awo_copy(i).wait())
                bw_copy(i).wait()

            z = i >> 20

            def flip_task(r):
                flip_refs[0][z, :256, _tile(r)] = awo_ref[i % NP, _tile(r), :].T
                return flip_refs[0]

            def permute_task(r):
                t = _permute_heads([flip_refs[0][0, r:r + 2 * G, _tile(c)] for c in range(NT)])
                flip_refs[1][z, r:r + 2 * G, :] = jnp.concatenate(t, axis=1)
                return flip_refs[1]

            def unflip_task(r):
                flip_refs[2][z, _tile(r), :] = flip_refs[1][0, :256, _tile(r)].T
                return flip_refs[2]

            def awo_task(p, r):
                put_weights(wao_ref.at[i % NP, p], r, lambda a, b: flip_refs[2][
                    0, (2 * p + a) * 128 + r:(2 * p + a) * 128 + r + G, _tile(b)])
                return wao_ref

            def bw_tasks(m):
                return nested_weight_tasks(
                    wb_ref, wb_ref.at[m, i], z, lambda a: bwqkv_ref[i, a, :, _tile(m, D)])

            def logits_task(p, r):
                q = [q_refs[p][c, r:r + 8, :] for c in (0, 1)]
                for w in range(WIN):
                    win = slice(HALO + r - DIL * w, HALO + r - DIL * w + 8)
                    a = q[0] * k_refs[p][0, win, :] + q[1] * k_refs[p][1, win, :]
                    if p > 0:
                        a = a + sum_refs[p - 1][0, w, r:r + 8, :]
                    if p == NP - 1:
                        a = a + pltpu.roll(a, 64, 1)
                    sum_refs[p][z, w, r:r + 8, :] = a
                return sum_refs[p]

            def fold_task(r):
                for w in range(WIN):
                    a = sum_refs[NP - 1][0, w, r:r + 8, :]
                    a = (a + pltpu.roll(a, 32, 1)) * QSCALE
                    if r < DIL * w:
                        pos = i * R + r + lax.broadcasted_iota(I32, (8, 128), 0)
                        a = jnp.where(pos >= DIL * w, a, NEG * LOG2E)
                    sum_refs[0][z, w, r:r + 8, :] = a
                return sum_refs[0]

            def softmax_task(r):
                logits = [sum_refs[0][0, w, r:r + 8, :] for w in range(WIN)]
                mx = functools.reduce(jnp.maximum, logits)
                e = [jnp.exp2(a - mx) for a in logits]
                inv = 1.0 / functools.reduce(jnp.add, e)
                for w in range(WIN):
                    prob_ref[i, w, r:r + 8, :] = e[w] * inv
                return prob_ref

            proj = _Projector(z)
            norm = norm_tasks(jnp.minimum(i + 1, NR - 1), z)
            proj.spread(norm[0], 0, 5)
            proj.spread(norm[1], 6, 15)
            proj.spread(norm[2], 23, 29)
            proj.spread(_tasks([awo_ref], flip_task, range(NT)), 2, 10)
            proj.spread(_tasks([flip_refs[0]], permute_task, range(0, 256, 2 * G)), 13, 29)
            proj.spread(_tasks([flip_refs[1]], unflip_task, range(NT)), 31, 39)
            proj.spread([t for p in range(NP) for t in
                         _tasks([flip_refs[2]], awo_task, p, range(0, 128, G))], 41, 57)
            proj.spread(bw_tasks(0) + bw_tasks(1) + bw_tasks(2), 1, 80)
            for p in range(NP):
                proj.spread(_tasks([q_refs[p], k_refs[p], *sum_refs[max(p - 1, 0):p]],
                                   logits_task, p, range(0, R, 8)), 14 * p + 15, 14 * p + 24)
            proj.spread(_tasks([sum_refs[NP - 1]], fold_task, range(0, R, 8)), 66, 73)
            proj.spread(_tasks([sum_refs[0]], softmax_task, range(0, R, 8)), 70, 79)
            proj.spread(left_tasks(lhs_ref), 77, 84)

            for p in range(NP):
                def emit_k(h, c, val):
                    k_refs[p][z + c, HALO + h * 128:HALO + (h + 1) * 128, :] = val
                    return k_refs[p]

                def emit_q(h, c, val):
                    q_refs[p][z + c, _tile(h), :] = val
                    return q_refs[p]

                k_refs[p][:, :HALO, :] = k_refs[p][:, R:R + HALO, :]
                proj.one_level(lhs_ref, wa_ref.at[NP + p], emit_k)
                proj.one_level(lhs_ref, wa_ref.at[p], emit_q)
            for p in range(NP):
                def emit_v(h, c, val):
                    v_ref[2 * p + c, _rows(i, R, HALO + h * 128, 128, 8), :] = val
                    return v_ref

                proj.one_level(lhs_ref, wa_ref.at[2 * NP + p], emit_v)

        def fetch(i, r):
            for t in range(NT):
                held_ref[0, t, r:r + 8, :] = v_ref[t, _rows(i, R, r, 8), :]
                if r < R:
                    held_ref[0, NT + t, r:r + 8, :] = prob_ref[i, t, r:r + 8, :]

        def mix_tasks(z, then):
            def task(r, p):
                a = [held_ref[0, NT + w, r:r + 8, :] for w in range(WIN)]
                for t in (2 * p, 2 * p + 1):
                    left_ref[z, t, r:r + 8, :] = functools.reduce(jnp.add, [
                        a[w] * held_ref[0, t, HALO + r - DIL * w:HALO + r - DIL * w + 8, :]
                        for w in range(WIN)])
                if p == NP - 1:
                    for done in range(r, r + 8 if r + 8 < R else R + HALO, 8):
                        fetch(then, done)
                return left_ref
            return [t for r in range(0, R, 8) for t in _tasks([held_ref], task, r, range(NP))]

        def output(i):
            proj = _Projector(i >> 20)
            proj.spread(mix_tasks(proj.z, jnp.minimum(i + 2, NR - 1)), 0, 21)
            proj.spread(left_tasks(lhs_ref), 21, 28)
            for p in range(NP):
                proj.one_level(lhs_ref, wao_ref.at[p], lambda h, c, val: add_to_stream(
                    i, h * 128, _tile(2 * p + c), val))

        for p in range(NP):
            k_refs[p][:, R:R + HALO, :] = jnp.zeros((2, HALO, 128), F32)
        _run(sum(norm_tasks(0, rep >> 20), []) + left_tasks(lhs_ref))
        pl.loop(0, NR)(qkv_softmax)
        for t in range(NT):
            v_ref[t, :HALO, :] = jnp.broadcast_to(v_ref[t, HALO:HALO + 1, :], (HALO, 128))
        for r in range(0, R + HALO, 8):
            fetch(0, r)
        held_ref[rep >> 20, 0, R + HALO:, :] = jnp.zeros((PAD, 128), F32)
        _run(mix_tasks(rep >> 20, 1) + left_tasks(lhs_ref))
        pl.loop(0, NR)(output)

    def full_layer(rep, lhs_ref, sum_refs, stage_refs, qt_ref, k_ref, vt_ref, ot_ref,
                   q_now, k_now, v_now, s_ref, m_ref):
        def qkv(i):
            z = i >> 20

            def flip_tasks(n, dst, scale):
                def task(t, h):
                    dst[t, i, :, _tile(h)] = _pack(scale(stage_refs[n][0, _tile(h), _tile(t)]).T)
                    return dst
                return [f for t in range(NT) for f in _tasks([stage_refs[n]], task, t, (0, 1))]

            def stage(n, r, c, val):
                stage_refs[n][z, _tile(r, 64), _tile(c, 256)] = val
                return stage_refs[n]

            def emit_k(r, c, val):
                val = _pack(val)
                for t in (0, 1):
                    k_ref[2 * c + t, _rows(i, R // 2, r * 32, 32), :] = val[:, _tile(t)]
                return k_ref

            proj = _Projector(z)
            norm = norm_tasks(jnp.minimum(i + 1, NR - 1), z)
            proj.spread(norm[0], 0, 6)
            proj.spread(norm[1], 7, 17)
            proj.spread(norm[2], 18, 25)
            proj.spread(flip_tasks(0, qt_ref, lambda q: q * QSCALE), 26, 44)
            proj.spread(nested_weight_tasks(
                wbo_ref, wbo_ref.at[i], z, lambda a: bwo_ref[a, _rows(i, 32), :]), 20, 50)
            proj.spread(flip_tasks(1, vt_ref, lambda v: v), 50.5, 68)
            tasks = nested_left_tasks(lhs_ref)
            proj.spread(tasks[:48], 52.5, 73.5)
            proj.two_levels(lhs_ref, wb_ref.at[0], sum_refs, functools.partial(stage, 0))
            proj.two_levels(lhs_ref, wb_ref.at[2], sum_refs, functools.partial(stage, 1))
            proj.two_levels(lhs_ref, wb_ref.at[1], sum_refs, emit_k)
            _run(tasks[48:])

        def attend(u, j, b, nxt, cur, then=None):
            hs = _tile(j, DH // 2)
            if cur is not None:
                m = jnp.broadcast_to(jnp.max(m_ref[u], axis=0, keepdims=True), (G, R))
            l = acc = m_acc = None
            for c in range(S // CK):
                def scores():
                    parts = [q_now[b, hs, :]]
                    if j > 0:
                        parts.insert(0, jnp.zeros((DH // 2 * j, R), I32))
                    if j < 3:
                        parts.append(jnp.zeros((DH // 2 * (3 - j), R), I32))
                    return _dot(_unpack(k_now[_tile(c, CK // 2), :]),
                                _unpack(jnp.concatenate(parts, axis=0)))

                late = then is not None and c == S // CK - 1
                if nxt is not None and not late:
                    s = scores()
                if cur is not None:
                    slabs = {}
                    for r in reversed(range(CK // G)):
                        p = jnp.exp2(s_ref[u, _tile(c * CK // G + r, G), :] - m)
                        ls = p[0:8] + p[8:16]
                        l = ls if l is None else l + ls
                        slabs[r] = p
                    p = jnp.concatenate([slabs[r] for r in range(CK // G)], axis=0).astype(BF16)
                    off = c * CK % R
                    a = _dot(_unpack(v_now[c * CK // R, hs, off:off + CK]), p)
                    acc = a if acc is None else acc + a
                if nxt is not None:
                    if late:
                        s = scores()
                    s_ref[u, _tile(c, CK), :] = s
                    mx = jnp.max(s.reshape(CK // 8, 8, R), axis=0)
                    m_acc = mx if m_acc is None else jnp.maximum(m_acc, mx)
                if then is not None:
                    k_now[_tile(c, CK // 2), :] = k_ref[then, _tile(c, CK // 2), :]
                    v_now[c * CK // R, :, off:off + CK] = vt_ref[nxt, c * CK // R, :, off:off + CK]
            if nxt is not None:
                m_ref[u] = m_acc
            if cur is not None:
                inv = 1.0 / jnp.sum(l, axis=0, keepdims=True)
                ot_ref[cur[0], cur[1], _tile(j, DH), :] = acc * inv

        def unflip_tasks(i, z):
            def task(t, h):
                left_ref[z, t, _tile(h), :] = ot_ref[t, i, :, _tile(h)].T
                return left_ref
            return [f for t in range(NT) for f in _tasks([], task, t, (0, 1))]

        def output(i):
            proj = _Projector(i >> 20)
            proj.spread(unflip_tasks(jnp.minimum(i + 1, NR - 1), proj.z), 0, 5)
            tasks = nested_left_tasks(lhs_ref)
            proj.spread(tasks[:48], 7, 24.5)
            proj.two_levels(lhs_ref, wbo_ref, sum_refs, lambda r, c, val: add_to_stream(
                i, r * 64, _tile(c, 256), val))
            _run(tasks[48:])
            pl.when(rep == 1)(lambda: out_copy(i).start())

        pl.when(rep == 0)(lambda: bwo_copy.wait())
        _run(sum(norm_tasks(0, rep >> 20), []) + nested_left_tasks(lhs_ref))
        pl.loop(0, NR)(qkv)
        nqb = NR // QB

        q_now[...] = qt_ref[0, :QB]
        k_now[...] = k_ref[0]
        v_now[...] = vt_ref[0]

        @pl.loop(0, QB)
        def _(b):
            for j in range(4):
                attend(b * 4 + j, j, b, 0, None)
            q_now[b] = qt_ref[0, QB + b]

        @pl.loop(0, NT * nqb - 1)
        def _(i):
            later = jnp.minimum(i + 2, NT * nqb - 1)
            for b in range(QB):
                for j in range(4):
                    attend(b * 4 + j, j, b, (i + 1) // nqb, (i // nqb, i % nqb * QB + b),
                           later // nqb if b == QB - 1 and j == 3 else None)
                q_now[b] = qt_ref[later // nqb, later % nqb * QB + b]

        @pl.loop(0, QB)
        def _(b):
            for j in range(4):
                attend(b * 4 + j, j, b, None, (NT - 1, NR - QB + b))

        _run(unflip_tasks(0, rep >> 20) + nested_left_tasks(lhs_ref))
        pl.loop(0, NR)(output)

    vmem = pltpu.VMEM
    pl.run_scoped(start_up, vmem((3 * NP, 256, D), BF16))

    @pl.loop(0, 2)
    def _(rep):
        pl.run_scoped(
            functools.partial(local_layer, rep),
            vmem((7, 64, D // 2), I32),
            [vmem((2, R + PAD, 128), F32)] * NP,
            [vmem((2, HALO + R + PAD, 128), F32)] * NP,
            vmem((NT, HALO + S, 128), F32),
            [vmem((1, WIN, R + PAD, 128), F32)] * NP,
            vmem((NR, WIN, R, 128), F32),
            vmem((1, NT + WIN, HALO + R + PAD, 128), F32),
            [vmem((1, 256 + G, D), BF16)] * 2 + [vmem((1, D + G, 256), BF16)])
        pl.run_scoped(
            functools.partial(full_layer, rep),
            vmem((49, 32, D // 4), I32),
            [[vmem((2, 64, 256), F32)] * 2] * 2,
            [vmem((1, R + PAD, D), F32)] * 2,
            vmem((NT, NR, 64, R), I32),
            vmem((NT, S // 2, 128), I32),
            vmem((NT, NR, 64, R), I32),
            vmem((NT, NR, 128, R), F32),
            vmem((QB, 64, R), I32),
            vmem((S // 2, 128), I32),
            vmem((NR, 64, R), I32),
            vmem((4 * QB, S, R), F32),
            vmem((4 * QB, 8, R), F32))

    for i in range(NR):
        out_copy(i).wait()


@jax.jit
def pallas_interleave_layers__sliding_local_dilated__softmax_full_mha__prompt_kernel(
    A_x: jax.Array,
    A_wqkv: jax.Array,
    A_wo: jax.Array,
    B_x: jax.Array,
    B_wqkv: jax.Array,
    B_wo: jax.Array,
):
    del B_x
    vmem = pltpu.VMEM
    dma = pltpu.SemaphoreType.DMA
    out = pl.pallas_call(
        _kernel,
        out_shape=jax.ShapeDtypeStruct((S, D), BF16),
        in_specs=[pl.BlockSpec(memory_space=pl.ANY)] * 5,
        out_specs=pl.BlockSpec(memory_space=pl.ANY),
        scratch_shapes=[
            vmem((S, D), BF16),
            vmem((1, R + G, D), BF16),
            vmem((1, NT, R + PAD, 128), F32),
            vmem((1, R, 128), F32),
            vmem((1, R, 128), F32),
            vmem((1, 4, 32 + G, D), BF16),
            vmem((3 * NP, NP, 7, 64, 128), I32),
            vmem((NP, NP, 7, 64, 128), I32),
            vmem((3, NR, 49, 16, 256), I32),
            vmem((NR, 49, 16, 256), I32),
            vmem((NP, D + G, 256), BF16),
            vmem((NR, 4, 32, 3 * D), BF16),
            vmem((4, 256, D), BF16),
            dma((NR,)), dma((3 * NP,)), dma((NP,)), dma((NR,)), dma(()),
        ],
        compiler_params=pltpu.CompilerParams(vmem_limit_bytes=120 * 2 ** 20),
        name="interleave_layers",
    )(A_x.reshape(S, D), A_wqkv, A_wo, B_wqkv.reshape(4, 256, 3 * D), B_wo.reshape(4, 256, D))
    return out.reshape(A_x.shape)
```

```python
import functools
import math

import jax
import jax.numpy as jnp
from jax import lax
import jax.experimental.pallas as pl
import jax.experimental.pallas.tpu as pltpu

F32 = jnp.float32
BF16 = jnp.bfloat16
I32 = jnp.int32

S = 2048
D = 1024
H = 32
DH = D // H
NT = D // 128
NP = NT // 2
WIN, DIL = 8, 2
HALO = 16
EPS = 1e-5
NEG = -1e9
LOG2E = math.log2(math.e)
QSCALE = DH ** -0.5 * LOG2E

R = 256
NR = S // R
CK = 128
QB = 2
G = 16
PAD = 8

LHS_TERMS = (((1, 1, 0), (1, 1, 1)), ((1, 1, 1),), ((1, 0, 0), (1, 1, 1)), ((1, 1, 0), (-1, 0, 0)),
             ((1, 0, 1), (-1, 1, 1)), ((1, 0, 0), (1, 0, 1)), ((1, 0, 0),))
RHS_TERMS = (((1, 0, 0),), ((1, 1, 0), (-1, 0, 0)), ((1, 0, 0), (1, 1, 1)), ((1, 0, 0), (1, 0, 1)),
             ((1, 1, 0), (1, 1, 1)), ((1, 1, 1),), ((1, 0, 1), (-1, 1, 1)))


def _term(spec, block):
    out = block(*spec[0][1:])
    for sign, r, c in spec[1:]:
        out = out + block(r, c) if sign > 0 else out - block(r, c)
    return out


def _nested_terms(specs, outer, block):
    inner = {(r, c): _term(specs[outer], lambda a, b: block(2 * a + r, 2 * b + c))
             for r in (0, 1) for c in (0, 1)}
    return [_term(spec, lambda r, c: inner[r, c]) for spec in specs]


def _combine(s, m, x, y, emit):
    if s == 0:
        return m, None
    if s == 1:
        emit(1, 0, x() + m)
        return None, m
    if s == 2:
        return m - x(), y() + m
    if s == 3:
        return x() + m, None
    if s == 4:
        return None, y() + m
    if s == 5:
        emit(0, 0, y() - m)
        return None, m
    emit(1, 1, x() + m)
    emit(0, 1, y() + m)
    return None, None


def _strassen(product, emit):
    x = y = None
    for s in range(7):
        new_x, new_y = _combine(s, product(s), lambda: x, lambda: y, emit)
        x = x if new_x is None else new_x
        y = y if new_y is None else new_y


def _dot(a, b):
    return jnp.dot(a, b, preferred_element_type=F32)


def _pack(x):
    return pltpu.bitcast(x.astype(BF16), I32)


def _unpack(x):
    return pltpu.bitcast(x, BF16)


def _tile(t, n=128):
    return slice(t * n, (t + 1) * n)


def _tasks(reads, fn, *args):
    return [(reads, functools.partial(fn, *args[:-1], a)) for a in args[-1]]


def _run(tasks):
    for _, task in tasks:
        task()


class _Projector:
    def __init__(self, z, early=8, slack=24):
        self.z, self.early, self.slack = z, early, slack
        self.never = jnp.full((8, 128), z) > 0
        self.results, self.deadlines, self.plan = [], {}, {}

    def spread(self, tasks, first, last):
        for n, task in enumerate(tasks):
            at = int(8 * (first + n * (last - first) / len(tasks)))
            self.plan.setdefault(at, []).append(task)

    def due(self, ref, at):
        if ref is not None:
            value = ref[(0,) * (len(ref.shape) - 2)
                        + (slice(32 // ref.dtype.itemsize), slice(128))]
            self.deadlines.setdefault(at, []).append(pltpu.bitcast(value, I32))

    def product(self, lhs, rhs):
        now = range(len(self.results), len(self.results) + lhs.shape[0] // 8)
        head = [lhs[_tile(n, 8), :128] for n in range(len(now))]
        for n, at in enumerate(now):
            if at in self.deadlines:
                value = functools.reduce(jnp.bitwise_or, self.deadlines.pop(at))
                head[n] = jnp.where(self.never, value, head[n])
        lhs = jnp.concatenate([jnp.concatenate(head, axis=0), lhs[:, 128:]], axis=1)
        out = _dot(_unpack(lhs), _unpack(rhs))
        self.results += [(out, n * G) for n in range(len(now))]
        for at in now:
            for reads, task in self.plan.pop(at, ()):
                for ref in reads if at >= self.early else ():
                    earlier, r = self.results[at - self.early]
                    spare = slice(ref.shape[-2] - PAD, None)
                    ref[(self.z,) + (0,) * (len(ref.shape) - 3) + (spare, slice(128))] = (
                        earlier[r:r + PAD, :128].astype(ref.dtype))
                self.due(task(), at + self.slack)
        return out

    def paced(self, emit):
        return lambda *args: self.due(emit(*args), len(self.results) + 16)

    def one_level(self, lhs_ref, w_ref, emit):
        _strassen(lambda s: self.product(lhs_ref[s], w_ref[:, s].reshape(D // 4, 128)),
                  self.paced(emit))

    def two_levels(self, lhs_ref, w_ref, sum_refs, emit):
        emit = self.paced(emit)
        for s in range(7):
            def fold(r, c, m):
                new = _combine(s, m, lambda: sum_refs[r][c][0], lambda: sum_refs[r][c][1],
                               lambda a, b, val: emit(2 * a + r, 2 * b + c, val))
                for n, val in enumerate(new):
                    if val is not None:
                        sum_refs[r][c][self.z + n] = val
                return sum_refs[r][c]

            _strassen(lambda t: self.product(lhs_ref[7 * s + t],
                                             w_ref[:, 7 * s + t].reshape(D // 8, 256)),
                      self.paced(fold))


def _permute_heads(tiles):
    dtype = tiles[0].dtype
    tiles = [pltpu.bitcast(t, I32) for t in tiles]
    lane = lax.broadcasted_iota(I32, tiles[0].shape, 1)
    for b in (1, 2, 4):
        swap = ((lane >> 2) & b) != 0
        tiles = [jnp.where(swap, tiles[i ^ b], tiles[i]) for i in range(NT)]
    e, j, hl = lane >> 5, (lane >> 2) & 7, lane & 3
    tiles = [jnp.take_along_axis(tiles[i], hl * 32 + (j ^ i) * 4 + e, axis=1) for i in range(NT)]
    return [pltpu.bitcast(t, dtype) for t in tiles]


def _rows(i, n=R, off=0, size=None, align=None):
    return pl.ds(pl.multiple_of(i * n + off, align or size or n), size or n)


def _kernel(x_hbm, awqkv_hbm, awo_hbm, bwqkv_hbm, bwo_hbm, out_hbm,
            x_ref, chunk_ref, left_ref, mean_ref, rstd_ref, piece_ref, lhs1_ref, v_ref, prob_ref,
            wa_ref, wao_ref, wb_ref, wbo_ref, awo_ref, bwqkv_ref, bwo_ref,
            x_sems, aw_sems, awo_sems, bw_sem, bwo_sem):
    def x_copy(i):
        return pltpu.make_async_copy(x_hbm.at[_rows(i)], x_ref.at[_rows(i)], x_sems.at[i])

    def out_copy(i):
        return pltpu.make_async_copy(x_ref.at[_rows(i)], out_hbm.at[_rows(i)], x_sems.at[i])

    def awo_copy(i):
        return pltpu.make_async_copy(
            awo_hbm.at[:, _rows(i, 256)], awo_ref.at[i, :D], awo_sems.at[i])

    bw_copy = pltpu.make_async_copy(bwqkv_hbm, bwqkv_ref, bw_sem)
    bwo_copy = pltpu.make_async_copy(bwo_hbm, bwo_ref, bwo_sem)

    def put_weights(w_ref, r, block):
        for s, spec in enumerate(RHS_TERMS):
            term = _pack(_term(spec, lambda a, b: block(a, b).astype(F32)))
            w_ref[s, r // 2:r // 2 + term.shape[0], :] = term

    def nested_weight_tasks(w_ref, dst, z, src):
        def fetch(a):
            piece_ref[z, a, :32, :] = src(a)
            return piece_ref

        def task(s, r, c):
            terms = _nested_terms(RHS_TERMS, s, lambda a, b: piece_ref[
                0, a, r:r + G, _tile(2 * b + c)].astype(F32))
            for t, term in enumerate(terms):
                dst[7 * s + t, r // 2:(r + G) // 2, _tile(c)] = _pack(term)
            return w_ref
        return _tasks([], fetch, range(4)) + [
            t for s in range(7) for r in (0, G) for t in _tasks([piece_ref], task, s, r, (0, 1))]

    def norm_tasks(i, z):
        def mean_task(r):
            x = x_ref[_rows(i, R, r, G), :]
            chunk_ref[z, r:r + G, :] = x
            mean_ref[z, r:r + G, :] = jnp.broadcast_to(
                jnp.mean(x.astype(F32), axis=-1, keepdims=True), (G, 128))
            return mean_ref

        def rstd_task(r):
            x = chunk_ref[0, r:r + G, :].astype(F32)
            mean = mean_ref[0, r:r + G, :]
            sq = functools.reduce(
                jnp.add, [jnp.square(x[:, _tile(t)] - mean) for t in range(NT)])
            var = jnp.sum(sq, axis=-1, keepdims=True) * (1.0 / D)
            rstd_ref[z, r:r + G, :] = lax.rsqrt(jnp.broadcast_to(var, (G, 128)) + EPS)
            return rstd_ref

        def scale_task(r):
            x = chunk_ref[0, r:r + G, :].astype(F32)
            mean, rstd = mean_ref[0, r:r + G, :], rstd_ref[0, r:r + G, :]
            for t in range(NT):
                left_ref[z, t, r:r + G, :] = (x[:, _tile(t)] - mean) * rstd
            return left_ref

        return [_tasks([chunk_ref], task, range(0, R, G))
                for task in (mean_task, rstd_task, scale_task)]

    def left_tasks(lhs_ref, src=left_ref, done=None):
        def task(s, r):
            lhs_ref[s, r // 2:(r + G) // 2, :] = _pack(jnp.concatenate([
                _term(LHS_TERMS[s], lambda a, b: src[
                    0, 2 * p + b, a * 128 + r:a * 128 + r + G, :]) for p in range(NP)], axis=1))
            return done
        return [t for s in range(7) for t in _tasks([src], task, s, range(0, 128, G))]

    def nested_left_tasks(lhs_ref):
        def task(s, r, c):
            terms = _nested_terms(LHS_TERMS, s, lambda a, b: left_ref[
                0, 2 * b + c, a * 64 + r:a * 64 + r + G, :])
            for t, term in enumerate(terms):
                lhs_ref[7 * s + t, r // 2:(r + G) // 2, _tile(c)] = _pack(term)
        return [t for s in range(7) for r in range(0, 64, G)
                for t in _tasks([left_ref], task, s, r, (0, 1))]

    def add_to_stream(i, r, cols, val):
        blk = (_rows(i, R, r, val.shape[0]), cols)
        x_ref[blk] = (x_ref[blk].astype(F32) + val).astype(BF16)

    def start_up(awqkv_ref):
        def aw_copy(i):
            return pltpu.make_async_copy(awqkv_hbm.at[_rows(i % NP, 256), _rows(i // NP, D)],
                                         awqkv_ref.at[i], aw_sems.at[i])

        x_copy(0).start()
        for i in range(3 * NP):
            aw_copy(i).start()
        x_copy(1).start()
        awo_ref[NP] = jnp.zeros(awo_ref.shape[1:], BF16)
        v_ref[...] = jnp.zeros(v_ref.shape, F32)
        prob_ref[...] = jnp.zeros(prob_ref.shape, F32)
        x_copy(0).wait()
        _run(sum(norm_tasks(0, 0), []) + left_tasks(lhs1_ref))

        @pl.loop(0, 3 * NP)
        def _(i):
            aw_copy(i).wait()
            t = _permute_heads([awqkv_ref[i, :, _tile(c)] for c in range(NT)])
            for p in range(NP):
                put_weights(wa_ref.at[i // NP * NP + p, i % NP], 0,
                            lambda a, b: t[2 * p + b][_tile(a)])

        for i in range(2, NR):
            x_copy(i).start()
        for i in range(NP):
            awo_copy(i).start()
        bw_copy.start()
        bwo_copy.start()

    def local_layer(rep, q_refs, k_refs, sum_refs, mix_ref, o_ref, flip_refs):
        lhs_ref = lhs1_ref

        def mix_tasks(i, z):
            def task(r, p):
                o = {}
                for w in range(WIN):
                    a = prob_ref[0, w, r:r + 8, :]
                    for t in (2 * p, 2 * p + 1):
                        b = a * v_ref[0, t, HALO + r - DIL * w:HALO + r - DIL * w + 8, :]
                        o[t] = o[t] + b if w else b
                for t, val in o.items():
                    mix_ref[z, t, r:r + 8, :] = val
                return mix_ref
            return ([t for r in range(0, R, 8) for t in _tasks([v_ref], task, r, range(NP))],
                    left_tasks(o_ref.at[i], mix_ref, o_ref))

        def qkv_softmax(i):
            @pl.when(rep == 0)
            def _():
                pl.when(i + 1 < NR)(lambda: x_copy(i + 1).wait())
                pl.when(i >= NP)(lambda: awo_copy(i - NP).wait())

            z = i >> 20

            def flip_task(r):
                flip_refs[0][z, :256, _tile(r)] = awo_ref[jnp.where(i < NP, NP, i - NP), _tile(r), :].T
                return flip_refs[0]

            def permute_task(r):
                t = _permute_heads([flip_refs[0][0, r:r + 2 * G, _tile(c)] for c in range(NT)])
                flip_refs[1][z, r:r + 2 * G, :] = jnp.concatenate(t, axis=1)
                return flip_refs[1]

            def unflip_task(r):
                flip_refs[2][z, _tile(r), :] = flip_refs[1][0, :256, _tile(r)].T
                return flip_refs[2]

            def awo_task(p, r):
                put_weights(wao_ref.at[i % NP, p], r, lambda a, b: flip_refs[2][
                    0, (2 * p + a) * 128 + r:(2 * p + a) * 128 + r + G, _tile(b)])
                return wao_ref

            def logits_task(p, r):
                q = [q_refs[p][c, r:r + 8, :] for c in (0, 1)]
                for w in range(WIN):
                    win = slice(HALO + r - DIL * w, HALO + r - DIL * w + 8)
                    a = q[0] * k_refs[p][0, win, :] + q[1] * k_refs[p][1, win, :]
                    if p > 0:
                        a = a + sum_refs[p - 1][0, w, r:r + 8, :]
                    if p == NP - 1:
                        a = a + pltpu.roll(a, 64, 1)
                    sum_refs[p][z, w, r:r + 8, :] = a
                return sum_refs[p]

            def fold_task(r):
                for w in range(WIN):
                    a = sum_refs[NP - 1][0, w, r:r + 8, :]
                    a = (a + pltpu.roll(a, 32, 1)) * QSCALE
                    if r < DIL * w:
                        pos = i * R + r + lax.broadcasted_iota(I32, (8, 128), 0)
                        a = jnp.where(pos >= DIL * w, a, NEG * LOG2E)
                    sum_refs[r // 128][z, w, r:r + 8, :] = a
                return sum_refs[r // 128]

            def softmax_task(r):
                logits = [sum_refs[r // 128][0, w, r:r + 8, :] for w in range(WIN)]
                mx = functools.reduce(jnp.maximum, logits)
                e = [jnp.exp2(a - mx) for a in logits]
                inv = 1.0 / functools.reduce(jnp.add, e)
                for w in range(WIN):
                    prob_ref[z, w, r:r + 8, :] = e[w] * inv
                return prob_ref

            proj = _Projector(z, 4, 28)
            norm = norm_tasks(jnp.minimum(i + 1, NR - 1), z)
            proj.spread(norm[0], 0, 5)
            proj.spread(norm[1], 6, 15)
            proj.spread(norm[2], 23, 29)
            proj.spread(_tasks([awo_ref], flip_task, range(NT)), 2, 10)
            proj.spread(_tasks([flip_refs[0]], permute_task, range(0, 256, 2 * G)), 13, 29)
            proj.spread(_tasks([flip_refs[1]], unflip_task, range(NT)), 31, 39)
            proj.spread([t for p in range(NP) for t in
                         _tasks([flip_refs[2]], awo_task, p, range(0, 128, G))], 41, 57)
            mix = mix_tasks(jnp.maximum(i - 1, 0), z)
            proj.spread(mix[0][:32], 1, 15)
            proj.spread(mix[0][32:48], 15, 24)
            proj.spread(mix[0][48:64], 24, 29)
            proj.spread(mix[0][64:80], 29, 38)
            proj.spread(mix[0][80:100], 38, 43)
            proj.spread(mix[0][100:112], 43, 52)
            proj.spread(mix[0][112:], 52, 56)
            proj.spread(mix[1], 58, 78)
            for p in range(NP):
                proj.spread(_tasks([k_refs[p], *sum_refs[max(p - 1, 0):p]], logits_task, p,
                                   range(0, R, 8)), 14 * p + 15, 14 * p + 24)
            proj.spread(_tasks([sum_refs[NP - 1]], fold_task, range(0, R, 8)), 66, 73)
            proj.spread([t for h in (0, 1) for t in _tasks(
                [sum_refs[h]], softmax_task, range(h * 128, h * 128 + 128, 8))], 70, 79)
            proj.spread(left_tasks(lhs_ref), 77, 84)

            for p in range(NP):
                def emit_k(h, c, val):
                    k_refs[p][z + c, HALO + h * 128:HALO + (h + 1) * 128, :] = val
                    return k_refs[p]

                def emit_q(h, c, val):
                    q_refs[p][z + c, _tile(h), :] = val
                    return q_refs[p]

                k_refs[p][:, :HALO, :] = k_refs[p][:, R:R + HALO, :]
                proj.one_level(lhs_ref, wa_ref.at[NP + p], emit_k)
                proj.one_level(lhs_ref, wa_ref.at[p], emit_q)
            v_ref[0, :, :HALO, :] = v_ref[0, :, R:R + HALO, :]
            for p in range(NP):
                def emit_v(h, c, val):
                    if h == 0:
                        v_ref[z, 2 * p + c, :HALO, :] = jnp.where(
                            i == 0, jnp.broadcast_to(val[:1], (HALO, 128)),
                            v_ref[0, 2 * p + c, :HALO, :])
                    v_ref[z, 2 * p + c, HALO + h * 128:HALO + (h + 1) * 128, :] = val
                    return v_ref

                proj.one_level(lhs_ref, wa_ref.at[2 * NP + p], emit_v)

        def output(i):
            def fetch(s, r):
                lhs_ref[s, r:r + 8, :] = o_ref[jnp.minimum(i + 1, NR - 1), s, r:r + 8, :]

            proj = _Projector(i >> 20)
            proj.spread([t for m in range(3) for t in nested_weight_tasks(
                wb_ref, wb_ref.at[m, i], proj.z,
                lambda a, m=m: bwqkv_ref[a, _rows(i, 32), _tile(m, D)])], 0, 28)
            proj.spread([t for s in range(7)
                         for t in _tasks([o_ref], fetch, s, range(0, 64, 8))], 21, 28)
            for p in range(NP):
                proj.one_level(lhs_ref, wao_ref.at[p], lambda h, c, val: add_to_stream(
                    i, h * 128, _tile(2 * p + c), val))

        for p in range(NP):
            k_refs[p][:, R:R + HALO, :] = jnp.zeros((2, HALO, 128), F32)
        pl.loop(0, NR)(qkv_softmax)
        pl.when(rep == 0)(lambda: bw_copy.wait())
        _run(sum(mix_tasks(NR - 1, rep >> 20), []))
        lhs_ref[...] = o_ref[0, :, :64, :]
        pl.loop(0, NR)(output)

    def full_layer(rep, lhs_ref, sum_refs, stage_refs, qt_ref, k_ref, vt_ref, ot_ref,
                   q_now, k_now, v_now, s_ref, m_ref):
        def qkv(i):
            z = i >> 20

            def flip_tasks(n, dst, scale):
                def task(t, h):
                    dst[t, i, :, _tile(h)] = _pack(scale(stage_refs[n][0, _tile(h), _tile(t)]).T)
                    return dst
                return [f for t in range(NT) for f in _tasks([stage_refs[n]], task, t, (0, 1))]

            def stage(n, r, c, val):
                stage_refs[n][z, _tile(r, 64), _tile(c, 256)] = val
                return stage_refs[n]

            def emit_k(r, c, val):
                val = _pack(val)
                for t in (0, 1):
                    k_ref[2 * c + t, _rows(i, R // 2, r * 32, 32), :] = val[:, _tile(t)]
                return k_ref

            proj = _Projector(z)
            norm = norm_tasks(jnp.minimum(i + 1, NR - 1), z)
            proj.spread(norm[0], 0, 6)
            proj.spread(norm[1], 7, 17)
            proj.spread(norm[2], 18, 25)
            proj.spread(flip_tasks(0, qt_ref, lambda q: q * QSCALE), 26, 44)
            proj.spread(nested_weight_tasks(
                wbo_ref, wbo_ref.at[i], z, lambda a: bwo_ref[a, _rows(i, 32), :]), 20, 50)
            proj.spread(flip_tasks(1, vt_ref, lambda v: v), 50.5, 68)
            tasks = nested_left_tasks(lhs_ref)
            proj.spread(tasks[:48], 52.5, 73.5)
            proj.two_levels(lhs_ref, wb_ref.at[0], sum_refs, functools.partial(stage, 0))
            proj.two_levels(lhs_ref, wb_ref.at[2], sum_refs, functools.partial(stage, 1))
            proj.two_levels(lhs_ref, wb_ref.at[1], sum_refs, emit_k)
            _run(tasks[48:])

        def attend(u, j, b, nxt, cur, then=None):
            hs = _tile(j, DH // 2)
            if cur is not None:
                m = jnp.broadcast_to(jnp.max(m_ref[u], axis=0, keepdims=True), (G, R))
            l = acc = m_acc = None
            for c in range(S // CK):
                def scores():
                    parts = [q_now[b, hs, :]]
                    if j > 0:
                        parts.insert(0, jnp.zeros((DH // 2 * j, R), I32))
                    if j < 3:
                        parts.append(jnp.zeros((DH // 2 * (3 - j), R), I32))
                    return _dot(_unpack(k_now[_tile(c, CK // 2), :]),
                                _unpack(jnp.concatenate(parts, axis=0)))

                late = then is not None and c == S // CK - 1
                if nxt is not None and not late:
                    s = scores()
                if cur is not None:
                    slabs = {}
                    for r in reversed(range(CK // G)):
                        p = jnp.exp2(s_ref[u, _tile(c * CK // G + r, G), :] - m)
                        ls = p[0:8] + p[8:16]
                        l = ls if l is None else l + ls
                        slabs[r] = p
                    p = jnp.concatenate([slabs[r] for r in range(CK // G)], axis=0).astype(BF16)
                    off = c * CK % R
                    a = _dot(_unpack(v_now[c * CK // R, hs, off:off + CK]), p)
                    acc = a if acc is None else acc + a
                if nxt is not None:
                    if late:
                        s = scores()
                    s_ref[u, _tile(c, CK), :] = s
                    mx = jnp.max(s.reshape(CK // 8, 8, R), axis=0)
                    m_acc = mx if m_acc is None else jnp.maximum(m_acc, mx)
                if then is not None:
                    k_now[_tile(c, CK // 2), :] = k_ref[then, _tile(c, CK // 2), :]
                    v_now[c * CK // R, :, off:off + CK] = vt_ref[nxt, c * CK // R, :, off:off + CK]
            if nxt is not None:
                m_ref[u] = m_acc
            if cur is not None:
                inv = 1.0 / jnp.sum(l, axis=0, keepdims=True)
                ot_ref[cur[0], cur[1], _tile(j, DH), :] = acc * inv

        def unflip_tasks(i, z):
            def task(t, h):
                left_ref[z, t, _tile(h), :] = ot_ref[t, i, :, _tile(h)].T
                return left_ref
            return [f for t in range(NT) for f in _tasks([], task, t, (0, 1))]

        def output(i):
            proj = _Projector(i >> 20)
            proj.spread(unflip_tasks(jnp.minimum(i + 1, NR - 1), proj.z), 0, 5)
            tasks = nested_left_tasks(lhs_ref)
            proj.spread(tasks[:48], 7, 24.5)
            proj.two_levels(lhs_ref, wbo_ref, sum_refs, lambda r, c, val: add_to_stream(
                i, r * 64, _tile(c, 256), val))
            _run(tasks[48:])
            pl.when(rep == 1)(lambda: out_copy(i).start())

        pl.when(rep == 0)(lambda: bwo_copy.wait())
        _run(sum(norm_tasks(0, rep >> 20), []) + nested_left_tasks(lhs_ref))
        pl.loop(0, NR)(qkv)
        nqb = NR // QB

        q_now[...] = qt_ref[0, :QB]
        k_now[...] = k_ref[0]
        v_now[...] = vt_ref[0]

        @pl.loop(0, QB)
        def _(b):
            for j in range(4):
                attend(b * 4 + j, j, b, 0, None)
            q_now[b] = qt_ref[0, QB + b]

        @pl.loop(0, NT * nqb - 1)
        def _(i):
            later = jnp.minimum(i + 2, NT * nqb - 1)
            for b in range(QB):
                for j in range(4):
                    attend(b * 4 + j, j, b, (i + 1) // nqb, (i // nqb, i % nqb * QB + b),
                           later // nqb if b == QB - 1 and j == 3 else None)
                q_now[b] = qt_ref[later // nqb, later % nqb * QB + b]

        @pl.loop(0, QB)
        def _(b):
            for j in range(4):
                attend(b * 4 + j, j, b, None, (NT - 1, NR - QB + b))

        _run(unflip_tasks(0, rep >> 20) + nested_left_tasks(lhs_ref))
        pl.loop(0, NR)(output)

    vmem = pltpu.VMEM
    pl.run_scoped(start_up, vmem((3 * NP, 256, D), BF16))

    @pl.loop(0, 2)
    def _(rep):
        pl.run_scoped(
            functools.partial(local_layer, rep),
            [vmem((2, R, 128), F32)] * NP,
            [vmem((2, HALO + R + PAD, 128), F32)] * NP,
            [vmem((1, WIN, R + PAD, 128), F32)] * NP,
            vmem((1, NT, R + PAD, 128), F32),
            vmem((NR, 7, 64 + PAD, D // 2), I32),
            [vmem((1, 256 + G, D), BF16)] * 2 + [vmem((1, D + G, 256), BF16)])
        pl.run_scoped(
            functools.partial(full_layer, rep),
            vmem((49, 32, D // 4), I32),
            [[vmem((2, 64, 256), F32)] * 2] * 2,
            [vmem((1, R + PAD, D), F32)] * 2,
            vmem((NT, NR, 64, R), I32),
            vmem((NT, S // 2, 128), I32),
            vmem((NT, NR, 64, R), I32),
            vmem((NT, NR, 128, R), F32),
            vmem((QB, 64, R), I32),
            vmem((S // 2, 128), I32),
            vmem((NR, 64, R), I32),
            vmem((4 * QB, S, R), F32),
            vmem((4 * QB, 8, R), F32))
        pl.when(rep == 0)(lambda: _run(sum(norm_tasks(0, rep >> 20), []) + left_tasks(lhs1_ref)))

    for i in range(NR):
        out_copy(i).wait()


@jax.jit
def pallas_interleave_layers__sliding_local_dilated__softmax_full_mha__prompt_kernel(
    A_x: jax.Array,
    A_wqkv: jax.Array,
    A_wo: jax.Array,
    B_x: jax.Array,
    B_wqkv: jax.Array,
    B_wo: jax.Array,
):
    del B_x
    vmem = pltpu.VMEM
    dma = pltpu.SemaphoreType.DMA
    out = pl.pallas_call(
        _kernel,
        out_shape=jax.ShapeDtypeStruct((S, D), BF16),
        in_specs=[pl.BlockSpec(memory_space=pl.ANY)] * 5,
        out_specs=pl.BlockSpec(memory_space=pl.ANY),
        scratch_shapes=[
            vmem((S, D), BF16),
            vmem((1, R + G, D), BF16),
            vmem((1, NT, R + PAD, 128), F32),
            vmem((1, R, 128), F32),
            vmem((1, R, 128), F32),
            vmem((1, 4, 32 + G, D), BF16),
            vmem((7, 64, D // 2), I32),
            vmem((1, NT, HALO + R + PAD, 128), F32),
            vmem((1, WIN, R, 128), F32),
            vmem((3 * NP, NP, 7, 64, 128), I32),
            vmem((NP, NP, 7, 64, 128), I32),
            vmem((3, NR, 49, 16, 256), I32),
            vmem((NR, 49, 16, 256), I32),
            vmem((NP + 1, D + G, 256), BF16),
            vmem((4, 256, 3 * D), BF16),
            vmem((4, 256, D), BF16),
            dma((NR,)), dma((3 * NP,)), dma((NP,)), dma(()), dma(()),
        ],
        compiler_params=pltpu.CompilerParams(vmem_limit_bytes=120 * 2 ** 20),
        name="interleave_layers",
    )(A_x.reshape(S, D), A_wqkv, A_wo, B_wqkv.reshape(4, 256, 3 * D), B_wo.reshape(4, 256, D))
    return out.reshape(A_x.shape)
```

```python
import functools
import math

import jax
import jax.numpy as jnp
from jax import lax
import jax.experimental.pallas as pl
import jax.experimental.pallas.tpu as pltpu

F32 = jnp.float32
BF16 = jnp.bfloat16
I32 = jnp.int32

S = 2048
D = 1024
H = 32
DH = D // H
NT = D // 128
NP = NT // 2
WIN, DIL = 8, 2
HALO = 16
EPS = 1e-5
NEG = -1e9
LOG2E = math.log2(math.e)
QSCALE = DH ** -0.5 * LOG2E

R = 256
NR = S // R
CK = 128
QB = 2
G = 16
AHEAD = 3
PAD = 8

LHS_TERMS = (((1, 1, 0), (1, 1, 1)), ((1, 1, 1),), ((1, 0, 0), (1, 1, 1)), ((1, 1, 0), (-1, 0, 0)),
             ((1, 0, 1), (-1, 1, 1)), ((1, 0, 0), (1, 0, 1)), ((1, 0, 0),))
RHS_TERMS = (((1, 0, 0),), ((1, 1, 0), (-1, 0, 0)), ((1, 0, 0), (1, 1, 1)), ((1, 0, 0), (1, 0, 1)),
             ((1, 1, 0), (1, 1, 1)), ((1, 1, 1),), ((1, 0, 1), (-1, 1, 1)))


def _term(spec, block):
    out = block(*spec[0][1:])
    for sign, r, c in spec[1:]:
        out = out + block(r, c) if sign > 0 else out - block(r, c)
    return out


def _nested_terms(specs, outer, block):
    inner = {(r, c): _term(specs[outer], lambda a, b: block(2 * a + r, 2 * b + c))
             for r in (0, 1) for c in (0, 1)}
    return [_term(spec, lambda r, c: inner[r, c]) for spec in specs]


def _combine(s, m, x, y, emit):
    if s == 0:
        return m, None
    if s == 1:
        emit(1, 0, x() + m)
        return None, m
    if s == 2:
        return m - x(), y() + m
    if s == 3:
        return x() + m, None
    if s == 4:
        return None, y() + m
    if s == 5:
        emit(0, 0, y() - m)
        return None, m
    emit(1, 1, x() + m)
    emit(0, 1, y() + m)
    return None, None


def _strassen(product, emit):
    x = y = None
    for s in range(7):
        new_x, new_y = _combine(s, product(s), lambda: x, lambda: y, emit)
        x = x if new_x is None else new_x
        y = y if new_y is None else new_y


def _dot(a, b):
    return jnp.dot(a, b, preferred_element_type=F32)


def _pack(x):
    return pltpu.bitcast(x.astype(BF16), I32)


def _unpack(x):
    return pltpu.bitcast(x, BF16)


def _tile(t, n=128):
    return slice(t * n, (t + 1) * n)


def _tasks(reads, fn, *args):
    return [(reads, functools.partial(fn, *args[:-1], a)) for a in args[-1]]


def _run(tasks):
    for _, task in tasks:
        task()


class _Projector:
    def __init__(self, z, early=8, slack=24):
        self.z, self.early, self.slack = z, early, slack
        self.never = jnp.full((8, 128), z) > 0
        self.results, self.deadlines, self.plan = [], {}, {}

    def spread(self, tasks, first, last):
        for n, task in enumerate(tasks):
            at = int(8 * (first + n * (last - first) / len(tasks)))
            self.plan.setdefault(at, []).append(task)

    def due(self, ref, at):
        if ref is not None:
            value = ref[(0,) * (len(ref.shape) - 2)
                        + (slice(32 // ref.dtype.itemsize), slice(128))]
            self.deadlines.setdefault(at, []).append(pltpu.bitcast(value, I32))

    def product(self, lhs, rhs):
        now = range(len(self.results), len(self.results) + lhs.shape[0] // 8)
        head = [lhs[_tile(n, 8), :128] for n in range(len(now))]
        for n, at in enumerate(now):
            if at in self.deadlines:
                value = functools.reduce(jnp.bitwise_or, self.deadlines.pop(at))
                head[n] = jnp.where(self.never, value, head[n])
        lhs = jnp.concatenate([jnp.concatenate(head, axis=0), lhs[:, 128:]], axis=1)
        out = _dot(_unpack(lhs), _unpack(rhs))
        self.results += [(out, n * G) for n in range(len(now))]
        for at in now:
            for reads, task in self.plan.pop(at, ()):
                for ref in reads if at >= self.early else ():
                    earlier, r = self.results[at - self.early]
                    spare = slice(ref.shape[-2] - PAD, None)
                    ref[(self.z,) + (0,) * (len(ref.shape) - 3) + (spare, slice(128))] = (
                        earlier[r:r + PAD, :128].astype(ref.dtype))
                self.due(task(), at + self.slack)
        return out

    def paced(self, emit):
        return lambda *args: self.due(emit(*args), len(self.results) + 16)

    def one_level(self, lhs_ref, w_ref, emit):
        _strassen(lambda s: self.product(lhs_ref[s], w_ref[:, s].reshape(D // 4, 128)),
                  self.paced(emit))

    def two_levels(self, lhs_ref, w_ref, sum_refs, emit):
        emit = self.paced(emit)
        for s in range(7):
            def fold(r, c, m):
                new = _combine(s, m, lambda: sum_refs[r][c][0], lambda: sum_refs[r][c][1],
                               lambda a, b, val: emit(2 * a + r, 2 * b + c, val))
                for n, val in enumerate(new):
                    if val is not None:
                        sum_refs[r][c][self.z + n] = val
                return sum_refs[r][c]

            _strassen(lambda t: self.product(lhs_ref[7 * s + t],
                                             w_ref[:, 7 * s + t].reshape(D // 8, 256)),
                      self.paced(fold))


def _permute_heads(tiles):
    dtype = tiles[0].dtype
    tiles = [pltpu.bitcast(t, I32) for t in tiles]
    lane = lax.broadcasted_iota(I32, tiles[0].shape, 1)
    for b in (1, 2, 4):
        swap = ((lane >> 2) & b) != 0
        tiles = [jnp.where(swap, tiles[i ^ b], tiles[i]) for i in range(NT)]
    e, j, hl = lane >> 5, (lane >> 2) & 7, lane & 3
    tiles = [jnp.take_along_axis(tiles[i], hl * 32 + (j ^ i) * 4 + e, axis=1) for i in range(NT)]
    return [pltpu.bitcast(t, dtype) for t in tiles]


def _rows(i, n=R, off=0, size=None, align=None):
    return pl.ds(pl.multiple_of(i * n + off, align or size or n), size or n)


def _kernel(x_hbm, awqkv_hbm, awo_hbm, bwqkv_hbm, bwo_hbm, out_hbm,
            x_ref, chunk_ref, left_ref, mean_ref, rstd_ref, piece_ref, lhs1_ref, v_ref, prob_ref,
            wa_ref, wao_ref, wb_ref, wbo_ref, awo_ref, bwqkv_ref, bwo_ref,
            x_sems, aw_sems, awo_sems, bw_sem, bwo_sem):
    def x_copy(i):
        return pltpu.make_async_copy(x_hbm.at[_rows(i)], x_ref.at[_rows(i)], x_sems.at[i])

    def out_copy(i):
        return pltpu.make_async_copy(x_ref.at[_rows(i)], out_hbm.at[_rows(i)], x_sems.at[i])

    def awo_copy(i):
        return pltpu.make_async_copy(
            awo_hbm.at[:, _rows(i, 256)], awo_ref.at[i, :D], awo_sems.at[i])

    bw_copy = pltpu.make_async_copy(bwqkv_hbm, bwqkv_ref, bw_sem)
    bwo_copy = pltpu.make_async_copy(bwo_hbm, bwo_ref, bwo_sem)

    def put_weights(w_ref, r, block):
        for s, spec in enumerate(RHS_TERMS):
            term = _pack(_term(spec, lambda a, b: block(a, b).astype(F32)))
            w_ref[s, r // 2:r // 2 + term.shape[0], :] = term

    def nested_weight_tasks(w_ref, dst, z, src):
        def fetch(a):
            piece_ref[z, a, :32, :] = src(a)
            return piece_ref

        def task(s, r, c):
            terms = _nested_terms(RHS_TERMS, s, lambda a, b: piece_ref[
                0, a, r:r + G, _tile(2 * b + c)].astype(F32))
            for t, term in enumerate(terms):
                dst[7 * s + t, r // 2:(r + G) // 2, _tile(c)] = _pack(term)
            return w_ref
        return _tasks([], fetch, range(4)) + [
            t for s in range(7) for r in (0, G) for t in _tasks([piece_ref], task, s, r, (0, 1))]

    def norm_tasks(i, z):
        def mean_task(r):
            x = x_ref[_rows(i, R, r, G), :]
            chunk_ref[z, r:r + G, :] = x
            mean_ref[z, r:r + G, :] = jnp.broadcast_to(
                jnp.mean(x.astype(F32), axis=-1, keepdims=True), (G, 128))
            return mean_ref

        def rstd_task(r):
            x = chunk_ref[0, r:r + G, :].astype(F32)
            mean = mean_ref[0, r:r + G, :]
            sq = functools.reduce(
                jnp.add, [jnp.square(x[:, _tile(t)] - mean) for t in range(NT)])
            var = jnp.sum(sq, axis=-1, keepdims=True) * (1.0 / D)
            rstd_ref[z, r:r + G, :] = lax.rsqrt(jnp.broadcast_to(var, (G, 128)) + EPS)
            return rstd_ref

        def scale_task(r):
            x = chunk_ref[0, r:r + G, :].astype(F32)
            mean, rstd = mean_ref[0, r:r + G, :], rstd_ref[0, r:r + G, :]
            for t in range(NT):
                left_ref[z, t, r:r + G, :] = (x[:, _tile(t)] - mean) * rstd
            return left_ref

        return [_tasks([chunk_ref], task, range(0, R, G))
                for task in (mean_task, rstd_task, scale_task)]

    def left_tasks(lhs_ref, src=left_ref, done=None):
        def task(s, r):
            lhs_ref[s, r // 2:(r + G) // 2, :] = _pack(jnp.concatenate([
                _term(LHS_TERMS[s], lambda a, b: src[
                    0, 2 * p + b, a * 128 + r:a * 128 + r + G, :]) for p in range(NP)], axis=1))
            return done
        return [t for s in range(7) for t in _tasks([src], task, s, range(0, 128, G))]

    def nested_left_tasks(lhs_ref):
        def task(s, r, c):
            terms = _nested_terms(LHS_TERMS, s, lambda a, b: left_ref[
                0, 2 * b + c, a * 64 + r:a * 64 + r + G, :])
            for t, term in enumerate(terms):
                lhs_ref[7 * s + t, r // 2:(r + G) // 2, _tile(c)] = _pack(term)
        return [t for s in range(7) for r in range(0, 64, G)
                for t in _tasks([left_ref], task, s, r, (0, 1))]

    def add_to_stream(i, r, cols, val):
        blk = (_rows(i, R, r, val.shape[0]), cols)
        x_ref[blk] = (x_ref[blk].astype(F32) + val).astype(BF16)

    def start_up(awqkv_ref):
        def aw_copy(i):
            return pltpu.make_async_copy(awqkv_hbm.at[_rows(i % NP, 256), _rows(i // NP, D)],
                                         awqkv_ref.at[i], aw_sems.at[i])

        x_copy(0).start()
        aw_copy(0).start()
        awo_ref[NP] = jnp.zeros(awo_ref.shape[1:], BF16)
        v_ref[...] = jnp.zeros(v_ref.shape, F32)
        prob_ref[...] = jnp.zeros(prob_ref.shape, F32)
        x_copy(0).wait()
        for i in range(1, AHEAD):
            aw_copy(i).start()
        _run(sum(norm_tasks(0, 0), []) + left_tasks(lhs1_ref))

        @pl.loop(0, 3 * NP)
        def _(i):
            aw_copy(i).wait()
            pl.when(i + AHEAD < 3 * NP)(lambda: aw_copy(i + AHEAD).start())
            pl.when(i + AHEAD == 3 * NP)(lambda: x_copy(1).start())
            t = _permute_heads([awqkv_ref[i, :, _tile(c)] for c in range(NT)])
            for p in range(NP):
                put_weights(wa_ref.at[i // NP * NP + p, i % NP], 0,
                            lambda a, b: t[2 * p + b][_tile(a)])

        for i in range(2, NR):
            x_copy(i).start()

    def local_layer(rep, q_refs, k_refs, sum_refs, mix_ref, o_ref, flip_refs):
        lhs_ref = lhs1_ref

        def mix_tasks(i, z):
            def task(r, p):
                o = {}
                for w in range(WIN):
                    a = prob_ref[0, w, r:r + 8, :]
                    for t in (2 * p, 2 * p + 1):
                        b = a * v_ref[0, t, HALO + r - DIL * w:HALO + r - DIL * w + 8, :]
                        o[t] = o[t] + b if w else b
                for t, val in o.items():
                    mix_ref[z, t, r:r + 8, :] = val
                return mix_ref
            return ([t for r in range(0, R, 8) for t in _tasks([v_ref], task, r, range(NP))],
                    left_tasks(o_ref.at[i], mix_ref, o_ref))

        def qkv_softmax(i):
            @pl.when(rep == 0)
            def _():
                pl.when(i + 1 < NR)(lambda: x_copy(i + 1).wait())
                pl.when(i >= NP)(lambda: awo_copy(i - NP).wait())

                @pl.when(i == 1)
                def _():
                    for n in range(NP):
                        awo_copy(n).start()
                    bw_copy.start()
                    bwo_copy.start()

            z = i >> 20

            def flip_task(r):
                flip_refs[0][z, :256, _tile(r)] = awo_ref[jnp.where(i < NP, NP, i - NP), _tile(r), :].T
                return flip_refs[0]

            def permute_task(r):
                t = _permute_heads([flip_refs[0][0, r:r + 2 * G, _tile(c)] for c in range(NT)])
                flip_refs[1][z, r:r + 2 * G, :] = jnp.concatenate(t, axis=1)
                return flip_refs[1]

            def unflip_task(r):
                flip_refs[2][z, _tile(r), :] = flip_refs[1][0, :256, _tile(r)].T
                return flip_refs[2]

            def awo_task(p, r):
                put_weights(wao_ref.at[i % NP, p], r, lambda a, b: flip_refs[2][
                    0, (2 * p + a) * 128 + r:(2 * p + a) * 128 + r + G, _tile(b)])
                return wao_ref

            def logits_task(p, r):
                q = [q_refs[p][c, r:r + 8, :] for c in (0, 1)]
                for w in range(WIN):
                    win = slice(HALO + r - DIL * w, HALO + r - DIL * w + 8)
                    a = q[0] * k_refs[p][0, win, :] + q[1] * k_refs[p][1, win, :]
                    if p > 0:
                        a = a + sum_refs[p - 1][0, w, r:r + 8, :]
                    if p == NP - 1:
                        a = a + pltpu.roll(a, 64, 1)
                    sum_refs[p][z, w, r:r + 8, :] = a
                return sum_refs[p]

            def fold_task(r):
                for w in range(WIN):
                    a = sum_refs[NP - 1][0, w, r:r + 8, :]
                    a = (a + pltpu.roll(a, 32, 1)) * QSCALE
                    if r < DIL * w:
                        pos = i * R + r + lax.broadcasted_iota(I32, (8, 128), 0)
                        a = jnp.where(pos >= DIL * w, a, NEG * LOG2E)
                    sum_refs[r // 128][z, w, r:r + 8, :] = a
                return sum_refs[r // 128]

            def softmax_task(r):
                logits = [sum_refs[r // 128][0, w, r:r + 8, :] for w in range(WIN)]
                mx = functools.reduce(jnp.maximum, logits)
                e = [jnp.exp2(a - mx) for a in logits]
                inv = 1.0 / functools.reduce(jnp.add, e)
                for w in range(WIN):
                    prob_ref[z, w, r:r + 8, :] = e[w] * inv
                return prob_ref

            proj = _Projector(z, 4, 28)
            norm = norm_tasks(jnp.minimum(i + 1, NR - 1), z)
            proj.spread(norm[0], 0, 5)
            proj.spread(norm[1], 6, 15)
            proj.spread(norm[2], 23, 29)
            proj.spread(_tasks([awo_ref], flip_task, range(NT)), 2, 10)
            proj.spread(_tasks([flip_refs[0]], permute_task, range(0, 256, 2 * G)), 13, 29)
            proj.spread(_tasks([flip_refs[1]], unflip_task, range(NT)), 31, 39)
            proj.spread([t for p in range(NP) for t in
                         _tasks([flip_refs[2]], awo_task, p, range(0, 128, G))], 41, 57)
            mix = mix_tasks(jnp.maximum(i - 1, 0), z)
            proj.spread(mix[0][:32], 1, 15)
            proj.spread(mix[0][32:48], 15, 24)
            proj.spread(mix[0][48:64], 24, 29)
            proj.spread(mix[0][64:80], 29, 38)
            proj.spread(mix[0][80:100], 38, 43)
            proj.spread(mix[0][100:112], 43, 52)
            proj.spread(mix[0][112:], 52, 56)
            proj.spread(mix[1], 58, 78)
            for p in range(NP):
                proj.spread(_tasks([k_refs[p], *sum_refs[max(p - 1, 0):p]], logits_task, p,
                                   range(0, R, 8)), 14 * p + 15, 14 * p + 24)
            proj.spread(_tasks([sum_refs[NP - 1]], fold_task, range(0, R, 8)), 66, 73)
            proj.spread([t for h in (0, 1) for t in _tasks(
                [sum_refs[h]], softmax_task, range(h * 128, h * 128 + 128, 8))], 70, 79)
            proj.spread(left_tasks(lhs_ref), 77, 84)

            for p in range(NP):
                def emit_k(h, c, val):
                    k_refs[p][z + c, HALO + h * 128:HALO + (h + 1) * 128, :] = val
                    return k_refs[p]

                def emit_q(h, c, val):
                    q_refs[p][z + c, _tile(h), :] = val
                    return q_refs[p]

                k_refs[p][:, :HALO, :] = k_refs[p][:, R:R + HALO, :]
                proj.one_level(lhs_ref, wa_ref.at[NP + p], emit_k)
                proj.one_level(lhs_ref, wa_ref.at[p], emit_q)
            v_ref[0, :, :HALO, :] = v_ref[0, :, R:R + HALO, :]
            for p in range(NP):
                def emit_v(h, c, val):
                    if h == 0:
                        v_ref[z, 2 * p + c, :HALO, :] = jnp.where(
                            i == 0, jnp.broadcast_to(val[:1], (HALO, 128)),
                            v_ref[0, 2 * p + c, :HALO, :])
                    v_ref[z, 2 * p + c, HALO + h * 128:HALO + (h + 1) * 128, :] = val
                    return v_ref

                proj.one_level(lhs_ref, wa_ref.at[2 * NP + p], emit_v)

        def output(i):
            def fetch(s, r):
                lhs_ref[s, r:r + 8, :] = o_ref[jnp.minimum(i + 1, NR - 1), s, r:r + 8, :]

            proj = _Projector(i >> 20)
            proj.spread([t for m in range(3) for t in nested_weight_tasks(
                wb_ref, wb_ref.at[m, i], proj.z,
                lambda a, m=m: bwqkv_ref[a, _rows(i, 32), _tile(m, D)])], 0, 28)
            proj.spread([t for s in range(7)
                         for t in _tasks([o_ref], fetch, s, range(0, 64, 8))], 21, 28)
            for p in range(NP):
                proj.one_level(lhs_ref, wao_ref.at[p], lambda h, c, val: add_to_stream(
                    i, h * 128, _tile(2 * p + c), val))

        for p in range(NP):
            k_refs[p][:, R:R + HALO, :] = jnp.zeros((2, HALO, 128), F32)
        pl.loop(0, NR)(qkv_softmax)
        pl.when(rep == 0)(lambda: bw_copy.wait())
        _run(sum(mix_tasks(NR - 1, rep >> 20), []))
        lhs_ref[...] = o_ref[0, :, :64, :]
        pl.loop(0, NR)(output)

    def full_layer(rep, lhs_ref, sum_refs, stage_refs, qt_ref, k_ref, vt_ref, ot_ref,
                   q_now, k_now, v_now, s_ref, m_ref):
        def qkv(i):
            z = i >> 20

            def flip_tasks(n, dst, scale):
                def task(t, h):
                    dst[t, i, :, _tile(h)] = _pack(scale(stage_refs[n][0, _tile(h), _tile(t)]).T)
                    return dst
                return [f for t in range(NT) for f in _tasks([stage_refs[n]], task, t, (0, 1))]

            def stage(n, r, c, val):
                stage_refs[n][z, _tile(r, 64), _tile(c, 256)] = val
                return stage_refs[n]

            def emit_k(r, c, val):
                val = _pack(val)
                for t in (0, 1):
                    k_ref[2 * c + t, _rows(i, R // 2, r * 32, 32), :] = val[:, _tile(t)]
                return k_ref

            proj = _Projector(z)
            norm = norm_tasks(jnp.minimum(i + 1, NR - 1), z)
            proj.spread(norm[0], 0, 6)
            proj.spread(norm[1], 7, 17)
            proj.spread(norm[2], 18, 25)
            proj.spread(flip_tasks(0, qt_ref, lambda q: q * QSCALE), 26, 44)
            proj.spread(nested_weight_tasks(
                wbo_ref, wbo_ref.at[i], z, lambda a: bwo_ref[a, _rows(i, 32), :]), 20, 50)
            proj.spread(flip_tasks(1, vt_ref, lambda v: v), 50.5, 68)
            tasks = nested_left_tasks(lhs_ref)
            proj.spread(tasks[:48], 52.5, 73.5)
            proj.two_levels(lhs_ref, wb_ref.at[0], sum_refs, functools.partial(stage, 0))
            proj.two_levels(lhs_ref, wb_ref.at[2], sum_refs, functools.partial(stage, 1))
            proj.two_levels(lhs_ref, wb_ref.at[1], sum_refs, emit_k)
            _run(tasks[48:])

        def attend(u, j, b, nxt, cur, then=None):
            hs = _tile(j, DH // 2)
            if cur is not None:
                m = jnp.broadcast_to(jnp.max(m_ref[u], axis=0, keepdims=True), (G, R))
            l = acc = m_acc = None
            for c in range(S // CK):
                def scores():
                    parts = [q_now[b, hs, :]]
                    if j > 0:
                        parts.insert(0, jnp.zeros((DH // 2 * j, R), I32))
                    if j < 3:
                        parts.append(jnp.zeros((DH // 2 * (3 - j), R), I32))
                    return _dot(_unpack(k_now[_tile(c, CK // 2), :]),
                                _unpack(jnp.concatenate(parts, axis=0)))

                late = then is not None and c == S // CK - 1
                if nxt is not None and not late:
                    s = scores()
                if cur is not None:
                    slabs = {}
                    for r in reversed(range(CK // G)):
                        p = jnp.exp2(s_ref[u, _tile(c * CK // G + r, G), :] - m)
                        ls = p[0:8] + p[8:16]
                        l = ls if l is None else l + ls
                        slabs[r] = p
                    p = jnp.concatenate([slabs[r] for r in range(CK // G)], axis=0).astype(BF16)
                    off = c * CK % R
                    a = _dot(_unpack(v_now[c * CK // R, hs, off:off + CK]), p)
                    acc = a if acc is None else acc + a
                if nxt is not None:
                    if late:
                        s = scores()
                    s_ref[u, _tile(c, CK), :] = s
                    mx = jnp.max(s.reshape(CK // 8, 8, R), axis=0)
                    m_acc = mx if m_acc is None else jnp.maximum(m_acc, mx)
                if then is not None:
                    k_now[_tile(c, CK // 2), :] = k_ref[then, _tile(c, CK // 2), :]
                    v_now[c * CK // R, :, off:off + CK] = vt_ref[nxt, c * CK // R, :, off:off + CK]
            if nxt is not None:
                m_ref[u] = m_acc
            if cur is not None:
                inv = 1.0 / jnp.sum(l, axis=0, keepdims=True)
                ot_ref[cur[0], cur[1], _tile(j, DH), :] = acc * inv

        def unflip_tasks(i, z):
            def task(t, h):
                left_ref[z, t, _tile(h), :] = ot_ref[t, i, :, _tile(h)].T
                return left_ref
            return [f for t in range(NT) for f in _tasks([], task, t, (0, 1))]

        def output(i):
            proj = _Projector(i >> 20)
            proj.spread(unflip_tasks(jnp.minimum(i + 1, NR - 1), proj.z), 0, 5)
            tasks = nested_left_tasks(lhs_ref)
            proj.spread(tasks[:48], 7, 24.5)
            proj.two_levels(lhs_ref, wbo_ref, sum_refs, lambda r, c, val: add_to_stream(
                i, r * 64, _tile(c, 256), val))
            _run(tasks[48:])
            pl.when(rep == 1)(lambda: out_copy(i).start())

        pl.when(rep == 0)(lambda: bwo_copy.wait())
        _run(sum(norm_tasks(0, rep >> 20), []) + nested_left_tasks(lhs_ref))
        pl.loop(0, NR)(qkv)
        nqb = NR // QB

        q_now[...] = qt_ref[0, :QB]
        k_now[...] = k_ref[0]
        v_now[...] = vt_ref[0]

        @pl.loop(0, QB)
        def _(b):
            for j in range(4):
                attend(b * 4 + j, j, b, 0, None)
            q_now[b] = qt_ref[0, QB + b]

        @pl.loop(0, NT * nqb - 1)
        def _(i):
            later = jnp.minimum(i + 2, NT * nqb - 1)
            for b in range(QB):
                for j in range(4):
                    attend(b * 4 + j, j, b, (i + 1) // nqb, (i // nqb, i % nqb * QB + b),
                           later // nqb if b == QB - 1 and j == 3 else None)
                q_now[b] = qt_ref[later // nqb, later % nqb * QB + b]

        @pl.loop(0, QB)
        def _(b):
            for j in range(4):
                attend(b * 4 + j, j, b, None, (NT - 1, NR - QB + b))

        _run(unflip_tasks(0, rep >> 20) + nested_left_tasks(lhs_ref))
        pl.loop(0, NR)(output)

    vmem = pltpu.VMEM
    pl.run_scoped(start_up, vmem((3 * NP, 256, D), BF16))

    @pl.loop(0, 2)
    def _(rep):
        pl.run_scoped(
            functools.partial(local_layer, rep),
            [vmem((2, R, 128), F32)] * NP,
            [vmem((2, HALO + R + PAD, 128), F32)] * NP,
            [vmem((1, WIN, R + PAD, 128), F32)] * NP,
            vmem((1, NT, R + PAD, 128), F32),
            vmem((NR, 7, 64 + PAD, D // 2), I32),
            [vmem((1, 256 + G, D), BF16)] * 2 + [vmem((1, D + G, 256), BF16)])
        pl.run_scoped(
            functools.partial(full_layer, rep),
            vmem((49, 32, D // 4), I32),
            [[vmem((2, 64, 256), F32)] * 2] * 2,
            [vmem((1, R + PAD, D), F32)] * 2,
            vmem((NT, NR, 64, R), I32),
            vmem((NT, S // 2, 128), I32),
            vmem((NT, NR, 64, R), I32),
            vmem((NT, NR, 128, R), F32),
            vmem((QB, 64, R), I32),
            vmem((S // 2, 128), I32),
            vmem((NR, 64, R), I32),
            vmem((4 * QB, S, R), F32),
            vmem((4 * QB, 8, R), F32))
        pl.when(rep == 0)(lambda: _run(sum(norm_tasks(0, rep >> 20), []) + left_tasks(lhs1_ref)))

    for i in range(NR):
        out_copy(i).wait()


@jax.jit
def pallas_interleave_layers__sliding_local_dilated__softmax_full_mha__prompt_kernel(
    A_x: jax.Array,
    A_wqkv: jax.Array,
    A_wo: jax.Array,
    B_x: jax.Array,
    B_wqkv: jax.Array,
    B_wo: jax.Array,
):
    del B_x
    vmem = pltpu.VMEM
    dma = pltpu.SemaphoreType.DMA
    out = pl.pallas_call(
        _kernel,
        out_shape=jax.ShapeDtypeStruct((S, D), BF16),
        in_specs=[pl.BlockSpec(memory_space=pl.ANY)] * 5,
        out_specs=pl.BlockSpec(memory_space=pl.ANY),
        scratch_shapes=[
            vmem((S, D), BF16),
            vmem((1, R + G, D), BF16),
            vmem((1, NT, R + PAD, 128), F32),
            vmem((1, R, 128), F32),
            vmem((1, R, 128), F32),
            vmem((1, 4, 32 + G, D), BF16),
            vmem((7, 64, D // 2), I32),
            vmem((1, NT, HALO + R + PAD, 128), F32),
            vmem((1, WIN, R, 128), F32),
            vmem((3 * NP, NP, 7, 64, 128), I32),
            vmem((NP, NP, 7, 64, 128), I32),
            vmem((3, NR, 49, 16, 256), I32),
            vmem((NR, 49, 16, 256), I32),
            vmem((NP + 1, D + G, 256), BF16),
            vmem((4, 256, 3 * D), BF16),
            vmem((4, 256, D), BF16),
            dma((NR,)), dma((3 * NP,)), dma((NP,)), dma(()), dma(()),
        ],
        compiler_params=pltpu.CompilerParams(vmem_limit_bytes=120 * 2 ** 20),
        name="interleave_layers",
    )(A_x.reshape(S, D), A_wqkv, A_wo, B_wqkv.reshape(4, 256, 3 * D), B_wo.reshape(4, 256, D))
    return out.reshape(A_x.shape)
```

```python
import functools
import math

import jax
import jax.numpy as jnp
from jax import lax
import jax.experimental.pallas as pl
import jax.experimental.pallas.tpu as pltpu

F32 = jnp.float32
BF16 = jnp.bfloat16
I32 = jnp.int32

S = 2048
D = 1024
H = 32
DH = D // H
NT = D // 128
NP = NT // 2
WIN, DIL = 8, 2
HALO = 16
EPS = 1e-5
NEG = -1e9
LOG2E = math.log2(math.e)
QSCALE = DH ** -0.5 * LOG2E

R = 256
NR = S // R
CK = 128
QB = 4
G = 16
AHEAD = 3
PAD = 8

LHS_TERMS = (((1, 1, 0), (1, 1, 1)), ((1, 1, 1),), ((1, 0, 0), (1, 1, 1)), ((1, 1, 0), (-1, 0, 0)),
             ((1, 0, 1), (-1, 1, 1)), ((1, 0, 0), (1, 0, 1)), ((1, 0, 0),))
RHS_TERMS = (((1, 0, 0),), ((1, 1, 0), (-1, 0, 0)), ((1, 0, 0), (1, 1, 1)), ((1, 0, 0), (1, 0, 1)),
             ((1, 1, 0), (1, 1, 1)), ((1, 1, 1),), ((1, 0, 1), (-1, 1, 1)))


def _term(spec, block):
    out = block(*spec[0][1:])
    for sign, r, c in spec[1:]:
        out = out + block(r, c) if sign > 0 else out - block(r, c)
    return out


def _nested_terms(specs, outer, block):
    inner = {(r, c): _term(specs[outer], lambda a, b: block(2 * a + r, 2 * b + c))
             for r in (0, 1) for c in (0, 1)}
    return [_term(spec, lambda r, c: inner[r, c]) for spec in specs]


def _combine(s, m, x, y, emit):
    if s == 0:
        return m, None
    if s == 1:
        emit(1, 0, x() + m)
        return None, m
    if s == 2:
        return m - x(), y() + m
    if s == 3:
        return x() + m, None
    if s == 4:
        return None, y() + m
    if s == 5:
        emit(0, 0, y() - m)
        return None, m
    emit(1, 1, x() + m)
    emit(0, 1, y() + m)
    return None, None


def _strassen(product, emit):
    x = y = None
    for s in range(7):
        new_x, new_y = _combine(s, product(s), lambda: x, lambda: y, emit)
        x = x if new_x is None else new_x
        y = y if new_y is None else new_y


def _dot(a, b):
    return jnp.dot(a, b, preferred_element_type=F32)


def _pack(x):
    return pltpu.bitcast(x.astype(BF16), I32)


def _unpack(x):
    return pltpu.bitcast(x, BF16)


def _tile(t, n=128):
    return slice(t * n, (t + 1) * n)


def _tasks(reads, fn, *args):
    return [(reads, functools.partial(fn, *args[:-1], a)) for a in args[-1]]


def _run(tasks):
    for _, task in tasks:
        task()


class _Projector:
    def __init__(self, z, early=8, slack=24):
        self.z, self.early, self.slack = z, early, slack
        self.never = jnp.full((8, 128), z) > 0
        self.results, self.deadlines, self.plan = [], {}, {}

    def spread(self, tasks, first, last):
        for n, task in enumerate(tasks):
            at = int(8 * (first + n * (last - first) / len(tasks)))
            self.plan.setdefault(at, []).append(task)

    def due(self, ref, at):
        if ref is not None:
            value = ref[(0,) * (len(ref.shape) - 2)
                        + (slice(32 // ref.dtype.itemsize), slice(128))]
            self.deadlines.setdefault(at, []).append(pltpu.bitcast(value, I32))

    def product(self, lhs, rhs):
        now = range(len(self.results), len(self.results) + lhs.shape[0] // 8)
        head = [lhs[_tile(n, 8), :128] for n in range(len(now))]
        for n, at in enumerate(now):
            if at in self.deadlines:
                value = functools.reduce(jnp.bitwise_or, self.deadlines.pop(at))
                head[n] = jnp.where(self.never, value, head[n])
        lhs = jnp.concatenate([jnp.concatenate(head, axis=0), lhs[:, 128:]], axis=1)
        out = _dot(_unpack(lhs), _unpack(rhs))
        self.results += [(out, n * G) for n in range(len(now))]
        for at in now:
            for reads, task in self.plan.pop(at, ()):
                for ref in reads if at >= self.early else ():
                    earlier, r = self.results[at - self.early]
                    spare = slice(ref.shape[-2] - PAD, None)
                    ref[(self.z,) + (0,) * (len(ref.shape) - 3) + (spare, slice(128))] = (
                        earlier[r:r + PAD, :128].astype(ref.dtype))
                self.due(task(), at + self.slack)
        return out

    def paced(self, emit):
        return lambda *args: self.due(emit(*args), len(self.results) + 16)

    def one_level(self, lhs_ref, w_ref, emit):
        _strassen(lambda s: self.product(lhs_ref[s], w_ref[:, s].reshape(D // 4, 128)),
                  self.paced(emit))

    def two_levels(self, lhs_refs, w_ref, sum_refs, emit):
        emit = self.paced(emit)
        for s in range(7):
            def fold(r, c, m):
                new = _combine(s, m, lambda: sum_refs[r][c][0], lambda: sum_refs[r][c][1],
                               lambda a, b, val: emit(2 * a + r, 2 * b + c, val))
                for n, val in enumerate(new):
                    if val is not None:
                        sum_refs[r][c][self.z + n] = val
                return sum_refs[r][c]

            _strassen(lambda t: self.product(lhs_refs[s][0, t],
                                             w_ref[:, 7 * s + t].reshape(D // 8, 256)),
                      self.paced(fold))


def _permute_heads(tiles):
    dtype = tiles[0].dtype
    tiles = [pltpu.bitcast(t, I32) for t in tiles]
    lane = lax.broadcasted_iota(I32, tiles[0].shape, 1)
    for b in (1, 2, 4):
        swap = ((lane >> 2) & b) != 0
        tiles = [jnp.where(swap, tiles[i ^ b], tiles[i]) for i in range(NT)]
    e, j, hl = lane >> 5, (lane >> 2) & 7, lane & 3
    tiles = [jnp.take_along_axis(tiles[i], hl * 32 + (j ^ i) * 4 + e, axis=1,
                                 mode="promise_in_bounds") for i in range(NT)]
    return [pltpu.bitcast(t, dtype) for t in tiles]


def _rows(i, n=R, off=0, size=None, align=None):
    return pl.ds(pl.multiple_of(i * n + off, align or size or n), size or n)


def _kernel(x_hbm, awqkv_hbm, awo_hbm, bwqkv_hbm, bwo_hbm, out_hbm,
            x_ref, chunk_ref, left_ref, mean_ref, rstd_ref, piece_ref, lhs1_ref, v_ref, prob_ref,
            wa_ref, wao_ref, wb_ref, wbo_ref, awo_ref, bwqkv_ref, bwo_ref,
            x_sems, aw_sems, awo_sems, bw_sem, bwo_sem):
    def x_copy(i):
        return pltpu.make_async_copy(x_hbm.at[_rows(i)], x_ref.at[_rows(i)], x_sems.at[i])

    def out_copy(i):
        return pltpu.make_async_copy(x_ref.at[_rows(i)], out_hbm.at[_rows(i)], x_sems.at[i])

    def awo_copy(i):
        return pltpu.make_async_copy(
            awo_hbm.at[:, _rows(i, 256)], awo_ref.at[i, :D], awo_sems.at[i])

    bw_copy = pltpu.make_async_copy(bwqkv_hbm, bwqkv_ref, bw_sem)
    bwo_copy = pltpu.make_async_copy(bwo_hbm, bwo_ref, bwo_sem)

    def put_weights(w_ref, r, block):
        for s, spec in enumerate(RHS_TERMS):
            term = _pack(_term(spec, lambda a, b: block(a, b).astype(F32)))
            w_ref[s, r // 2:r // 2 + term.shape[0], :] = term

    def nested_weight_tasks(w_ref, dst, z, src):
        def fetch(a):
            piece_ref[z, a, :32, :] = src(a)
            return piece_ref

        def task(s, r, c):
            terms = _nested_terms(RHS_TERMS, s, lambda a, b: piece_ref[
                0, a, r:r + G, _tile(2 * b + c)].astype(F32))
            for t, term in enumerate(terms):
                dst[7 * s + t, r // 2:(r + G) // 2, _tile(c)] = _pack(term)
            return w_ref
        return _tasks([], fetch, range(4)) + [
            t for s in range(7) for r in (0, G) for t in _tasks([piece_ref], task, s, r, (0, 1))]

    def norm_tasks(i, z):
        def mean_task(r):
            x = x_ref[_rows(i, R, r, G), :]
            chunk_ref[z, r:r + G, :] = x
            mean_ref[z, r:r + G, :] = jnp.broadcast_to(
                jnp.mean(x.astype(F32), axis=-1, keepdims=True), (G, 128))
            return mean_ref

        def rstd_task(r):
            x = chunk_ref[0, r:r + G, :].astype(F32)
            mean = mean_ref[0, r:r + G, :]
            sq = functools.reduce(
                jnp.add, [jnp.square(x[:, _tile(t)] - mean) for t in range(NT)])
            var = jnp.sum(sq, axis=-1, keepdims=True) * (1.0 / D)
            rstd_ref[z, r:r + G, :] = lax.rsqrt(jnp.broadcast_to(var, (G, 128)) + EPS)
            return rstd_ref

        def scale_task(r):
            x = chunk_ref[0, r:r + G, :].astype(F32)
            mean, rstd = mean_ref[0, r:r + G, :], rstd_ref[0, r:r + G, :]
            for t in range(NT):
                left_ref[z, t, r:r + G, :] = (x[:, _tile(t)] - mean) * rstd
            return left_ref

        return [_tasks([chunk_ref], task, range(0, R, G))
                for task in (mean_task, rstd_task, scale_task)]

    def left_tasks(lhs_ref, src=left_ref, done=None):
        def task(s, r):
            lhs_ref[s, r // 2:(r + G) // 2, :] = _pack(jnp.concatenate([
                _term(LHS_TERMS[s], lambda a, b: src[
                    0, 2 * p + b, a * 128 + r:a * 128 + r + G, :]) for p in range(NP)], axis=1))
            return done
        return [t for s in range(7) for t in _tasks([src], task, s, range(0, 128, G))]

    def nested_left_tasks(lhs_refs, z, outer):
        def task(s, r, c):
            terms = _nested_terms(LHS_TERMS, s, lambda a, b: left_ref[
                0, 2 * b + c, a * 64 + r:a * 64 + r + G, :])
            for t, term in enumerate(terms):
                lhs_refs[s][z, t, r // 2:(r + G) // 2, _tile(c)] = _pack(term)
            return lhs_refs[s]
        return [t for s in outer for r in range(0, 64, G)
                for t in _tasks([left_ref], task, s, r, (0, 1))]

    def add_to_stream(i, r, cols, val):
        blk = (_rows(i, R, r, val.shape[0]), cols)
        x_ref[blk] = (x_ref[blk].astype(F32) + val).astype(BF16)

    def start_up(awqkv_ref):
        def aw_copy(i):
            return pltpu.make_async_copy(awqkv_hbm.at[_rows(i % NP, 256), _rows(i // NP, D)],
                                         awqkv_ref.at[i], aw_sems.at[i])

        x_copy(0).start()
        aw_copy(0).start()
        awo_ref[NP] = jnp.zeros(awo_ref.shape[1:], BF16)
        v_ref[...] = jnp.zeros(v_ref.shape, F32)
        prob_ref[...] = jnp.zeros(prob_ref.shape, F32)
        x_copy(0).wait()
        for i in range(1, AHEAD):
            aw_copy(i).start()
        _run(sum(norm_tasks(0, 0), []) + left_tasks(lhs1_ref))

        @pl.loop(0, 3 * NP)
        def _(i):
            aw_copy(i).wait()
            pl.when(i + AHEAD < 3 * NP)(lambda: aw_copy(i + AHEAD).start())
            pl.when(i + AHEAD == 3 * NP)(lambda: x_copy(1).start())
            t = _permute_heads([awqkv_ref[i, :, _tile(c)] for c in range(NT)])
            for p in range(NP):
                put_weights(wa_ref.at[i // NP * NP + p, i % NP], 0,
                            lambda a, b: t[2 * p + b][_tile(a)])

        for i in range(2, NR):
            x_copy(i).start()

    def local_layer(rep, q_refs, k_refs, sum_refs, mix_ref, o_ref, flip_refs):
        lhs_ref = lhs1_ref

        def mix_tasks(i, z):
            def task(r, p):
                o = {}
                for w in range(WIN):
                    a = prob_ref[0, w, r:r + 8, :]
                    for t in (2 * p, 2 * p + 1):
                        b = a * v_ref[0, t, HALO + r - DIL * w:HALO + r - DIL * w + 8, :]
                        o[t] = o[t] + b if w else b
                for t, val in o.items():
                    mix_ref[z, t, r:r + 8, :] = val
                return mix_ref
            return ([t for r in range(0, R, 8) for t in _tasks([v_ref], task, r, range(NP))],
                    left_tasks(o_ref.at[i], mix_ref, o_ref))

        def qkv_softmax(i):
            @pl.when(rep == 0)
            def _():
                pl.when(i + 1 < NR)(lambda: x_copy(i + 1).wait())
                pl.when(i >= NP)(lambda: awo_copy(i - NP).wait())

                @pl.when(i == 1)
                def _():
                    for n in range(NP):
                        awo_copy(n).start()
                    bw_copy.start()
                    bwo_copy.start()

            z = i >> 20

            def flip_task(r):
                flip_refs[0][z, :256, _tile(r)] = awo_ref[jnp.where(i < NP, NP, i - NP), _tile(r), :].T
                return flip_refs[0]

            def permute_task(r):
                t = _permute_heads([flip_refs[0][0, r:r + 2 * G, _tile(c)] for c in range(NT)])
                flip_refs[1][z, r:r + 2 * G, :] = jnp.concatenate(t, axis=1)
                return flip_refs[1]

            def unflip_task(r):
                flip_refs[2][z, _tile(r), :] = flip_refs[1][0, :256, _tile(r)].T
                return flip_refs[2]

            def awo_task(p, r):
                put_weights(wao_ref.at[i % NP, p], r, lambda a, b: flip_refs[2][
                    0, (2 * p + a) * 128 + r:(2 * p + a) * 128 + r + G, _tile(b)])
                return wao_ref

            def logits_task(p, r):
                q = [q_refs[p][c, r:r + 8, :] for c in (0, 1)]
                for w in range(WIN):
                    win = slice(HALO + r - DIL * w, HALO + r - DIL * w + 8)
                    a = q[0] * k_refs[p][0, win, :] + q[1] * k_refs[p][1, win, :]
                    if p > 0:
                        a = a + sum_refs[p - 1][0, w, r:r + 8, :]
                    if p == NP - 1:
                        a = a + pltpu.roll(a, 64, 1)
                    sum_refs[p][z, w, r:r + 8, :] = a
                return sum_refs[p]

            def fold_task(r):
                for w in range(WIN):
                    a = sum_refs[NP - 1][0, w, r:r + 8, :]
                    a = (a + pltpu.roll(a, 32, 1)) * QSCALE
                    if r < DIL * w:
                        pos = i * R + r + lax.broadcasted_iota(I32, (8, 128), 0)
                        a = jnp.where(pos >= DIL * w, a, NEG * LOG2E)
                    sum_refs[r // 128][z, w, r:r + 8, :] = a
                return sum_refs[r // 128]

            def softmax_task(r):
                logits = [sum_refs[r // 128][0, w, r:r + 8, :] for w in range(WIN)]
                mx = functools.reduce(jnp.maximum, logits)
                e = [jnp.exp2(a - mx) for a in logits]
                inv = 1.0 / functools.reduce(jnp.add, e)
                for w in range(WIN):
                    prob_ref[z, w, r:r + 8, :] = e[w] * inv
                return prob_ref

            proj = _Projector(z, 4, 28)
            norm = norm_tasks(jnp.minimum(i + 1, NR - 1), z)
            proj.spread(norm[0], 0, 5)
            proj.spread(norm[1], 6, 15)
            proj.spread(norm[2], 23, 29)
            proj.spread(_tasks([awo_ref], flip_task, range(NT)), 2, 10)
            proj.spread(_tasks([flip_refs[0]], permute_task, range(0, 256, 2 * G)), 13, 29)
            proj.spread(_tasks([flip_refs[1]], unflip_task, range(NT)), 31, 39)
            proj.spread([t for p in range(NP) for t in
                         _tasks([flip_refs[2]], awo_task, p, range(0, 128, G))], 41, 57)
            mix = mix_tasks(jnp.maximum(i - 1, 0), z)
            proj.spread(mix[0][:32], 1, 15)
            proj.spread(mix[0][32:48], 15, 24)
            proj.spread(mix[0][48:64], 24, 29)
            proj.spread(mix[0][64:80], 29, 38)
            proj.spread(mix[0][80:100], 38, 43)
            proj.spread(mix[0][100:112], 43, 52)
            proj.spread(mix[0][112:], 52, 56)
            proj.spread(mix[1], 58, 78)
            for p in range(NP):
                proj.spread(_tasks([k_refs[p], *sum_refs[max(p - 1, 0):p]], logits_task, p,
                                   range(0, R, 8)), 14 * p + 15, 14 * p + 24)
            proj.spread(_tasks([sum_refs[NP - 1]], fold_task, range(0, R, 8)), 66, 73)
            proj.spread([t for h in (0, 1) for t in _tasks(
                [sum_refs[h]], softmax_task, range(h * 128, h * 128 + 128, 8))], 70, 79)
            proj.spread(left_tasks(lhs_ref), 77, 84)

            for p in range(NP):
                def emit_k(h, c, val):
                    k_refs[p][z + c, HALO + h * 128:HALO + (h + 1) * 128, :] = val
                    return k_refs[p]

                def emit_q(h, c, val):
                    q_refs[p][z + c, _tile(h), :] = val
                    return q_refs[p]

                k_refs[p][:, :HALO, :] = k_refs[p][:, R:R + HALO, :]
                proj.one_level(lhs_ref, wa_ref.at[NP + p], emit_k)
                proj.one_level(lhs_ref, wa_ref.at[p], emit_q)
            v_ref[0, :, :HALO, :] = v_ref[0, :, R:R + HALO, :]
            for p in range(NP):
                def emit_v(h, c, val):
                    if h == 0:
                        v_ref[z, 2 * p + c, :HALO, :] = jnp.where(
                            i == 0, jnp.broadcast_to(val[:1], (HALO, 128)),
                            v_ref[0, 2 * p + c, :HALO, :])
                    v_ref[z, 2 * p + c, HALO + h * 128:HALO + (h + 1) * 128, :] = val
                    return v_ref

                proj.one_level(lhs_ref, wa_ref.at[2 * NP + p], emit_v)

        def output(i):
            def fetch(s, r):
                lhs_ref[s, r:r + 8, :] = o_ref[jnp.minimum(i + 1, NR - 1), s, r:r + 8, :]

            proj = _Projector(i >> 20)
            proj.spread([t for m in range(3) for t in nested_weight_tasks(
                wb_ref, wb_ref.at[m, i], proj.z,
                lambda a, m=m: bwqkv_ref[a, _rows(i, 32), _tile(m, D)])], 0, 28)
            proj.spread([t for s in range(7)
                         for t in _tasks([o_ref], fetch, s, range(0, 64, 8))], 21, 28)
            for p in range(NP):
                proj.one_level(lhs_ref, wao_ref.at[p], lambda h, c, val: add_to_stream(
                    i, h * 128, _tile(2 * p + c), val))

        for p in range(NP):
            k_refs[p][:, R:R + HALO, :] = jnp.zeros((2, HALO, 128), F32)
        pl.loop(0, NR)(qkv_softmax)
        pl.when(rep == 0)(lambda: bw_copy.wait())
        _run(sum(mix_tasks(NR - 1, rep >> 20), []))
        lhs_ref[...] = o_ref[0, :, :64, :]
        pl.loop(0, NR)(output)

    def full_layer(rep, lhs_refs, sum_refs, stage_refs, qt_ref, k_ref, vt_ref, ot_ref,
                   q_now, k_now, v_now, s_ref, m_ref):
        def qkv(i):
            z = i >> 20

            def flip_tasks(n, dst, scale):
                def task(t, h):
                    dst[t, i, :, _tile(h)] = _pack(scale(stage_refs[n][0, _tile(h), _tile(t)]).T)
                    return dst
                return [f for t in range(NT) for f in _tasks([stage_refs[n]], task, t, (0, 1))]

            def stage(n, r, c, val):
                stage_refs[n][z, _tile(r, 64), _tile(c, 256)] = val
                return stage_refs[n]

            def emit_k(r, c, val):
                val = _pack(val)
                for t in (0, 1):
                    k_ref[2 * c + t, _rows(i, R // 2, r * 32, 32), :] = val[:, _tile(t)]
                return k_ref

            proj = _Projector(z)
            norm = norm_tasks(jnp.minimum(i + 1, NR - 1), z)
            proj.spread(norm[0], 16, 22)
            proj.spread(norm[1], 23, 35)
            proj.spread(norm[2], 44, 51)
            proj.spread(flip_tasks(0, qt_ref, lambda q: q * QSCALE), 26, 44)
            proj.spread(nested_weight_tasks(
                wbo_ref, wbo_ref.at[i], z, lambda a: bwo_ref[a, _rows(i, 32), :]), 34, 60)
            proj.spread(flip_tasks(1, vt_ref, lambda v: v), 50.5, 68)
            proj.spread(nested_left_tasks(lhs_refs, z, range(2, 7)), 0, 16)
            proj.spread(nested_left_tasks(lhs_refs, z, range(2)), 57, 70)
            proj.two_levels(lhs_refs, wb_ref.at[0], sum_refs, functools.partial(stage, 0))
            proj.two_levels(lhs_refs, wb_ref.at[2], sum_refs, functools.partial(stage, 1))
            proj.two_levels(lhs_refs, wb_ref.at[1], sum_refs, emit_k)

        def attend(u, j, b, nxt, cur, then=None):
            hs = _tile(j, DH // 2)
            if cur is not None:
                m = jnp.broadcast_to(jnp.max(m_ref[u], axis=0, keepdims=True), (G, R))
            l = acc = m_acc = None
            for c in range(S // CK):
                def scores():
                    parts = [q_now[b, hs, :]]
                    if j > 0:
                        parts.insert(0, jnp.zeros((DH // 2 * j, R), I32))
                    if j < 3:
                        parts.append(jnp.zeros((DH // 2 * (3 - j), R), I32))
                    return _dot(_unpack(k_now[_tile(c, CK // 2), :]),
                                _unpack(jnp.concatenate(parts, axis=0)))

                late = then is not None and c == S // CK - 1
                if nxt is not None and not late:
                    s = scores()
                if cur is not None:
                    slabs = {}
                    for r in reversed(range(CK // G)):
                        p = jnp.exp2(s_ref[u, _tile(c * CK // G + r, G), :] - m)
                        ls = p[0:8] + p[8:16]
                        l = ls if l is None else l + ls
                        slabs[r] = p
                    p = jnp.concatenate([slabs[r] for r in range(CK // G)], axis=0).astype(BF16)
                    off = c * CK % R
                    a = _dot(_unpack(v_now[c * CK // R, hs, off:off + CK]), p)
                    acc = a if acc is None else acc + a
                if nxt is not None:
                    if late:
                        s = scores()
                    s_ref[u, _tile(c, CK), :] = s
                    mx = jnp.max(s.reshape(CK // 8, 8, R), axis=0)
                    m_acc = mx if m_acc is None else jnp.maximum(m_acc, mx)
                if then is not None:
                    k_now[_tile(c, CK // 2), :] = k_ref[then, _tile(c, CK // 2), :]
                    v_now[c * CK // R, :, off:off + CK] = vt_ref[
                        nxt, c * CK // R, :, off:off + CK]
                if c + 1 < S // CK:
                    yield
            if nxt is not None:
                m_ref[u] = m_acc
            if cur is not None:
                inv = 1.0 / jnp.sum(l, axis=0, keepdims=True)
                cur[_tile(j, DH), :] = acc * inv
            yield

        def unflip_tasks(i, z):
            def task(t, h):
                left_ref[z, t, _tile(h), :] = ot_ref[t, i, :, _tile(h)].T
                return left_ref
            return [f for t in range(NT) for f in _tasks([], task, t, (0, 1))]

        def output(drain, i):
            proj = _Projector(i >> 20)
            proj.spread(nested_left_tasks(lhs_refs, proj.z, range(3, 7)), 0, 10)
            proj.spread(unflip_tasks(jnp.minimum(i + 1, NR - 1), proj.z), 10, 15)
            proj.spread(nested_left_tasks(lhs_refs, proj.z, range(3)), 15, 23)
            if drain:
                units = [attend(i * 4 + j, j, i, None, ot_ref.at[NT - 1, NR - QB + i])
                         for j in range(4)]
                proj.spread([([], functools.partial(next, unit))
                             for unit in units for _ in range(S // CK)], 0.5, 23.5)
            proj.two_levels(lhs_refs, wbo_ref, sum_refs, lambda r, c, val: add_to_stream(
                i, r * 64, _tile(c, 256), val))
            pl.when(rep == 1)(lambda: out_copy(i).start())

        pl.when(rep == 0)(lambda: bwo_copy.wait())
        _run(sum(norm_tasks(0, rep >> 20), []) + nested_left_tasks(lhs_refs, 0, range(2)))
        pl.loop(0, NR)(qkv)
        nqb = NR // QB

        q_now[...] = qt_ref[0, :QB]
        k_now[...] = k_ref[0]
        v_now[...] = vt_ref[0]

        @pl.loop(0, QB)
        def _(b):
            for j in range(4):
                list(attend(b * 4 + j, j, b, 0, None))
            q_now[b] = qt_ref[1, b]

        k_now[...] = k_ref[1]

        @pl.loop(0, NT * nqb - 1)
        def _(i):
            later = jnp.minimum(i + 2, NT * nqb - 1)
            for b in range(QB):
                for j in range(4):
                    list(attend(b * 4 + j, j, b, (i + 1) % NT, ot_ref.at[i % NT, i // NT * QB + b],
                                later % NT if b == QB - 1 and j == 3 else None))
                q_now[b] = qt_ref[later % NT, later // NT * QB + b]

        _run(unflip_tasks(0, rep >> 20) + nested_left_tasks(lhs_refs, 0, range(3)))
        pl.loop(0, QB)(functools.partial(output, True))
        pl.loop(QB, NR)(functools.partial(output, False))

    vmem = pltpu.VMEM
    pl.run_scoped(start_up, vmem((3 * NP, 256, D), BF16))

    @pl.loop(0, 2)
    def _(rep):
        pl.run_scoped(
            functools.partial(local_layer, rep),
            [vmem((2, R, 128), F32)] * NP,
            [vmem((2, HALO + R + PAD, 128), F32)] * NP,
            [vmem((1, WIN, R + PAD, 128), F32)] * NP,
            vmem((1, NT, R + PAD, 128), F32),
            vmem((NR, 7, 64 + PAD, D // 2), I32),
            [vmem((1, 256 + G, D), BF16)] * 2 + [vmem((1, D + G, 256), BF16)])
        pl.run_scoped(
            functools.partial(full_layer, rep),
            [vmem((1, 7, 32, D // 4), I32)] * 7,
            [[vmem((2, 64, 256), F32)] * 2] * 2,
            [vmem((1, R + PAD, D), F32)] * 2,
            vmem((NT, NR, 64, R), I32),
            vmem((NT, S // 2, 128), I32),
            vmem((NT, NR, 64, R), I32),
            vmem((NT, NR, 128, R), F32),
            vmem((QB, 64, R), I32),
            vmem((S // 2, 128), I32),
            vmem((NR, 64, R), I32),
            vmem((4 * QB, S, R), F32),
            vmem((4 * QB, 8, R), F32))
        pl.when(rep == 0)(lambda: _run(sum(norm_tasks(0, rep >> 20), []) + left_tasks(lhs1_ref)))

    for i in range(NR):
        out_copy(i).wait()


@jax.jit
def pallas_interleave_layers__sliding_local_dilated__softmax_full_mha__prompt_kernel(
    A_x: jax.Array,
    A_wqkv: jax.Array,
    A_wo: jax.Array,
    B_x: jax.Array,
    B_wqkv: jax.Array,
    B_wo: jax.Array,
):
    del B_x
    vmem = pltpu.VMEM
    dma = pltpu.SemaphoreType.DMA
    out = pl.pallas_call(
        _kernel,
        out_shape=jax.ShapeDtypeStruct((S, D), BF16),
        in_specs=[pl.BlockSpec(memory_space=pl.ANY)] * 5,
        out_specs=pl.BlockSpec(memory_space=pl.ANY),
        scratch_shapes=[
            vmem((S, D), BF16),
            vmem((1, R + G, D), BF16),
            vmem((1, NT, R + PAD, 128), F32),
            vmem((1, R, 128), F32),
            vmem((1, R, 128), F32),
            vmem((1, 4, 32 + G, D), BF16),
            vmem((7, 64, D // 2), I32),
            vmem((1, NT, HALO + R + PAD, 128), F32),
            vmem((1, WIN, R, 128), F32),
            vmem((3 * NP, NP, 7, 64, 128), I32),
            vmem((NP, NP, 7, 64, 128), I32),
            vmem((3, NR, 49, 16, 256), I32),
            vmem((NR, 49, 16, 256), I32),
            vmem((NP + 1, D + G, 256), BF16),
            vmem((4, 256, 3 * D), BF16),
            vmem((4, 256, D), BF16),
            dma((NR,)), dma((3 * NP,)), dma((NP,)), dma(()), dma(()),
        ],
        compiler_params=pltpu.CompilerParams(vmem_limit_bytes=120 * 2 ** 20),
        name="interleave_layers",
    )(A_x.reshape(S, D), A_wqkv, A_wo, B_wqkv.reshape(4, 256, 3 * D), B_wo.reshape(4, 256, D))
    return out.reshape(A_x.shape)
```

```python
import functools
import math

import jax
import jax.numpy as jnp
from jax import lax
import jax.experimental.pallas as pl
import jax.experimental.pallas.tpu as pltpu

F32 = jnp.float32
BF16 = jnp.bfloat16
I32 = jnp.int32

S = 2048
D = 1024
H = 32
DH = D // H
NT = D // 128
NP = NT // 2
WIN, DIL = 8, 2
HALO = 16
EPS = 1e-5
NEG = -1e9
LOG2E = math.log2(math.e)
QSCALE = DH ** -0.5 * LOG2E

R = 256
NR = S // R
CK = 128
QB = 4
G = 16
AHEAD = 3
PAD = 8

LHS_TERMS = (((1, 1, 0), (1, 1, 1)), ((1, 1, 1),), ((1, 0, 0), (1, 1, 1)), ((1, 1, 0), (-1, 0, 0)),
             ((1, 0, 1), (-1, 1, 1)), ((1, 0, 0), (1, 0, 1)), ((1, 0, 0),))
RHS_TERMS = (((1, 0, 0),), ((1, 1, 0), (-1, 0, 0)), ((1, 0, 0), (1, 1, 1)), ((1, 0, 0), (1, 0, 1)),
             ((1, 1, 0), (1, 1, 1)), ((1, 1, 1),), ((1, 0, 1), (-1, 1, 1)))


def _term(spec, block):
    out = block(*spec[0][1:])
    for sign, r, c in spec[1:]:
        out = out + block(r, c) if sign > 0 else out - block(r, c)
    return out


def _nested_terms(specs, outer, block):
    inner = {(r, c): _term(specs[outer], lambda a, b: block(2 * a + r, 2 * b + c))
             for r in (0, 1) for c in (0, 1)}
    return [_term(spec, lambda r, c: inner[r, c]) for spec in specs]


def _combine(s, m, x, y, emit):
    if s == 0:
        return m, None
    if s == 1:
        emit(1, 0, x() + m)
        return None, m
    if s == 2:
        return m - x(), y() + m
    if s == 3:
        return x() + m, None
    if s == 4:
        return None, y() + m
    if s == 5:
        emit(0, 0, y() - m)
        return None, m
    emit(1, 1, x() + m)
    emit(0, 1, y() + m)
    return None, None


def _strassen(product, emit):
    x = y = None
    for s in range(7):
        new_x, new_y = _combine(s, product(s), lambda: x, lambda: y, emit)
        x = x if new_x is None else new_x
        y = y if new_y is None else new_y


def _dot(a, b):
    return jnp.dot(a, b, preferred_element_type=F32)


def _pack(x):
    return pltpu.bitcast(x.astype(BF16), I32)


def _unpack(x):
    return pltpu.bitcast(x, BF16)


def _tile(t, n=128):
    return slice(t * n, (t + 1) * n)


def _tasks(reads, fn, *args):
    return [(reads, functools.partial(fn, *args[:-1], a)) for a in args[-1]]


def _run(tasks):
    for _, task in tasks:
        task()


class _Projector:
    def __init__(self, z, early, slack):
        self.z, self.early, self.slack = z, early, slack
        self.never = jnp.full((8, 128), z) > 0
        self.results, self.deadlines, self.plan = [], {}, {}

    def spread(self, tasks, first, last):
        for n, task in enumerate(tasks):
            at = int(8 * (first + n * (last - first) / len(tasks)))
            self.plan.setdefault(at, []).append(task)

    def due(self, ref, at):
        if ref is not None:
            value = ref[(0,) * (len(ref.shape) - 2)
                        + (slice(32 // ref.dtype.itemsize), slice(128))]
            self.deadlines.setdefault(at, []).append(pltpu.bitcast(value, I32))

    def product(self, lhs, rhs):
        now = range(len(self.results), len(self.results) + lhs.shape[0] // 8)
        head = [lhs[_tile(n, 8), :128] for n in range(len(now))]
        for n, at in enumerate(now):
            if at in self.deadlines:
                value = functools.reduce(jnp.bitwise_or, self.deadlines.pop(at))
                head[n] = jnp.where(self.never, value, head[n])
        lhs = jnp.concatenate([jnp.concatenate(head, axis=0), lhs[:, 128:]], axis=1)
        out = _dot(_unpack(lhs), _unpack(rhs))
        self.results += [(out, n * G) for n in range(len(now))]
        for at in now:
            for reads, task in self.plan.pop(at, ()):
                for ref in reads if at >= self.early else ():
                    earlier, r = self.results[at - self.early]
                    spare = slice(ref.shape[-2] - PAD, None)
                    ref[(self.z,) + (0,) * (len(ref.shape) - 3) + (spare, slice(128))] = (
                        earlier[r:r + PAD, :128].astype(ref.dtype))
                self.due(task(), at + self.slack)
        return out

    def paced(self, emit):
        return lambda *args: self.due(emit(*args), len(self.results) + 16)

    def one_level(self, lhs_ref, w_ref, emit):
        _strassen(lambda s: self.product(lhs_ref[s], w_ref[:, s].reshape(D // 4, 128)),
                  self.paced(emit))

    def two_levels(self, lhs_refs, w_ref, sum_refs, emit):
        emit = self.paced(emit)
        for s in range(7):
            def fold(r, c, m):
                new = _combine(s, m, lambda: sum_refs[r][c][0], lambda: sum_refs[r][c][1],
                               lambda a, b, val: emit(2 * a + r, 2 * b + c, val))
                for n, val in enumerate(new):
                    if val is not None:
                        sum_refs[r][c][self.z + n] = val
                return sum_refs[r][c]

            _strassen(lambda t: self.product(lhs_refs[s][0, t],
                                             w_ref[:, 7 * s + t].reshape(D // 8, 256)),
                      self.paced(fold))


def _permute_heads(tiles):
    dtype = tiles[0].dtype
    tiles = [pltpu.bitcast(t, I32) for t in tiles]
    lane = lax.broadcasted_iota(I32, tiles[0].shape, 1)
    for b in (1, 2, 4):
        swap = ((lane >> 2) & b) != 0
        tiles = [jnp.where(swap, tiles[i ^ b], tiles[i]) for i in range(NT)]
    e, j, hl = lane >> 5, (lane >> 2) & 7, lane & 3
    tiles = [jnp.take_along_axis(tiles[i], hl * 32 + (j ^ i) * 4 + e, axis=1,
                                 mode="promise_in_bounds") for i in range(NT)]
    return [pltpu.bitcast(t, dtype) for t in tiles]


def _rows(i, n=R, off=0, size=None, align=None):
    return pl.ds(pl.multiple_of(i * n + off, align or size or n), size or n)


def _kernel(x_hbm, awqkv_hbm, awo_hbm, bwqkv_hbm, bwo_hbm, out_hbm,
            x_ref, chunk_ref, left_ref, mean_ref, rstd_ref, piece_ref, lhs1_ref, v_ref, prob_ref,
            wa_ref, wao_ref, wb_ref, wbo_ref, awo_ref, bwqkv_ref, bwo_ref,
            x_sems, aw_sems, awo_sems, bw_sem, bwo_sem):
    def x_copy(i):
        return pltpu.make_async_copy(x_hbm.at[_rows(i)], x_ref.at[_rows(i)], x_sems.at[i])

    def out_copy(i):
        return pltpu.make_async_copy(x_ref.at[_rows(i)], out_hbm.at[_rows(i)], x_sems.at[i])

    def awo_copy(i):
        return pltpu.make_async_copy(
            awo_hbm.at[:, _rows(i, 256)], awo_ref.at[i, :D], awo_sems.at[i])

    bw_copy = pltpu.make_async_copy(bwqkv_hbm, bwqkv_ref, bw_sem)
    bwo_copy = pltpu.make_async_copy(bwo_hbm, bwo_ref, bwo_sem)

    def put_weights(w_ref, r, block):
        for s, spec in enumerate(RHS_TERMS):
            term = _pack(_term(spec, lambda a, b: block(a, b).astype(F32)))
            w_ref[s, r // 2:r // 2 + term.shape[0], :] = term

    def nested_weight_tasks(w_ref, dst, z, src):
        def fetch(a):
            piece_ref[z, a, :32, :] = src(a)
            return piece_ref

        def task(s, r, c):
            terms = _nested_terms(RHS_TERMS, s, lambda a, b: piece_ref[
                0, a, r:r + G, _tile(2 * b + c)].astype(F32))
            for t, term in enumerate(terms):
                dst[7 * s + t, r // 2:(r + G) // 2, _tile(c)] = _pack(term)
            return w_ref
        return _tasks([], fetch, range(4)) + [
            t for s in range(7) for r in (0, G) for t in _tasks([piece_ref], task, s, r, (0, 1))]

    def norm_tasks(i, z):
        def mean_task(r):
            x = x_ref[_rows(i, R, r, G), :]
            chunk_ref[z, r:r + G, :] = x
            mean_ref[z, r:r + G, :] = jnp.broadcast_to(
                jnp.mean(x.astype(F32), axis=-1, keepdims=True), (G, 128))
            return mean_ref

        def rstd_task(r):
            x = chunk_ref[0, r:r + G, :].astype(F32)
            mean = mean_ref[0, r:r + G, :]
            sq = functools.reduce(
                jnp.add, [jnp.square(x[:, _tile(t)] - mean) for t in range(NT)])
            var = jnp.sum(sq, axis=-1, keepdims=True) * (1.0 / D)
            rstd_ref[z, r:r + G, :] = lax.rsqrt(jnp.broadcast_to(var, (G, 128)) + EPS)
            return rstd_ref

        def scale_task(r):
            x = chunk_ref[0, r:r + G, :].astype(F32)
            mean, rstd = mean_ref[0, r:r + G, :], rstd_ref[0, r:r + G, :]
            for t in range(NT):
                left_ref[z, t, r:r + G, :] = (x[:, _tile(t)] - mean) * rstd
            return left_ref

        return [_tasks([chunk_ref], task, range(0, R, G))
                for task in (mean_task, rstd_task, scale_task)]

    def left_tasks(lhs_ref, src=left_ref, done=None):
        def task(s, r):
            lhs_ref[s, r // 2:(r + G) // 2, :] = _pack(jnp.concatenate([
                _term(LHS_TERMS[s], lambda a, b: src[
                    0, 2 * p + b, a * 128 + r:a * 128 + r + G, :]) for p in range(NP)], axis=1))
            return done
        return [t for s in range(7) for t in _tasks([src], task, s, range(0, 128, G))]

    def nested_left_tasks(lhs_refs, z, outer):
        def task(s, r, c):
            terms = _nested_terms(LHS_TERMS, s, lambda a, b: left_ref[
                0, 2 * b + c, a * 64 + r:a * 64 + r + G, :])
            for t, term in enumerate(terms):
                lhs_refs[s][z, t, r // 2:(r + G) // 2, _tile(c)] = _pack(term)
            return lhs_refs[s]
        return [t for s in outer for r in range(0, 64, G)
                for t in _tasks([left_ref], task, s, r, (0, 1))]

    def add_to_stream(i, r, cols, val):
        blk = (_rows(i, R, r, val.shape[0]), cols)
        x_ref[blk] = (x_ref[blk].astype(F32) + val).astype(BF16)

    def start_up(awqkv_ref):
        def aw_copy(i):
            return pltpu.make_async_copy(awqkv_hbm.at[_rows(i % NP, 256), _rows(i // NP, D)],
                                         awqkv_ref.at[i], aw_sems.at[i])

        x_copy(0).start()
        aw_copy(0).start()
        awo_ref[NP] = jnp.zeros(awo_ref.shape[1:], BF16)
        v_ref[...] = jnp.zeros(v_ref.shape, F32)
        prob_ref[...] = jnp.zeros(prob_ref.shape, F32)
        x_copy(0).wait()
        for i in range(1, AHEAD):
            aw_copy(i).start()
        _run(sum(norm_tasks(0, 0), []) + left_tasks(lhs1_ref))

        @pl.loop(0, 3 * NP)
        def _(i):
            aw_copy(i).wait()
            pl.when(i + AHEAD < 3 * NP)(lambda: aw_copy(i + AHEAD).start())
            pl.when(i + AHEAD == 3 * NP)(lambda: x_copy(1).start())
            t = _permute_heads([awqkv_ref[i, :, _tile(c)] for c in range(NT)])
            for p in range(NP):
                put_weights(wa_ref.at[i // NP * NP + p, i % NP], 0,
                            lambda a, b: t[2 * p + b][_tile(a)])

        for i in range(2, NR):
            x_copy(i).start()

    def local_layer(rep, q_refs, k_refs, sum_refs, mix_ref, o_ref, flip_refs):
        lhs_ref = lhs1_ref

        def mix_tasks(i, z):
            def task(r, p):
                o = {}
                for w in range(WIN):
                    a = prob_ref[0, w, r:r + 8, :]
                    for t in (2 * p, 2 * p + 1):
                        b = a * v_ref[0, t, HALO + r - DIL * w:HALO + r - DIL * w + 8, :]
                        o[t] = o[t] + b if w else b
                for t, val in o.items():
                    mix_ref[z, t, r:r + 8, :] = val
                return mix_ref
            return ([t for r in range(0, R, 8) for t in _tasks([v_ref], task, r, range(NP))],
                    left_tasks(o_ref.at[i], mix_ref, o_ref))

        def qkv_softmax(i):
            @pl.when(rep == 0)
            def _():
                pl.when(i + 1 < NR)(lambda: x_copy(i + 1).wait())
                pl.when(i >= NP)(lambda: awo_copy(i - NP).wait())

                @pl.when(i == 1)
                def _():
                    for n in range(NP):
                        awo_copy(n).start()
                    bw_copy.start()
                    bwo_copy.start()

            z = i >> 20

            def flip_task(r):
                flip_refs[0][z, :256, _tile(r)] = awo_ref[jnp.where(i < NP, NP, i - NP), _tile(r), :].T
                return flip_refs[0]

            def permute_task(r):
                t = _permute_heads([flip_refs[0][0, r:r + 2 * G, _tile(c)] for c in range(NT)])
                flip_refs[1][z, r:r + 2 * G, :] = jnp.concatenate(t, axis=1)
                return flip_refs[1]

            def unflip_task(r):
                flip_refs[2][z, _tile(r), :] = flip_refs[1][0, :256, _tile(r)].T
                return flip_refs[2]

            def awo_task(p, r):
                put_weights(wao_ref.at[i % NP, p], r, lambda a, b: flip_refs[2][
                    0, (2 * p + a) * 128 + r:(2 * p + a) * 128 + r + G, _tile(b)])
                return wao_ref

            def logits_task(p, r):
                q = [q_refs[p][c, r:r + 8, :] for c in (0, 1)]
                for w in range(WIN):
                    win = slice(HALO + r - DIL * w, HALO + r - DIL * w + 8)
                    a = q[0] * k_refs[p][0, win, :] + q[1] * k_refs[p][1, win, :]
                    if p > 0:
                        a = a + sum_refs[p - 1][0, w, r:r + 8, :]
                    if p == NP - 1:
                        a = a + pltpu.roll(a, 64, 1)
                    sum_refs[p][z, w, r:r + 8, :] = a
                return sum_refs[p]

            def fold_task(r):
                for w in range(WIN):
                    a = sum_refs[NP - 1][0, w, r:r + 8, :]
                    a = (a + pltpu.roll(a, 32, 1)) * QSCALE
                    if r < DIL * w:
                        pos = i * R + r + lax.broadcasted_iota(I32, (8, 128), 0)
                        a = jnp.where(pos >= DIL * w, a, NEG * LOG2E)
                    sum_refs[r // 128][z, w, r:r + 8, :] = a
                return sum_refs[r // 128]

            def softmax_task(r):
                logits = [sum_refs[r // 128][0, w, r:r + 8, :] for w in range(WIN)]
                mx = functools.reduce(jnp.maximum, logits)
                e = [jnp.exp2(a - mx) for a in logits]
                inv = 1.0 / functools.reduce(jnp.add, e)
                for w in range(WIN):
                    prob_ref[z, w, r:r + 8, :] = e[w] * inv
                return prob_ref

            proj = _Projector(z, 4, 28)
            norm = norm_tasks(jnp.minimum(i + 1, NR - 1), z)
            proj.spread(norm[0], 0, 5)
            proj.spread(norm[1], 6, 16)
            proj.spread(norm[2], 24, 30)
            proj.spread(_tasks([awo_ref], flip_task, range(NT)), 2, 10)
            proj.spread(_tasks([flip_refs[0]], permute_task, range(0, 256, 2 * G)), 13, 29)
            proj.spread(_tasks([flip_refs[1]], unflip_task, range(NT)), 31, 39)
            proj.spread([t for p in range(NP) for t in
                         _tasks([flip_refs[2]], awo_task, p, range(0, 128, G))], 41, 56)
            mix = mix_tasks(jnp.maximum(i - 1, 0), z)
            proj.spread(mix[0][:32], 1, 16)
            proj.spread(mix[0][32:48], 16, 24)
            proj.spread(mix[0][48:64], 24, 29)
            proj.spread(mix[0][64:80], 29, 38)
            proj.spread(mix[0][80:100], 38, 43)
            proj.spread(mix[0][100:112], 43, 52)
            proj.spread(mix[0][112:], 53, 56)
            proj.spread(mix[1], 58, 78)
            for p in range(NP):
                proj.spread(_tasks([k_refs[p], *sum_refs[max(p - 1, 0):p]], logits_task, p,
                                   range(0, R, 8)), 14 * p + 15, 14 * p + 24)
            proj.spread(_tasks([sum_refs[NP - 1]], fold_task, range(0, R, 8)), 66, 74)
            proj.spread([t for h in (0, 1) for t in _tasks(
                [sum_refs[h]], softmax_task, range(h * 128, h * 128 + 128, 8))], 71, 79)
            proj.spread(left_tasks(lhs_ref), 77, 84)

            for p in range(NP):
                def emit_k(h, c, val):
                    k_refs[p][z + c, HALO + h * 128:HALO + (h + 1) * 128, :] = val
                    return k_refs[p]

                def emit_q(h, c, val):
                    q_refs[p][z + c, _tile(h), :] = val
                    return q_refs[p]

                k_refs[p][:, :HALO, :] = k_refs[p][:, R:R + HALO, :]
                proj.one_level(lhs_ref, wa_ref.at[NP + p], emit_k)
                proj.one_level(lhs_ref, wa_ref.at[p], emit_q)
            v_ref[0, :, :HALO, :] = v_ref[0, :, R:R + HALO, :]
            for p in range(NP):
                def emit_v(h, c, val):
                    if h == 0:
                        v_ref[z, 2 * p + c, :HALO, :] = jnp.where(
                            i == 0, jnp.broadcast_to(val[:1], (HALO, 128)),
                            v_ref[0, 2 * p + c, :HALO, :])
                    v_ref[z, 2 * p + c, HALO + h * 128:HALO + (h + 1) * 128, :] = val
                    return v_ref

                proj.one_level(lhs_ref, wa_ref.at[2 * NP + p], emit_v)

        def output(i):
            def fetch(s, r):
                lhs_ref[s, r:r + 8, :] = o_ref[jnp.minimum(i + 1, NR - 1), s, r:r + 8, :]

            proj = _Projector(i >> 20, 5, 20)
            proj.spread([t for m in range(3) for t in nested_weight_tasks(
                wb_ref, wb_ref.at[m, i], proj.z,
                lambda a, m=m: bwqkv_ref[a, _rows(i, 32), _tile(m, D)])], 0, 20)
            proj.spread([t for s in range(7)
                         for t in _tasks([o_ref], fetch, s, range(0, 64, 8))], 21, 28)
            for p in range(NP):
                proj.one_level(lhs_ref, wao_ref.at[p], lambda h, c, val: add_to_stream(
                    i, h * 128, _tile(2 * p + c), val))

        for p in range(NP):
            k_refs[p][:, R:R + HALO, :] = jnp.zeros((2, HALO, 128), F32)
        pl.loop(0, NR)(qkv_softmax)
        pl.when(rep == 0)(lambda: bw_copy.wait())
        _run(sum(mix_tasks(NR - 1, rep >> 20), []))
        lhs_ref[...] = o_ref[0, :, :64, :]
        pl.loop(0, NR)(output)

    def full_layer(rep, lhs_refs, sum_refs, stage_refs, qt_ref, k_ref, vt_ref, ot_ref,
                   q_now, k_now, v_now, s_ref, m_ref):
        def qkv(i):
            z = i >> 20

            def flip_tasks(n, dst, scale):
                def task(t, h):
                    dst[t, i, :, _tile(h)] = _pack(scale(stage_refs[n][0, _tile(h), _tile(t)]).T)
                    return dst
                return [f for t in range(NT) for f in _tasks([stage_refs[n]], task, t, (0, 1))]

            def stage(n, r, c, val):
                stage_refs[n][z, _tile(r, 64), _tile(c, 256)] = val
                return stage_refs[n]

            def emit_k(r, c, val):
                val = _pack(val)
                for t in (0, 1):
                    k_ref[2 * c + t, _rows(i, R // 2, r * 32, 32), :] = val[:, _tile(t)]
                return k_ref

            proj = _Projector(z, 7, 25)
            norm = norm_tasks(jnp.minimum(i + 1, NR - 1), z)
            proj.spread(norm[0], 19, 28)
            proj.spread(norm[1], 29, 39)
            proj.spread(norm[2], 44, 50)
            proj.spread(flip_tasks(0, qt_ref, lambda q: q * QSCALE), 26, 44)
            proj.spread(nested_weight_tasks(
                wbo_ref, wbo_ref.at[i], z, lambda a: bwo_ref[a, _rows(i, 32), :]), 35, 61)
            proj.spread(flip_tasks(1, vt_ref, lambda v: v), 50.5, 69)
            proj.spread(nested_left_tasks(lhs_refs, z, range(2, 7)), 1, 15)
            proj.spread(nested_left_tasks(lhs_refs, z, range(2)), 58, 72)
            proj.two_levels(lhs_refs, wb_ref.at[0], sum_refs, functools.partial(stage, 0))
            proj.two_levels(lhs_refs, wb_ref.at[2], sum_refs, functools.partial(stage, 1))
            proj.two_levels(lhs_refs, wb_ref.at[1], sum_refs, emit_k)

        def attend(u, j, b, nxt, cur, then=None):
            hs = _tile(j, DH // 2)
            if cur is not None:
                m = jnp.broadcast_to(jnp.max(m_ref[u], axis=0, keepdims=True), (G, R))
            l = acc = m_acc = None
            for c in range(S // CK):
                def scores():
                    parts = [q_now[b, hs, :]]
                    if j > 0:
                        parts.insert(0, jnp.zeros((DH // 2 * j, R), I32))
                    if j < 3:
                        parts.append(jnp.zeros((DH // 2 * (3 - j), R), I32))
                    return _dot(_unpack(k_now[_tile(c, CK // 2), :]),
                                _unpack(jnp.concatenate(parts, axis=0)))

                late = then is not None and c == S // CK - 1
                if nxt is not None and not late:
                    s = scores()
                if cur is not None:
                    slabs = {}
                    for r in reversed(range(CK // G)):
                        p = jnp.exp2(s_ref[u, _tile(c * CK // G + r, G), :] - m)
                        ls = p[0:8] + p[8:16]
                        l = ls if l is None else l + ls
                        slabs[r] = p
                    p = jnp.concatenate([slabs[r] for r in range(CK // G)], axis=0).astype(BF16)
                    off = c * CK % R
                    a = _dot(_unpack(v_now[c * CK // R, hs, off:off + CK]), p)
                    acc = a if acc is None else acc + a
                if nxt is not None:
                    if late:
                        s = scores()
                    s_ref[u, _tile(c, CK), :] = s
                    mx = jnp.max(s.reshape(CK // 8, 8, R), axis=0)
                    m_acc = mx if m_acc is None else jnp.maximum(m_acc, mx)
                if then is not None:
                    k_now[_tile(c, CK // 2), :] = k_ref[then, _tile(c, CK // 2), :]
                    v_now[c * CK // R, :, off:off + CK] = vt_ref[
                        nxt, c * CK // R, :, off:off + CK]
                if c + 1 < S // CK:
                    yield
            if nxt is not None:
                m_ref[u] = m_acc
            if cur is not None:
                inv = 1.0 / jnp.sum(l, axis=0, keepdims=True)
                cur[_tile(j, DH), :] = acc * inv
            yield

        def unflip_tasks(i, z):
            def task(t, h):
                left_ref[z, t, _tile(h), :] = ot_ref[t, i, :128, _tile(h)].T
                return left_ref
            return [f for t in range(NT) for f in _tasks([ot_ref], task, t, (0, 1))]

        def output(drain, i):
            proj = _Projector(i >> 20, 8, 25)
            proj.spread(nested_left_tasks(lhs_refs, proj.z, range(3, 7)), 0, 8)
            proj.spread(unflip_tasks(jnp.minimum(i + 1, NR - 1), proj.z), 10, 15.5)
            proj.spread(nested_left_tasks(lhs_refs, proj.z, range(3)), 15.5, 21.5)
            if drain:
                units = [attend(i * 4 + j, j, i, None, ot_ref.at[NT - 1, NR - QB + i])
                         for j in range(4)]
                proj.spread([([], functools.partial(next, unit))
                             for unit in units for _ in range(S // CK)], 0, 21.5)
            proj.two_levels(lhs_refs, wbo_ref, sum_refs, lambda r, c, val: add_to_stream(
                i, r * 64, _tile(c, 256), val))
            pl.when(rep == 1)(lambda: out_copy(i).start())

        pl.when(rep == 0)(lambda: bwo_copy.wait())
        _run(sum(norm_tasks(0, rep >> 20), []) + nested_left_tasks(lhs_refs, 0, range(2)))
        pl.loop(0, NR)(qkv)
        nqb = NR // QB

        q_now[...] = qt_ref[0, :QB]
        k_now[...] = k_ref[0]
        v_now[...] = vt_ref[0]

        @pl.loop(0, QB)
        def _(b):
            for j in range(4):
                list(attend(b * 4 + j, j, b, 0, None))
            q_now[b] = qt_ref[1, b]

        k_now[...] = k_ref[1]

        @pl.loop(0, NT * nqb - 1)
        def _(i):
            later = jnp.minimum(i + 2, NT * nqb - 1)
            for b in range(QB):
                for j in range(4):
                    list(attend(b * 4 + j, j, b, (i + 1) % NT, ot_ref.at[i % NT, i // NT * QB + b],
                                later % NT if b == QB - 1 and j == 3 else None))
                q_now[b] = qt_ref[later % NT, later // NT * QB + b]

        _run(unflip_tasks(0, rep >> 20) + nested_left_tasks(lhs_refs, 0, range(3)))
        pl.loop(0, QB)(functools.partial(output, True))
        pl.loop(QB, NR)(functools.partial(output, False))

    vmem = pltpu.VMEM
    pl.run_scoped(start_up, vmem((3 * NP, 256, D), BF16))

    @pl.loop(0, 2)
    def _(rep):
        pl.run_scoped(
            functools.partial(local_layer, rep),
            [vmem((2, R, 128), F32)] * NP,
            [vmem((2, HALO + R + PAD, 128), F32)] * NP,
            [vmem((1, WIN, R + PAD, 128), F32)] * NP,
            vmem((1, NT, R + PAD, 128), F32),
            vmem((NR, 7, 64 + PAD, D // 2), I32),
            [vmem((1, 256 + G, D), BF16)] * 2 + [vmem((1, D + G, 256), BF16)])
        pl.run_scoped(
            functools.partial(full_layer, rep),
            [vmem((1, 7, 32, D // 4), I32)] * 7,
            [[vmem((2, 64, 256), F32)] * 2] * 2,
            [vmem((1, R + PAD, D), F32)] * 2,
            vmem((NT, NR, 64, R), I32),
            vmem((NT, S // 2, 128), I32),
            vmem((NT, NR, 64, R), I32),
            vmem((NT, NR, 128 + PAD, R), F32),
            vmem((QB, 64, R), I32),
            vmem((S // 2, 128), I32),
            vmem((NR, 64, R), I32),
            vmem((4 * QB, S, R), F32),
            vmem((4 * QB, 8, R), F32))
        pl.when(rep == 0)(lambda: _run(sum(norm_tasks(0, rep >> 20), []) + left_tasks(lhs1_ref)))

    for i in range(NR):
        out_copy(i).wait()


@jax.jit
def pallas_interleave_layers__sliding_local_dilated__softmax_full_mha__prompt_kernel(
    A_x: jax.Array,
    A_wqkv: jax.Array,
    A_wo: jax.Array,
    B_x: jax.Array,
    B_wqkv: jax.Array,
    B_wo: jax.Array,
):
    del B_x
    vmem = pltpu.VMEM
    dma = pltpu.SemaphoreType.DMA
    out = pl.pallas_call(
        _kernel,
        out_shape=jax.ShapeDtypeStruct((S, D), BF16),
        in_specs=[pl.BlockSpec(memory_space=pl.ANY)] * 5,
        out_specs=pl.BlockSpec(memory_space=pl.ANY),
        scratch_shapes=[
            vmem((S, D), BF16),
            vmem((1, R + G, D), BF16),
            vmem((1, NT, R + PAD, 128), F32),
            vmem((1, R, 128), F32),
            vmem((1, R, 128), F32),
            vmem((1, 4, 32 + G, D), BF16),
            vmem((7, 64, D // 2), I32),
            vmem((1, NT, HALO + R + PAD, 128), F32),
            vmem((1, WIN, R, 128), F32),
            vmem((3 * NP, NP, 7, 64, 128), I32),
            vmem((NP, NP, 7, 64, 128), I32),
            vmem((3, NR, 49, 16, 256), I32),
            vmem((NR, 49, 16, 256), I32),
            vmem((NP + 1, D + G, 256), BF16),
            vmem((4, 256, 3 * D), BF16),
            vmem((4, 256, D), BF16),
            dma((NR,)), dma((3 * NP,)), dma((NP,)), dma(()), dma(()),
        ],
        compiler_params=pltpu.CompilerParams(vmem_limit_bytes=120 * 2 ** 20),
        name="interleave_layers",
    )(A_x.reshape(S, D), A_wqkv, A_wo, B_wqkv.reshape(4, 256, 3 * D), B_wo.reshape(4, 256, D))
    return out.reshape(A_x.shape)
```

```python
import functools
import math

import jax
import jax.numpy as jnp
from jax import lax
import jax.experimental.pallas as pl
import jax.experimental.pallas.tpu as pltpu

F32 = jnp.float32
BF16 = jnp.bfloat16
I32 = jnp.int32

S = 2048
D = 1024
H = 32
DH = D // H
NT = D // 128
NP = NT // 2
WIN, DIL = 8, 2
HALO = 16
EPS = 1e-5
NEG = -1e9
LOG2E = math.log2(math.e)
QSCALE = DH ** -0.5 * LOG2E

R = 256
NR = S // R
CK = 128
QB = 4
SIDE = (1, 2, 7, 12)
SIDE_WORK = (5, 13, 17, 17, 18, 18, 18, 17, 17, 17, 17, 15, 17, 17, 16, 17)
assert sum(SIDE_WORK) == 2 * len(SIDE) * DH and len(SIDE_WORK) == S // CK
G = 16
AHEAD = 3
PAD = 8

LHS_TERMS = (((1, 1, 0), (1, 1, 1)), ((1, 1, 1),), ((1, 0, 0), (1, 1, 1)), ((1, 1, 0), (-1, 0, 0)),
             ((1, 0, 1), (-1, 1, 1)), ((1, 0, 0), (1, 0, 1)), ((1, 0, 0),))
RHS_TERMS = (((1, 0, 0),), ((1, 1, 0), (-1, 0, 0)), ((1, 0, 0), (1, 1, 1)), ((1, 0, 0), (1, 0, 1)),
             ((1, 1, 0), (1, 1, 1)), ((1, 1, 1),), ((1, 0, 1), (-1, 1, 1)))


def _term(spec, block):
    out = block(*spec[0][1:])
    for sign, r, c in spec[1:]:
        out = out + block(r, c) if sign > 0 else out - block(r, c)
    return out


def _nested_terms(specs, outer, block):
    inner = {(r, c): _term(specs[outer], lambda a, b: block(2 * a + r, 2 * b + c))
             for r in (0, 1) for c in (0, 1)}
    return [_term(spec, lambda r, c: inner[r, c]) for spec in specs]


def _combine(s, m, x, y, emit):
    if s == 0:
        return m, None
    if s == 1:
        emit(1, 0, x() + m)
        return None, m
    if s == 2:
        return m - x(), y() + m
    if s == 3:
        return x() + m, None
    if s == 4:
        return None, y() + m
    if s == 5:
        emit(0, 0, y() - m)
        return None, m
    emit(1, 1, x() + m)
    emit(0, 1, y() + m)
    return None, None


def _strassen(product, emit):
    x = y = None
    for s in range(7):
        new_x, new_y = _combine(s, product(s), lambda: x, lambda: y, emit)
        x = x if new_x is None else new_x
        y = y if new_y is None else new_y


def _dot(a, b):
    return jnp.dot(a, b, preferred_element_type=F32)


def _pack(x):
    return pltpu.bitcast(x.astype(BF16), I32)


def _unpack(x):
    return pltpu.bitcast(x, BF16)


def _tile(t, n=128):
    return slice(t * n, (t + 1) * n)


def _tasks(reads, fn, *args):
    return [(reads, functools.partial(fn, *args[:-1], a)) for a in args[-1]]


def _run(tasks):
    for _, task in tasks:
        task()


def _corner(ref):
    return (0,) * (len(ref.shape) - 2) + (slice(32 // ref.dtype.itemsize), slice(128))


def _clear_corners(*refs):
    for ref in refs:
        ref[_corner(ref)] = jnp.zeros((32 // ref.dtype.itemsize, 128), ref.dtype)


class _Projector:
    def __init__(self, z, early, slack):
        self.z, self.early, self.slack = z, early, slack
        self.never = jnp.full((8, 128), z) > 0
        self.results, self.deadlines, self.plan = [], {}, {}

    def spread(self, tasks, first, last):
        for n, task in enumerate(tasks):
            at = int(8 * (first + n * (last - first) / len(tasks)))
            self.plan.setdefault(at, []).append(task)

    def due(self, ref, at):
        if ref is not None:
            self.deadlines.setdefault(at, []).append(pltpu.bitcast(ref[_corner(ref)], I32))

    def product(self, lhs, rhs):
        now = range(len(self.results), len(self.results) + lhs.shape[0] // 8)
        head = [lhs[_tile(n, 8), :128] for n in range(len(now))]
        for n, at in enumerate(now):
            if at in self.deadlines:
                value = functools.reduce(jnp.bitwise_or, self.deadlines.pop(at))
                head[n] = jnp.where(self.never, value, head[n])
        lhs = jnp.concatenate([jnp.concatenate(head, axis=0), lhs[:, 128:]], axis=1)
        out = _dot(_unpack(lhs), _unpack(rhs))
        self.results += [(out, n * G) for n in range(len(now))]
        for at in now:
            for reads, task in self.plan.pop(at, ()):
                for ref in reads if at >= self.early else ():
                    earlier, r = self.results[at - self.early]
                    spare = slice(ref.shape[-2] - PAD, None)
                    ref[(self.z,) + (0,) * (len(ref.shape) - 3) + (spare, slice(128))] = (
                        earlier[r:r + PAD, :128].astype(ref.dtype))
                self.due(task(), at + self.slack)
        return out

    def paced(self, emit):
        return lambda *args: self.due(emit(*args), len(self.results) + 16)

    def one_level(self, lhs_ref, w_ref, emit):
        _strassen(lambda s: self.product(lhs_ref[s], w_ref[:, s].reshape(D // 4, 128)),
                  self.paced(emit))

    def two_levels(self, lhs_refs, w_ref, sum_refs, emit):
        emit = self.paced(emit)
        for s in range(7):
            def fold(r, c, m):
                new = _combine(s, m, lambda: sum_refs[r][c][0], lambda: sum_refs[r][c][1],
                               lambda a, b, val: emit(2 * a + r, 2 * b + c, val))
                for n, val in enumerate(new):
                    if val is not None:
                        sum_refs[r][c][self.z + n] = val
                return sum_refs[r][c]

            _strassen(lambda t: self.product(lhs_refs[s][0, t],
                                             w_ref[:, 7 * s + t].reshape(D // 8, 256)),
                      self.paced(fold))


class _Side:
    def __init__(self, z, keys, values):
        self.z, self.keys, self.values = z, keys, values
        self.never = jnp.full((8, 128), z) > 0
        self.done, self.dots = None, []


def _permute_heads(tiles):
    dtype = tiles[0].dtype
    tiles = [pltpu.bitcast(t, I32) for t in tiles]
    lane = lax.broadcasted_iota(I32, tiles[0].shape, 1)
    for b in (1, 2, 4):
        swap = ((lane >> 2) & b) != 0
        tiles = [jnp.where(swap, tiles[i ^ b], tiles[i]) for i in range(NT)]
    e, j, hl = lane >> 5, (lane >> 2) & 7, lane & 3
    tiles = [jnp.take_along_axis(tiles[i], hl * 32 + (j ^ i) * 4 + e, axis=1,
                                 mode="promise_in_bounds") for i in range(NT)]
    return [pltpu.bitcast(t, dtype) for t in tiles]


def _rows(i, n=R, off=0, size=None, align=None):
    return pl.ds(pl.multiple_of(i * n + off, align or size or n), size or n)


def _kernel(x_hbm, awqkv_hbm, awo_hbm, bwqkv_hbm, bwo_hbm, out_hbm,
            x_ref, chunk_ref, left_ref, mean_ref, rstd_ref, piece_ref, lhs1_ref, v_ref, prob_ref,
            wa_ref, wao_ref, wb_ref, wbo_ref, awo_ref, bwqkv_ref, bwo_ref,
            x_sems, aw_sems, awo_sems, bw_sem, bwo_sem):
    def x_copy(i):
        return pltpu.make_async_copy(x_hbm.at[_rows(i)], x_ref.at[_rows(i)], x_sems.at[i])

    def out_copy(i):
        return pltpu.make_async_copy(x_ref.at[_rows(i)], out_hbm.at[_rows(i)], x_sems.at[i])

    def awo_copy(i):
        return pltpu.make_async_copy(
            awo_hbm.at[:, _rows(i, 256)], awo_ref.at[i, :D], awo_sems.at[i])

    bw_copy = pltpu.make_async_copy(bwqkv_hbm, bwqkv_ref, bw_sem)
    bwo_copy = pltpu.make_async_copy(bwo_hbm, bwo_ref, bwo_sem)

    def put_weights(w_ref, r, block):
        for s, spec in enumerate(RHS_TERMS):
            term = _pack(_term(spec, lambda a, b: block(a, b).astype(F32)))
            w_ref[s, r // 2:r // 2 + term.shape[0], :] = term

    def nested_weight_tasks(w_ref, dst, z, src):
        def fetch(a):
            piece_ref[z, a, :32, :] = src(a)
            return piece_ref

        def task(s, r, c):
            terms = _nested_terms(RHS_TERMS, s, lambda a, b: piece_ref[
                0, a, r:r + G, _tile(2 * b + c)].astype(F32))
            for t, term in enumerate(terms):
                dst[7 * s + t, r // 2:(r + G) // 2, _tile(c)] = _pack(term)
            return w_ref
        return _tasks([], fetch, range(4)) + [
            t for s in range(7) for r in (0, G) for t in _tasks([piece_ref], task, s, r, (0, 1))]

    def norm_tasks(i, z):
        def mean_task(r):
            x = x_ref[_rows(i, R, r, G), :]
            chunk_ref[z, r:r + G, :] = x
            mean_ref[z, r:r + G, :] = jnp.broadcast_to(
                jnp.mean(x.astype(F32), axis=-1, keepdims=True), (G, 128))
            return mean_ref

        def rstd_task(r):
            x = chunk_ref[0, r:r + G, :].astype(F32)
            mean = mean_ref[0, r:r + G, :]
            sq = functools.reduce(
                jnp.add, [jnp.square(x[:, _tile(t)] - mean) for t in range(NT)])
            var = jnp.sum(sq, axis=-1, keepdims=True) * (1.0 / D)
            rstd_ref[z, r:r + G, :] = lax.rsqrt(jnp.broadcast_to(var, (G, 128)) + EPS)
            return rstd_ref

        def scale_task(r):
            x = chunk_ref[0, r:r + G, :].astype(F32)
            mean, rstd = mean_ref[0, r:r + G, :], rstd_ref[0, r:r + G, :]
            for t in range(NT):
                left_ref[z, t, r:r + G, :] = (x[:, _tile(t)] - mean) * rstd
            return left_ref

        return [_tasks([chunk_ref], task, range(0, R, G))
                for task in (mean_task, rstd_task, scale_task)]

    def left_tasks(lhs_ref, src=left_ref, done=None):
        def task(s, r):
            lhs_ref[s, r // 2:(r + G) // 2, :] = _pack(jnp.concatenate([
                _term(LHS_TERMS[s], lambda a, b: src[
                    0, 2 * p + b, a * 128 + r:a * 128 + r + G, :]) for p in range(NP)], axis=1))
            return done
        return [t for s in range(7) for t in _tasks([src], task, s, range(0, 128, G))]

    def nested_left_tasks(lhs_refs, z, outer):
        def task(s, r, c):
            terms = _nested_terms(LHS_TERMS, s, lambda a, b: left_ref[
                0, 2 * b + c, a * 64 + r:a * 64 + r + G, :])
            for t, term in enumerate(terms):
                lhs_refs[s][z, t, r // 2:(r + G) // 2, _tile(c)] = _pack(term)
            return lhs_refs[s]
        return [t for s in outer for r in range(0, 64, G)
                for t in _tasks([left_ref], task, s, r, (0, 1))]

    def add_to_stream(i, r, cols, val):
        blk = (_rows(i, R, r, val.shape[0]), cols)
        x_ref[blk] = (x_ref[blk].astype(F32) + val).astype(BF16)

    def start_up(awqkv_ref):
        def aw_copy(i):
            return pltpu.make_async_copy(awqkv_hbm.at[_rows(i % NP, 256), _rows(i // NP, D)],
                                         awqkv_ref.at[i], aw_sems.at[i])

        x_copy(0).start()
        aw_copy(0).start()
        awo_ref[NP] = jnp.zeros(awo_ref.shape[1:], BF16)
        v_ref[...] = jnp.zeros(v_ref.shape, F32)
        prob_ref[...] = jnp.zeros(prob_ref.shape, F32)
        x_copy(0).wait()
        for i in range(1, AHEAD):
            aw_copy(i).start()
        _run(sum(norm_tasks(0, 0), []) + left_tasks(lhs1_ref))

        @pl.loop(0, 3 * NP)
        def _(i):
            aw_copy(i).wait()
            pl.when(i + AHEAD < 3 * NP)(lambda: aw_copy(i + AHEAD).start())
            pl.when(i + AHEAD == 3 * NP)(lambda: x_copy(1).start())
            t = _permute_heads([awqkv_ref[i, :, _tile(c)] for c in range(NT)])
            for p in range(NP):
                put_weights(wa_ref.at[i // NP * NP + p, i % NP], 0,
                            lambda a, b: t[2 * p + b][_tile(a)])

        for i in range(2, NR):
            x_copy(i).start()

    def local_layer(rep, q_refs, k_refs, sum_refs, mix_ref, o_ref, flip_refs):
        lhs_ref = lhs1_ref

        def mix_tasks(i, z):
            def task(r, p):
                o = {}
                for w in range(WIN):
                    a = prob_ref[0, w, r:r + 8, :]
                    for t in (2 * p, 2 * p + 1):
                        b = a * v_ref[0, t, HALO + r - DIL * w:HALO + r - DIL * w + 8, :]
                        o[t] = o[t] + b if w else b
                for t, val in o.items():
                    mix_ref[z, t, r:r + 8, :] = val
                return mix_ref
            return ([t for r in range(0, R, 8) for t in _tasks([v_ref], task, r, range(NP))],
                    left_tasks(o_ref.at[i], mix_ref, o_ref))

        def qkv_softmax(i):
            @pl.when(rep == 0)
            def _():
                pl.when(i + 1 < NR)(lambda: x_copy(i + 1).wait())
                pl.when(i >= NP)(lambda: awo_copy(i - NP).wait())

                @pl.when(i == 1)
                def _():
                    for n in range(NP):
                        awo_copy(n).start()
                    bw_copy.start()
                    bwo_copy.start()

            z = i >> 20

            def flip_task(r):
                flip_refs[0][z, :256, _tile(r)] = awo_ref[jnp.where(i < NP, NP, i - NP), _tile(r), :].T
                return flip_refs[0]

            def permute_task(r):
                t = _permute_heads([flip_refs[0][0, r:r + 2 * G, _tile(c)] for c in range(NT)])
                flip_refs[1][z, r:r + 2 * G, :] = jnp.concatenate(t, axis=1)
                return flip_refs[1]

            def unflip_task(r):
                flip_refs[2][z, _tile(r), :] = flip_refs[1][0, :256, _tile(r)].T
                return flip_refs[2]

            def awo_task(p, r):
                put_weights(wao_ref.at[i % NP, p], r, lambda a, b: flip_refs[2][
                    0, (2 * p + a) * 128 + r:(2 * p + a) * 128 + r + G, _tile(b)])
                return wao_ref

            def logits_task(p, r):
                q = [q_refs[p][c, r:r + 8, :] for c in (0, 1)]
                for w in range(WIN):
                    win = slice(HALO + r - DIL * w, HALO + r - DIL * w + 8)
                    a = q[0] * k_refs[p][0, win, :] + q[1] * k_refs[p][1, win, :]
                    if p > 0:
                        a = a + sum_refs[p - 1][0, w, r:r + 8, :]
                    if p == NP - 1:
                        a = a + pltpu.roll(a, 64, 1)
                    sum_refs[p][z, w, r:r + 8, :] = a
                return sum_refs[p]

            def fold_task(r):
                for w in range(WIN):
                    a = sum_refs[NP - 1][0, w, r:r + 8, :]
                    a = (a + pltpu.roll(a, 32, 1)) * QSCALE
                    if r < DIL * w:
                        pos = i * R + r + lax.broadcasted_iota(I32, (8, 128), 0)
                        a = jnp.where(pos >= DIL * w, a, NEG * LOG2E)
                    sum_refs[r // 128][z, w, r:r + 8, :] = a
                return sum_refs[r // 128]

            def softmax_task(r):
                logits = [sum_refs[r // 128][0, w, r:r + 8, :] for w in range(WIN)]
                mx = functools.reduce(jnp.maximum, logits)
                e = [jnp.exp2(a - mx) for a in logits]
                inv = 1.0 / functools.reduce(jnp.add, e)
                for w in range(WIN):
                    prob_ref[z, w, r:r + 8, :] = e[w] * inv
                return prob_ref

            proj = _Projector(z, 4, 28)
            norm = norm_tasks(jnp.minimum(i + 1, NR - 1), z)
            proj.spread(norm[0], 0, 5)
            proj.spread(norm[1], 6, 16)
            proj.spread(norm[2], 24, 30)
            proj.spread(_tasks([awo_ref], flip_task, range(NT)), 2, 10)
            proj.spread(_tasks([flip_refs[0]], permute_task, range(0, 256, 2 * G)), 13, 29)
            proj.spread(_tasks([flip_refs[1]], unflip_task, range(NT)), 31, 39)
            proj.spread([t for p in range(NP) for t in
                         _tasks([flip_refs[2]], awo_task, p, range(0, 128, G))], 41, 56)
            mix = mix_tasks(jnp.maximum(i - 1, 0), z)
            proj.spread(mix[0][:32], 1, 16)
            proj.spread(mix[0][32:48], 16, 24)
            proj.spread(mix[0][48:64], 24, 29)
            proj.spread(mix[0][64:80], 29, 38)
            proj.spread(mix[0][80:100], 38, 43)
            proj.spread(mix[0][100:112], 43, 52)
            proj.spread(mix[0][112:], 53, 56)
            proj.spread(mix[1], 58, 78)
            for p in range(NP):
                proj.spread(_tasks([k_refs[p], *sum_refs[max(p - 1, 0):p]], logits_task, p,
                                   range(0, R, 8)), 14 * p + 15, 14 * p + 24)
            proj.spread(_tasks([sum_refs[NP - 1]], fold_task, range(0, R, 8)), 66, 74)
            proj.spread([t for h in (0, 1) for t in _tasks(
                [sum_refs[h]], softmax_task, range(h * 128, h * 128 + 128, 8))], 71, 79)
            proj.spread(left_tasks(lhs_ref), 77, 84)

            for p in range(NP):
                def emit_k(h, c, val):
                    k_refs[p][z + c, HALO + h * 128:HALO + (h + 1) * 128, :] = val
                    return k_refs[p]

                def emit_q(h, c, val):
                    q_refs[p][z + c, _tile(h), :] = val
                    return q_refs[p]

                k_refs[p][:, :HALO, :] = k_refs[p][:, R:R + HALO, :]
                proj.one_level(lhs_ref, wa_ref.at[NP + p], emit_k)
                proj.one_level(lhs_ref, wa_ref.at[p], emit_q)
            v_ref[0, :, :HALO, :] = v_ref[0, :, R:R + HALO, :]
            for p in range(NP):
                def emit_v(h, c, val):
                    if h == 0:
                        v_ref[z, 2 * p + c, :HALO, :] = jnp.where(
                            i == 0, jnp.broadcast_to(val[:1], (HALO, 128)),
                            v_ref[0, 2 * p + c, :HALO, :])
                    v_ref[z, 2 * p + c, HALO + h * 128:HALO + (h + 1) * 128, :] = val
                    return v_ref

                proj.one_level(lhs_ref, wa_ref.at[2 * NP + p], emit_v)
            assert not proj.plan

        def output(i):
            def fetch(s, r):
                lhs_ref[s, r:r + 8, :] = o_ref[jnp.minimum(i + 1, NR - 1), s, r:r + 8, :]

            proj = _Projector(i >> 20, 5, 20)
            proj.spread([t for m in range(3) for t in nested_weight_tasks(
                wb_ref, wb_ref.at[m, i], proj.z,
                lambda a, m=m: bwqkv_ref[a, _rows(i, 32), _tile(m, D)])], 0, 20)
            proj.spread([t for s in range(7)
                         for t in _tasks([o_ref], fetch, s, range(0, 64, 8))], 21, 28)
            for p in range(NP):
                proj.one_level(lhs_ref, wao_ref.at[p], lambda h, c, val: add_to_stream(
                    i, h * 128, _tile(2 * p + c), val))
            assert not proj.plan

        for p in range(NP):
            k_refs[p][:, R:R + HALO, :] = jnp.zeros((2, HALO, 128), F32)
        _clear_corners(*q_refs)
        pl.loop(0, NR)(qkv_softmax)
        pl.when(rep == 0)(lambda: bw_copy.wait())
        _run(sum(mix_tasks(NR - 1, rep >> 20), []))
        lhs_ref[...] = o_ref[0, :, :64, :]
        pl.loop(0, NR)(output)

    def full_layer(rep, lhs_refs, sum_refs, stage_refs, qt_ref, k_ref, vt_ref, ot_ref,
                   q_now, k_now, v_now, qrow_ref, kcol_ref, skew_ref, s_ref, m_ref):
        def qkv(i):
            z = i >> 20

            def flip_tasks(n, dst, scale):
                def task(t, h):
                    dst[t, i, :, _tile(h)] = _pack(scale(stage_refs[n][0, _tile(h), _tile(t)]).T)
                    return dst
                return [f for t in range(NT) for f in _tasks([stage_refs[n]], task, t, (0, 1))]

            def stage(n, r, c, val):
                stage_refs[n][z, _tile(r, 64), _tile(c, 256)] = val
                return stage_refs[n]

            def emit_k(r, c, val):
                val = _pack(val)
                for t in (0, 1):
                    k_ref[2 * c + t, _rows(i, R // 2, r * 32, 32), :] = val[:, _tile(t)]
                return k_ref

            proj = _Projector(z, 7, 25)
            norm = norm_tasks(jnp.minimum(i + 1, NR - 1), z)
            proj.spread(norm[0], 19, 28)
            proj.spread(norm[1], 29, 39)
            proj.spread(norm[2], 44, 50)
            proj.spread(flip_tasks(0, qt_ref, lambda q: q * QSCALE), 26, 44)
            proj.spread(nested_weight_tasks(
                wbo_ref, wbo_ref.at[i], z, lambda a: bwo_ref[a, _rows(i, 32), :]), 35, 61)
            proj.spread(flip_tasks(1, vt_ref, lambda v: v), 50.5, 69)
            proj.spread(nested_left_tasks(lhs_refs, z, range(2, 7)), 1, 15)
            proj.spread(nested_left_tasks(lhs_refs, z, range(2)), 58, 72)
            proj.two_levels(lhs_refs, wb_ref.at[0], sum_refs, functools.partial(stage, 0))
            proj.two_levels(lhs_refs, wb_ref.at[2], sum_refs, functools.partial(stage, 1))
            proj.two_levels(lhs_refs, wb_ref.at[1], sum_refs, emit_k)
            assert not proj.plan

        def skew_keys(z, keys):
            row, lane = (lax.broadcasted_iota(I32, (8, 128), axis) for axis in (0, 1))
            skew = (lane & -DH) | ((lane + row) & (DH - 1))
            for n, c in enumerate(SIDE):
                k = pltpu.bitcast(_unpack(keys[c * CK // 2:c * CK // 2 + 8, :]).astype(F32), I32)
                skew_ref[z, _tile(n, 8), :] = jnp.take_along_axis(
                    lax.shift_right_logical(k[:8], 16) | k[8:], skew, axis=1,
                    mode="promise_in_bounds")

        def spread_keys(z, j, d, n):
            k = skew_ref[0, _tile(n, 8), :]
            k = jnp.broadcast_to(k[:, j * DH + d:j * DH + d + 1], k.shape)
            kcol_ref[z + j % 2, d, _tile(n, G), :] = pltpu.bitcast(
                jnp.concatenate([k << 16, k & -65536], axis=0), F32)

        def widen_queries(z, u):
            q = _unpack(q_now[u % QB, _tile(u // QB, DH // 2), :]).astype(F32)
            for t in (0, 1):
                qrow_ref[z + u % 2, t, :DH, :] = q[:, _tile(t)]
                qrow_ref[z + u % 2, t, DH:DH + 8, :] = q[:8, _tile(t)]

        def attend(j, b, scores, cur, side=None):
            u, hs = j * QB + b, _tile(j, DH // 2)
            if cur is not None:
                m = jnp.broadcast_to(jnp.max(m_ref[u], axis=0, keepdims=True), (G, R))
            l = acc = m_acc = dot = None
            todo = [(n, d) for n in range(2 * len(SIDE)) for d in range(DH)]
            for c in range(S // CK):
                first = G if side and c in SIDE else 0

                def multiply():
                    parts = [q_now[b, hs, :]]
                    if j > 0:
                        parts.insert(0, jnp.zeros((DH // 2 * j, R), I32))
                    if j < 3:
                        parts.append(jnp.zeros((DH // 2 * (3 - j), R), I32))
                    k = k_now[(c * CK + first) // 2:(c + 1) * CK // 2, :]
                    if side and len(side.dots) >= 4:
                        late = pltpu.bitcast(side.dots[-2], I32)
                        k = jnp.concatenate([
                            k[:-32], jnp.where(side.never, late[:, :128], k[-32:-24]),
                            jnp.where(side.never, late[:, 128:], k[-24:-16]), k[-16:]], axis=0)
                    return _dot(_unpack(k), _unpack(jnp.concatenate(parts, axis=0)))

                last = side and u == 4 * QB - 1
                if scores and not (last and c == S // CK - 1):
                    s = multiply()
                if cur is not None:
                    slabs = {}
                    for r in reversed(range(CK // G)):
                        p = jnp.exp2(s_ref[u, _tile(c * CK // G + r, G), :] - m)
                        ls = p[0:8] + p[8:16]
                        l = ls if l is None else l + ls
                        slabs[r] = p
                    p = jnp.concatenate([slabs[r] for r in range(CK // G)], axis=0).astype(BF16)
                    a = _dot(_unpack(v_now[c // 2, hs, _tile(c % 2)]), p)
                    acc = a if acc is None else acc + a
                if last and c == S // CK - 1:
                    s = multiply()
                if scores:
                    s_ref[u, c * CK + first:(c + 1) * CK, :] = s
                    mx = jnp.max(s.reshape(-1, 8, R), axis=0)
                    m_acc = mx if m_acc is None else jnp.maximum(m_acc, mx)
                if not side:
                    if c + 1 < S // CK:
                        yield
                    continue
                if side.done is not None:
                    kcol_ref[side.z, DH, :8, :] = side.done
                    qrow_ref[side.z, 0, DH + 8:, :] = side.done
                side.done = s[-64:-56, :128]
                for n, d in todo[sum(SIDE_WORK[:c]):sum(SIDE_WORK[:c + 1])]:
                    kcol = kcol_ref[j % 2, d, _tile(n, 8), :]
                    prod = jnp.concatenate(
                        [kcol * qrow_ref[u % 2, t, d:d + 8, :] for t in (0, 1)], axis=1)
                    dot = dot + prod if d else prod
                    if d == DH - 1:
                        assert SIDE[n // 2] <= c
                        s_ref[u, _tile(SIDE[n // 2] * CK // 8 + n % 2, 8), :] = dot
                        m_acc = jnp.maximum(m_acc, dot)
                side.dots.append(dot)
                if c == 7:
                    widen_queries(side.z, (u + 1) % (4 * QB))
                for n in range(DH * len(SIDE))[_tile(b * S // CK + c, 2 * len(SIDE) // QB)]:
                    spread_keys(side.z, (j + 1) % 4, *divmod(n, len(SIDE)))
                if (j, b, c) == (2, QB - 1, S // CK - 1):
                    skew_keys(side.z, side.keys)
                if last:
                    k_now[_tile(c, CK // 2), :] = side.keys[_tile(c, CK // 2), :]
                if b == QB - 1:
                    v_now[c // 2, hs, _tile(c % 2)] = side.values[c // 2, hs, _tile(c % 2)]
            if scores:
                m_ref[u] = m_acc
            if cur is not None:
                inv = 1.0 / jnp.sum(l, axis=0, keepdims=True)
                cur[_tile(j, DH), :] = acc * inv
            yield

        def unflip_tasks(i, z):
            def task(t, h):
                left_ref[z, t, _tile(h), :] = ot_ref[t, i, :128, _tile(h)].T
                return left_ref
            return [f for t in range(NT) for f in _tasks([ot_ref], task, t, (0, 1))]

        def output(drain, i):
            proj = _Projector(i >> 20, 8, 25)
            proj.spread(nested_left_tasks(lhs_refs, proj.z, range(3, 7)), 0, 8)
            proj.spread(unflip_tasks(jnp.minimum(i + 1, NR - 1), proj.z), 10, 15.5)
            proj.spread(nested_left_tasks(lhs_refs, proj.z, range(3)), 15.5, 21.5)
            if drain:
                units = [attend(j, i, False, ot_ref.at[NT - 1, NR - QB + i])
                         for j in range(4)]
                proj.spread([([], functools.partial(next, unit))
                             for unit in units for _ in range(S // CK)], 0, 21.5)
            proj.two_levels(lhs_refs, wbo_ref, sum_refs, lambda r, c, val: add_to_stream(
                i, r * 64, _tile(c, 256), val))
            assert not proj.plan
            pl.when(rep == 1)(lambda: out_copy(i).start())

        pl.when(rep == 0)(lambda: bwo_copy.wait())
        _run(sum(norm_tasks(0, rep >> 20), []) + nested_left_tasks(lhs_refs, 0, range(2)))
        _clear_corners(*stage_refs, k_ref)
        pl.loop(0, NR)(qkv)
        nqb = NR // QB

        q_now[...] = qt_ref[0, :QB]
        k_now[...] = k_ref[0]

        @pl.loop(0, QB)
        def _(b):
            for j in range(4):
                list(attend(j, b, True, None))
            q_now[b] = qt_ref[1, b]
            v_now[...] = vt_ref[0]
            widen_queries(0, 0)
            skew_keys(0, k_ref.at[1])
            for d in range(DH):
                for n in range(len(SIDE)):
                    spread_keys(0, 0, d, n)

        k_now[...] = k_ref[1]

        @pl.loop(0, NT * nqb - 1)
        def _(i):
            later = jnp.minimum(i + 2, NT * nqb - 1)
            side = _Side(i >> 20, k_ref.at[later % NT], vt_ref.at[(i + 1) % NT])
            for j in range(4):
                for b in range(QB):
                    list(attend(j, b, True, ot_ref.at[i % NT, i // NT * QB + b], side))
                    q_now[b, _tile(j, DH // 2)] = qt_ref[
                        later % NT, later // NT * QB + b, _tile(j, DH // 2)]

        _run(unflip_tasks(0, rep >> 20) + nested_left_tasks(lhs_refs, 0, range(3)))
        pl.loop(0, QB)(functools.partial(output, True))
        pl.loop(QB, NR)(functools.partial(output, False))

    vmem = pltpu.VMEM
    pl.run_scoped(start_up, vmem((3 * NP, 256, D), BF16))

    @pl.loop(0, 2)
    def _(rep):
        pl.run_scoped(
            functools.partial(local_layer, rep),
            [vmem((2, R, 128), F32)] * NP,
            [vmem((2, HALO + R + PAD, 128), F32)] * NP,
            [vmem((1, WIN, R + PAD, 128), F32)] * NP,
            vmem((1, NT, R + PAD, 128), F32),
            vmem((NR, 7, 64 + PAD, D // 2), I32),
            [vmem((1, 256 + G, D), BF16)] * 2 + [vmem((1, D + G, 256), BF16)])
        pl.run_scoped(
            functools.partial(full_layer, rep),
            [vmem((1, 7, 32, D // 4), I32)] * 7,
            [[vmem((2, 64, 256), F32)] * 2] * 2,
            [vmem((1, R + PAD, D), F32)] * 2,
            vmem((NT, NR, 64, R), I32),
            vmem((NT, S // 2, 128), I32),
            vmem((NT, NR, 64, R), I32),
            vmem((NT, NR, 128 + PAD, R), F32),
            vmem((QB, 64, R), I32),
            vmem((S // 2, 128), I32),
            vmem((NR, 64, R), I32),
            vmem((2, 2, DH + 16, 128), F32),
            vmem((2, DH + 1, G * len(SIDE), 128), F32),
            vmem((1, 8 * len(SIDE), 128), I32),
            vmem((4 * QB, S, R), F32),
            vmem((4 * QB, 8, R), F32))
        pl.when(rep == 0)(lambda: _run(sum(norm_tasks(0, rep >> 20), []) + left_tasks(lhs1_ref)))

    for i in range(NR):
        out_copy(i).wait()


@jax.jit
def pallas_interleave_layers__sliding_local_dilated__softmax_full_mha__prompt_kernel(
    A_x: jax.Array,
    A_wqkv: jax.Array,
    A_wo: jax.Array,
    B_x: jax.Array,
    B_wqkv: jax.Array,
    B_wo: jax.Array,
):
    del B_x
    vmem = pltpu.VMEM
    dma = pltpu.SemaphoreType.DMA
    out = pl.pallas_call(
        _kernel,
        out_shape=jax.ShapeDtypeStruct((S, D), BF16),
        in_specs=[pl.BlockSpec(memory_space=pl.ANY)] * 5,
        out_specs=pl.BlockSpec(memory_space=pl.ANY),
        scratch_shapes=[
            vmem((S, D), BF16),
            vmem((1, R + G, D), BF16),
            vmem((1, NT, R + PAD, 128), F32),
            vmem((1, R, 128), F32),
            vmem((1, R, 128), F32),
            vmem((1, 4, 32 + G, D), BF16),
            vmem((7, 64, D // 2), I32),
            vmem((1, NT, HALO + R + PAD, 128), F32),
            vmem((1, WIN, R, 128), F32),
            vmem((3 * NP, NP, 7, 64, 128), I32),
            vmem((NP, NP, 7, 64, 128), I32),
            vmem((3, NR, 49, 16, 256), I32),
            vmem((NR, 49, 16, 256), I32),
            vmem((NP + 1, D + G, 256), BF16),
            vmem((4, 256, 3 * D), BF16),
            vmem((4, 256, D), BF16),
            dma((NR,)), dma((3 * NP,)), dma((NP,)), dma(()), dma(()),
        ],
        compiler_params=pltpu.CompilerParams(vmem_limit_bytes=120 * 2 ** 20),
        name="interleave_layers",
    )(A_x.reshape(S, D), A_wqkv, A_wo, B_wqkv.reshape(4, 256, 3 * D), B_wo.reshape(4, 256, D))
    return out.reshape(A_x.shape)
```

```python
import functools
import math

import jax
import jax.numpy as jnp
from jax import lax
import jax.experimental.pallas as pl
import jax.experimental.pallas.tpu as pltpu

F32 = jnp.float32
BF16 = jnp.bfloat16
I32 = jnp.int32

S = 2048
D = 1024
H = 32
DH = D // H
NT = D // 128
NP = NT // 2
WIN, DIL = 8, 2
HALO = 16
EPS = 1e-5
NEG = -1e9
LOG2E = math.log2(math.e)
QSCALE = DH ** -0.5 * LOG2E

R = 256
NR = S // R
CK = 128
QB = 4
SIDE = (1, 2, 7, 12)
SIDE_WORK = (5, 13, 17, 17, 18, 18, 18, 17, 17, 17, 17, 15, 17, 17, 16, 17)
assert sum(SIDE_WORK) == 2 * len(SIDE) * DH and len(SIDE_WORK) == S // CK
G = 16
AHEAD = 3
PAD = 8

LHS_TERMS = (((1, 1, 0), (1, 1, 1)), ((1, 1, 1),), ((1, 0, 0), (1, 1, 1)), ((1, 1, 0), (-1, 0, 0)),
             ((1, 0, 1), (-1, 1, 1)), ((1, 0, 0), (1, 0, 1)), ((1, 0, 0),))
RHS_TERMS = (((1, 0, 0),), ((1, 1, 0), (-1, 0, 0)), ((1, 0, 0), (1, 1, 1)), ((1, 0, 0), (1, 0, 1)),
             ((1, 1, 0), (1, 1, 1)), ((1, 1, 1),), ((1, 0, 1), (-1, 1, 1)))


def _term(spec, block):
    out = block(*spec[0][1:])
    for sign, r, c in spec[1:]:
        out = out + block(r, c) if sign > 0 else out - block(r, c)
    return out


def _nested_terms(specs, outer, block):
    inner = {(r, c): _term(specs[outer], lambda a, b: block(2 * a + r, 2 * b + c))
             for r in (0, 1) for c in (0, 1)}
    return [_term(spec, lambda r, c: inner[r, c]) for spec in specs]


def _combine(s, m, x, y, emit):
    if s == 0:
        return m, None
    if s == 1:
        emit(1, 0, x() + m)
        return None, m
    if s == 2:
        return m - x(), y() + m
    if s == 3:
        return x() + m, None
    if s == 4:
        return None, y() + m
    if s == 5:
        emit(0, 0, y() - m)
        return None, m
    emit(1, 1, x() + m)
    emit(0, 1, y() + m)
    return None, None


def _strassen(product, emit):
    x = y = None
    for s in range(7):
        new_x, new_y = _combine(s, product(s), lambda: x, lambda: y, emit)
        x = x if new_x is None else new_x
        y = y if new_y is None else new_y


def _dot(a, b):
    return jnp.dot(a, b, preferred_element_type=F32)


def _pack(x):
    return pltpu.bitcast(x.astype(BF16), I32)


def _unpack(x):
    return pltpu.bitcast(x, BF16)


def _tile(t, n=128):
    return slice(t * n, (t + 1) * n)


def _tasks(reads, fn, *args):
    return [(reads, functools.partial(fn, *args[:-1], a)) for a in args[-1]]


def _run(tasks):
    for _, task in tasks:
        task()


def _corner(ref):
    return (0,) * (len(ref.shape) - 2) + (slice(32 // ref.dtype.itemsize), slice(128))


def _clear_corners(*refs):
    for ref in refs:
        ref[_corner(ref)] = jnp.zeros((32 // ref.dtype.itemsize, 128), ref.dtype)


class _Projector:
    def __init__(self, z, early, slack):
        self.z, self.early, self.slack = z, early, slack
        self.never = jnp.full((8, 128), z) > 0
        self.results, self.deadlines, self.plan = [], {}, {}

    def spread(self, tasks, first, last):
        for n, task in enumerate(tasks):
            at = int(8 * (first + n * (last - first) / len(tasks)))
            self.plan.setdefault(at, []).append(task)

    def due(self, ref, at):
        if ref is not None:
            self.deadlines.setdefault(at, []).append(pltpu.bitcast(ref[_corner(ref)], I32))

    def product(self, lhs, rhs):
        now = range(len(self.results), len(self.results) + lhs.shape[0] // 8)
        head = [lhs[_tile(n, 8), :128] for n in range(len(now))]
        for n, at in enumerate(now):
            if at in self.deadlines:
                value = functools.reduce(jnp.bitwise_or, self.deadlines.pop(at))
                head[n] = jnp.where(self.never, value, head[n])
        lhs = jnp.concatenate([jnp.concatenate(head, axis=0), lhs[:, 128:]], axis=1)
        out = _dot(_unpack(lhs), _unpack(rhs))
        self.results += [(out, n * G) for n in range(len(now))]
        for at in now:
            for reads, task in self.plan.pop(at, ()):
                for ref in reads if at >= self.early else ():
                    earlier, r = self.results[at - self.early]
                    spare = slice(ref.shape[-2] - PAD, None)
                    ref[(self.z,) + (0,) * (len(ref.shape) - 3) + (spare, slice(128))] = (
                        earlier[r:r + PAD, :128].astype(ref.dtype))
                self.due(task(), at + self.slack)
        return out

    def paced(self, emit):
        return lambda *args: self.due(emit(*args), len(self.results) + 16)

    def one_level(self, lhs_ref, w_ref, emit):
        _strassen(lambda s: self.product(lhs_ref[s], w_ref[:, s].reshape(D // 4, 128)),
                  self.paced(emit))

    def two_levels(self, lhs_refs, w_ref, sum_refs, emit):
        emit = self.paced(emit)
        for s in range(7):
            def fold(r, c, m):
                new = _combine(s, m, lambda: sum_refs[r][c][0], lambda: sum_refs[r][c][1],
                               lambda a, b, val: emit(2 * a + r, 2 * b + c, val))
                for n, val in enumerate(new):
                    if val is not None:
                        sum_refs[r][c][self.z + n] = val
                return sum_refs[r][c]

            _strassen(lambda t: self.product(lhs_refs[s][0, t],
                                             w_ref[:, 7 * s + t].reshape(D // 8, 256)),
                      self.paced(fold))


class _Side:
    def __init__(self, z, keys, values):
        self.z, self.keys, self.values = z, keys, values
        self.never = jnp.full((8, 128), z) > 0
        self.done, self.dots = None, []


def _permute_heads(tiles):
    dtype = tiles[0].dtype
    tiles = [pltpu.bitcast(t, I32) for t in tiles]
    lane = lax.broadcasted_iota(I32, tiles[0].shape, 1)
    for b in (1, 2, 4):
        swap = ((lane >> 2) & b) != 0
        tiles = [jnp.where(swap, tiles[i ^ b], tiles[i]) for i in range(NT)]
    e, j, hl = lane >> 5, (lane >> 2) & 7, lane & 3
    tiles = [jnp.take_along_axis(tiles[i], hl * 32 + (j ^ i) * 4 + e, axis=1,
                                 mode="promise_in_bounds") for i in range(NT)]
    return [pltpu.bitcast(t, dtype) for t in tiles]


def _rows(i, n=R, off=0, size=None):
    return pl.ds(pl.multiple_of(i * n + off, size or n), size or n)


def _kernel(x_hbm, awqkv_hbm, awo_hbm, bwqkv_hbm, bwo_hbm, out_hbm,
            x_ref, chunk_ref, left_ref, mean_ref, rstd_ref, piece_ref, lhs1_ref, v_ref, prob_ref,
            wa_ref, wao_ref, wb_ref, wbo_ref, awo_ref, bwqkv_ref, bwo_ref,
            x_sems, aw_sems, awo_sems, bw_sem, bwo_sem):
    def x_copy(i):
        return pltpu.make_async_copy(x_hbm.at[_rows(i)], x_ref.at[_rows(i)], x_sems.at[i])

    def out_copy(i):
        return pltpu.make_async_copy(x_ref.at[_rows(i)], out_hbm.at[_rows(i)], x_sems.at[i])

    def awo_copy(i):
        return pltpu.make_async_copy(
            awo_hbm.at[:, _rows(i, 256)], awo_ref.at[i, :D], awo_sems.at[i])

    bw_copy = pltpu.make_async_copy(bwqkv_hbm, bwqkv_ref, bw_sem)
    bwo_copy = pltpu.make_async_copy(bwo_hbm, bwo_ref, bwo_sem)

    def put_weights(w_ref, r, block):
        for s, spec in enumerate(RHS_TERMS):
            term = _pack(_term(spec, lambda a, b: block(a, b).astype(F32)))
            w_ref[s, r // 2:r // 2 + term.shape[0], :] = term

    def nested_weight_tasks(w_ref, dst, z, src):
        def fetch(a):
            piece_ref[z, a, :32, :] = src(a)
            return piece_ref

        def task(s, r, c):
            terms = _nested_terms(RHS_TERMS, s, lambda a, b: piece_ref[
                0, a, r:r + G, _tile(2 * b + c)].astype(F32))
            for t, term in enumerate(terms):
                dst[7 * s + t, r // 2:(r + G) // 2, _tile(c)] = _pack(term)
            return w_ref
        return _tasks([], fetch, range(4)) + [
            t for s in range(7) for r in (0, G) for t in _tasks([piece_ref], task, s, r, (0, 1))]

    def norm_tasks(i, z):
        def mean_task(r):
            x = x_ref[_rows(i, R, r, G), :]
            chunk_ref[z, r:r + G, :] = x
            mean_ref[z, r:r + G, :] = jnp.broadcast_to(
                jnp.mean(x.astype(F32), axis=-1, keepdims=True), (G, 128))
            return mean_ref

        def rstd_task(r):
            x = chunk_ref[0, r:r + G, :].astype(F32)
            mean = mean_ref[0, r:r + G, :]
            sq = functools.reduce(
                jnp.add, [jnp.square(x[:, _tile(t)] - mean) for t in range(NT)])
            var = jnp.sum(sq, axis=-1, keepdims=True) * (1.0 / D)
            rstd_ref[z, r:r + G, :] = lax.rsqrt(jnp.broadcast_to(var, (G, 128)) + EPS)
            return rstd_ref

        def scale_task(r):
            x = chunk_ref[0, r:r + G, :].astype(F32)
            mean, rstd = mean_ref[0, r:r + G, :], rstd_ref[0, r:r + G, :]
            for t in range(NT):
                left_ref[z, t, r:r + G, :] = (x[:, _tile(t)] - mean) * rstd
            return left_ref

        return [_tasks([chunk_ref], task, range(0, R, G))
                for task in (mean_task, rstd_task, scale_task)]

    def left_tasks(lhs_ref, src=left_ref, done=None):
        def task(s, r):
            lhs_ref[s, r // 2:(r + G) // 2, :] = _pack(jnp.concatenate([
                _term(LHS_TERMS[s], lambda a, b: src[
                    0, 2 * p + b, a * 128 + r:a * 128 + r + G, :]) for p in range(NP)], axis=1))
            return done
        return [t for s in range(7) for t in _tasks([src], task, s, range(0, 128, G))]

    def nested_left_tasks(lhs_refs, z, outer):
        def task(s, r, c):
            terms = _nested_terms(LHS_TERMS, s, lambda a, b: left_ref[
                0, 2 * b + c, a * 64 + r:a * 64 + r + G, :])
            for t, term in enumerate(terms):
                lhs_refs[s][z, t, r // 2:(r + G) // 2, _tile(c)] = _pack(term)
            return lhs_refs[s]
        return [t for s in outer for r in range(0, 64, G)
                for t in _tasks([left_ref], task, s, r, (0, 1))]

    def add_to_stream(i, r, cols, val):
        blk = (_rows(i, R, r, val.shape[0]), cols)
        x_ref[blk] = (x_ref[blk].astype(F32) + val).astype(BF16)

    def start_up(awqkv_ref):
        def aw_copy(i):
            return pltpu.make_async_copy(awqkv_hbm.at[_rows(i % NP, 256), _rows(i // NP, D)],
                                         awqkv_ref.at[i], aw_sems.at[i])

        x_copy(0).start()
        aw_copy(0).start()
        awo_ref[NP] = jnp.zeros(awo_ref.shape[1:], BF16)
        v_ref[...] = jnp.zeros(v_ref.shape, F32)
        prob_ref[...] = jnp.zeros(prob_ref.shape, F32)
        x_copy(0).wait()
        for i in range(1, AHEAD):
            aw_copy(i).start()
        _run(sum(norm_tasks(0, 0), []) + left_tasks(lhs1_ref))

        @pl.loop(0, 3 * NP)
        def _(i):
            aw_copy(i).wait()
            pl.when(i + AHEAD < 3 * NP)(lambda: aw_copy(i + AHEAD).start())
            pl.when(i + AHEAD == 3 * NP)(lambda: x_copy(1).start())
            t = _permute_heads([awqkv_ref[i, :, _tile(c)] for c in range(NT)])
            for p in range(NP):
                put_weights(wa_ref.at[i // NP * NP + p, i % NP], 0,
                            lambda a, b: t[2 * p + b][_tile(a)])

        for i in range(2, NR):
            x_copy(i).start()

    def local_layer(rep, q_refs, k_refs, sum_refs, mix_ref, o_ref, flip_refs):
        lhs_ref = lhs1_ref

        def mix_tasks(i, z):
            def task(r, p):
                o = {}
                for w in range(WIN):
                    a = prob_ref[0, w, r:r + 8, :]
                    for t in (2 * p, 2 * p + 1):
                        b = a * v_ref[0, t, HALO + r - DIL * w:HALO + r - DIL * w + 8, :]
                        o[t] = o[t] + b if w else b
                for t, val in o.items():
                    mix_ref[z, t, r:r + 8, :] = val
                return mix_ref
            return ([t for r in range(0, R, 8) for t in _tasks([v_ref], task, r, range(NP))],
                    left_tasks(o_ref.at[i], mix_ref, o_ref))

        def qkv_softmax(i):
            @pl.when(rep == 0)
            def _():
                pl.when(i + 1 < NR)(lambda: x_copy(i + 1).wait())
                pl.when(i >= NP)(lambda: awo_copy(i - NP).wait())

                @pl.when(i == 1)
                def _():
                    for n in range(NP):
                        awo_copy(n).start()
                    bw_copy.start()
                    bwo_copy.start()

            z = i >> 20

            def flip_task(r):
                flip_refs[0][z, :256, _tile(r)] = awo_ref[
                    jnp.where(i < NP, NP, i - NP), _tile(r), :].T
                return flip_refs[0]

            def permute_task(r):
                t = _permute_heads([flip_refs[0][0, r:r + 2 * G, _tile(c)] for c in range(NT)])
                flip_refs[1][z, r:r + 2 * G, :] = jnp.concatenate(t, axis=1)
                return flip_refs[1]

            def unflip_task(r):
                flip_refs[2][z, _tile(r), :] = flip_refs[1][0, :256, _tile(r)].T
                return flip_refs[2]

            def awo_task(p, r):
                put_weights(wao_ref.at[i % NP, p], r, lambda a, b: flip_refs[2][
                    0, (2 * p + a) * 128 + r:(2 * p + a) * 128 + r + G, _tile(b)])
                return wao_ref

            def logits_task(p, r):
                q = [q_refs[p][c, r:r + 8, :] for c in (0, 1)]
                for w in range(WIN):
                    win = slice(HALO + r - DIL * w, HALO + r - DIL * w + 8)
                    a = q[0] * k_refs[p][0, win, :] + q[1] * k_refs[p][1, win, :]
                    if p > 0:
                        a = a + sum_refs[p - 1][0, w, r:r + 8, :]
                    if p == NP - 1:
                        a = a + pltpu.roll(a, 64, 1)
                    sum_refs[p][z, w, r:r + 8, :] = a
                return sum_refs[p]

            def fold_task(r):
                for w in range(WIN):
                    a = sum_refs[NP - 1][0, w, r:r + 8, :]
                    a = (a + pltpu.roll(a, 32, 1)) * QSCALE
                    if r < DIL * w:
                        pos = i * R + r + lax.broadcasted_iota(I32, (8, 128), 0)
                        a = jnp.where(pos >= DIL * w, a, NEG * LOG2E)
                    sum_refs[r // 128][z, w, r:r + 8, :] = a
                return sum_refs[r // 128]

            def softmax_task(r):
                logits = [sum_refs[r // 128][0, w, r:r + 8, :] for w in range(WIN)]
                mx = functools.reduce(jnp.maximum, logits)
                e = [jnp.exp2(a - mx) for a in logits]
                inv = 1.0 / functools.reduce(jnp.add, e)
                for w in range(WIN):
                    prob_ref[z, w, r:r + 8, :] = e[w] * inv
                return prob_ref

            proj = _Projector(z, 4, 28)
            norm = norm_tasks(jnp.minimum(i + 1, NR - 1), z)
            proj.spread(norm[0], 0, 5)
            proj.spread(norm[1], 6, 16)
            proj.spread(norm[2], 24, 30)
            proj.spread(_tasks([awo_ref], flip_task, range(NT)), 2, 10)
            proj.spread(_tasks([flip_refs[0]], permute_task, range(0, 256, 2 * G)), 13, 29)
            proj.spread(_tasks([flip_refs[1]], unflip_task, range(NT)), 31, 39)
            proj.spread([t for p in range(NP) for t in
                         _tasks([flip_refs[2]], awo_task, p, range(0, 128, G))], 41, 56)
            mix = mix_tasks(jnp.maximum(i - 1, 0), z)
            proj.spread(mix[0][:32], 1, 16)
            proj.spread(mix[0][32:48], 16, 24)
            proj.spread(mix[0][48:64], 24, 29)
            proj.spread(mix[0][64:80], 29, 38)
            proj.spread(mix[0][80:100], 38, 43)
            proj.spread(mix[0][100:112], 43, 52)
            proj.spread(mix[0][112:], 53, 56)
            proj.spread(mix[1], 58, 78)
            for p in range(NP):
                proj.spread(_tasks([k_refs[p], *sum_refs[max(p - 1, 0):p]], logits_task, p,
                                   range(0, R, 8)), 14 * p + 15, 14 * p + 24)
            proj.spread(_tasks([sum_refs[NP - 1]], fold_task, range(0, R, 8)), 66, 74)
            proj.spread([t for h in (0, 1) for t in _tasks(
                [sum_refs[h]], softmax_task, range(h * 128, h * 128 + 128, 8))], 71, 79)
            proj.spread(left_tasks(lhs_ref), 77, 84)

            for p in range(NP):
                def emit_k(h, c, val):
                    k_refs[p][z + c, HALO + h * 128:HALO + (h + 1) * 128, :] = val
                    return k_refs[p]

                def emit_q(h, c, val):
                    q_refs[p][z + c, _tile(h), :] = val
                    return q_refs[p]

                k_refs[p][:, :HALO, :] = k_refs[p][:, R:R + HALO, :]
                proj.one_level(lhs_ref, wa_ref.at[NP + p], emit_k)
                proj.one_level(lhs_ref, wa_ref.at[p], emit_q)
            v_ref[0, :, :HALO, :] = v_ref[0, :, R:R + HALO, :]
            for p in range(NP):
                def emit_v(h, c, val):
                    if h == 0:
                        v_ref[z, 2 * p + c, :HALO, :] = jnp.where(
                            i == 0, jnp.broadcast_to(val[:1], (HALO, 128)),
                            v_ref[0, 2 * p + c, :HALO, :])
                    v_ref[z, 2 * p + c, HALO + h * 128:HALO + (h + 1) * 128, :] = val
                    return v_ref

                proj.one_level(lhs_ref, wa_ref.at[2 * NP + p], emit_v)
            assert not proj.plan

        def output(i):
            def fetch(s, r):
                lhs_ref[s, r:r + 8, :] = o_ref[jnp.minimum(i + 1, NR - 1), s, r:r + 8, :]

            proj = _Projector(i >> 20, 5, 20)
            proj.spread([t for m in range(3) for t in nested_weight_tasks(
                wb_ref, wb_ref.at[m, i], proj.z,
                lambda a, m=m: bwqkv_ref[a, _rows(i, 32), _tile(m, D)])], 0, 20)
            proj.spread([t for s in range(7)
                         for t in _tasks([o_ref], fetch, s, range(0, 64, 8))], 21, 28)
            for p in range(NP):
                proj.one_level(lhs_ref, wao_ref.at[p], lambda h, c, val: add_to_stream(
                    i, h * 128, _tile(2 * p + c), val))
            assert not proj.plan

        for p in range(NP):
            k_refs[p][:, R:R + HALO, :] = jnp.zeros((2, HALO, 128), F32)
        _clear_corners(*q_refs)
        pl.loop(0, NR)(qkv_softmax)
        pl.when(rep == 0)(lambda: bw_copy.wait())
        _run(sum(mix_tasks(NR - 1, rep >> 20), []))
        lhs_ref[...] = o_ref[0, :, :64, :]
        pl.loop(0, NR)(output)

    def full_layer(rep, lhs_refs, sum_refs, stage_refs, qt_ref, k_ref, vt_ref, ot_ref,
                   q_now, k_now, v_now, qrow_ref, kcol_ref, skew_ref, s_ref, m_ref):
        def qkv(i):
            z = i >> 20

            def flip_tasks(n, dst, scale):
                def task(t, h):
                    dst[t, i, :, _tile(h)] = _pack(scale(stage_refs[n][0, _tile(h), _tile(t)]).T)
                    return dst
                return [f for t in range(NT) for f in _tasks([stage_refs[n]], task, t, (0, 1))]

            def stage(n, r, c, val):
                stage_refs[n][z, _tile(r, 64), _tile(c, 256)] = val
                return stage_refs[n]

            def emit_k(r, c, val):
                val = _pack(val)
                for t in (0, 1):
                    k_ref[2 * c + t, _rows(i, R // 2, r * 32, 32), :] = val[:, _tile(t)]
                return k_ref

            proj = _Projector(z, 7, 25)
            norm = norm_tasks(jnp.minimum(i + 1, NR - 1), z)
            proj.spread(norm[0], 19, 28)
            proj.spread(norm[1], 29, 39)
            proj.spread(norm[2], 44, 50)
            proj.spread(flip_tasks(0, qt_ref, lambda q: q * QSCALE), 26, 44)
            proj.spread(nested_weight_tasks(
                wbo_ref, wbo_ref.at[i], z, lambda a: bwo_ref[a, _rows(i, 32), :]), 35, 61)
            proj.spread(flip_tasks(1, vt_ref, lambda v: v), 50.5, 69)
            proj.spread(nested_left_tasks(lhs_refs, z, range(2, 7)), 1, 15)
            proj.spread(nested_left_tasks(lhs_refs, z, range(2)), 58, 72)
            proj.two_levels(lhs_refs, wb_ref.at[0], sum_refs, functools.partial(stage, 0))
            proj.two_levels(lhs_refs, wb_ref.at[2], sum_refs, functools.partial(stage, 1))
            proj.two_levels(lhs_refs, wb_ref.at[1], sum_refs, emit_k)
            assert not proj.plan

        def skew_keys(z, keys):
            row, lane = (lax.broadcasted_iota(I32, (8, 128), axis) for axis in (0, 1))
            skew = (lane & -DH) | ((lane + row) & (DH - 1))
            for n, c in enumerate(SIDE):
                k = pltpu.bitcast(_unpack(keys[c * CK // 2:c * CK // 2 + 8, :]).astype(F32), I32)
                skew_ref[z, _tile(n, 8), :] = jnp.take_along_axis(
                    lax.shift_right_logical(k[:8], 16) | k[8:], skew, axis=1,
                    mode="promise_in_bounds")

        def spread_keys(z, j, d, n):
            k = skew_ref[0, _tile(n, 8), :]
            k = jnp.broadcast_to(k[:, j * DH + d:j * DH + d + 1], k.shape)
            kcol_ref[z + j % 2, d, _tile(n, G), :] = pltpu.bitcast(
                jnp.concatenate([k << 16, k & -65536], axis=0), F32)

        def widen_queries(z, u):
            q = _unpack(q_now[u % QB, _tile(u // QB, DH // 2), :]).astype(F32)
            for t in (0, 1):
                qrow_ref[z + u % 2, t, :DH, :] = q[:, _tile(t)]
                qrow_ref[z + u % 2, t, DH:DH + 8, :] = q[:8, _tile(t)]

        def attend(j, b, scores, cur, side=None):
            u, hs = j * QB + b, _tile(j, DH // 2)
            if cur is not None:
                m = jnp.broadcast_to(jnp.max(m_ref[u], axis=0, keepdims=True), (G, R))
            l = acc = m_acc = dot = None
            todo = [(n, d) for n in range(2 * len(SIDE)) for d in range(DH)]
            for c in range(S // CK):
                first = G if side and c in SIDE else 0

                def multiply():
                    parts = [q_now[b, hs, :]]
                    if j > 0:
                        parts.insert(0, jnp.zeros((DH // 2 * j, R), I32))
                    if j < 3:
                        parts.append(jnp.zeros((DH // 2 * (3 - j), R), I32))
                    k = k_now[(c * CK + first) // 2:(c + 1) * CK // 2, :]
                    if side and len(side.dots) >= 4:
                        late = pltpu.bitcast(side.dots[-2], I32)
                        k = jnp.concatenate([
                            k[:-32], jnp.where(side.never, late[:, :128], k[-32:-24]),
                            jnp.where(side.never, late[:, 128:], k[-24:-16]), k[-16:]], axis=0)
                    return _dot(_unpack(k), _unpack(jnp.concatenate(parts, axis=0)))

                last = side and u == 4 * QB - 1
                if scores and not (last and c == S // CK - 1):
                    s = multiply()
                if cur is not None:
                    slabs = {}
                    for r in reversed(range(CK // G)):
                        p = jnp.exp2(s_ref[u, _tile(c * CK // G + r, G), :] - m)
                        ls = p[0:8] + p[8:16]
                        l = ls if l is None else l + ls
                        slabs[r] = p
                    p = jnp.concatenate([slabs[r] for r in range(CK // G)], axis=0).astype(BF16)
                    a = _dot(_unpack(v_now[c // 2, hs, _tile(c % 2)]), p)
                    acc = a if acc is None else acc + a
                if last and c == S // CK - 1:
                    s = multiply()
                if scores:
                    s_ref[u, c * CK + first:(c + 1) * CK, :] = s
                    mx = jnp.max(s.reshape(-1, 8, R), axis=0)
                    m_acc = mx if m_acc is None else jnp.maximum(m_acc, mx)
                if not side:
                    if c + 1 < S // CK:
                        yield
                    continue
                if side.done is not None:
                    kcol_ref[side.z, DH, :8, :] = side.done
                    qrow_ref[side.z, 0, DH + 8:, :] = side.done
                side.done = s[-64:-56, :128]
                for n, d in todo[sum(SIDE_WORK[:c]):sum(SIDE_WORK[:c + 1])]:
                    kcol = kcol_ref[j % 2, d, _tile(n, 8), :]
                    prod = jnp.concatenate(
                        [kcol * qrow_ref[u % 2, t, d:d + 8, :] for t in (0, 1)], axis=1)
                    dot = dot + prod if d else prod
                    if d == DH - 1:
                        assert SIDE[n // 2] <= c
                        s_ref[u, _tile(SIDE[n // 2] * CK // 8 + n % 2, 8), :] = dot
                        m_acc = jnp.maximum(m_acc, dot)
                side.dots.append(dot)
                if c == 7:
                    widen_queries(side.z, (u + 1) % (4 * QB))
                for n in range(DH * len(SIDE))[_tile(b * S // CK + c, 2 * len(SIDE) // QB)]:
                    spread_keys(side.z, (j + 1) % 4, *divmod(n, len(SIDE)))
                if (j, b, c) == (2, QB - 1, S // CK - 1):
                    skew_keys(side.z, side.keys)
                if last:
                    k_now[_tile(c, CK // 2), :] = side.keys[_tile(c, CK // 2), :]
                if b == QB - 1:
                    v_now[c // 2, hs, _tile(c % 2)] = side.values[c // 2, hs, _tile(c % 2)]
            if scores:
                m_ref[u] = m_acc
            if cur is not None:
                inv = 1.0 / jnp.sum(l, axis=0, keepdims=True)
                cur[_tile(j, DH), :] = acc * inv
            yield

        def unflip_tasks(i, z):
            def task(t, h):
                left_ref[z, t, _tile(h), :] = ot_ref[t, i, :128, _tile(h)].T
                return left_ref
            return [f for t in range(NT) for f in _tasks([ot_ref], task, t, (0, 1))]

        def output(drain, i):
            proj = _Projector(i >> 20, 8, 25)
            proj.spread(nested_left_tasks(lhs_refs, proj.z, range(3, 7)), 0, 8)
            proj.spread(unflip_tasks(jnp.minimum(i + 1, NR - 1), proj.z), 10, 15.5)
            proj.spread(nested_left_tasks(lhs_refs, proj.z, range(3)), 15.5, 21.5)
            if drain:
                units = [attend(j, i, False, ot_ref.at[NT - 1, NR - QB + i])
                         for j in range(4)]
                proj.spread([([], functools.partial(next, unit))
                             for unit in units for _ in range(S // CK)], 0, 21.5)
            proj.two_levels(lhs_refs, wbo_ref, sum_refs, lambda r, c, val: add_to_stream(
                i, r * 64, _tile(c, 256), val))
            assert not proj.plan
            pl.when(rep == 1)(lambda: out_copy(i).start())

        pl.when(rep == 0)(lambda: bwo_copy.wait())
        _run(sum(norm_tasks(0, rep >> 20), []) + nested_left_tasks(lhs_refs, 0, range(2)))
        _clear_corners(*stage_refs, k_ref)
        pl.loop(0, NR)(qkv)
        nqb = NR // QB

        q_now[...] = qt_ref[0, :QB]
        k_now[...] = k_ref[0]

        @pl.loop(0, QB)
        def _(b):
            for j in range(4):
                list(attend(j, b, True, None))
            q_now[b] = qt_ref[1, b]
            v_now[...] = vt_ref[0]
            widen_queries(0, 0)
            skew_keys(0, k_ref.at[1])
            for d in range(DH):
                for n in range(len(SIDE)):
                    spread_keys(0, 0, d, n)

        k_now[...] = k_ref[1]

        @pl.loop(0, NT * nqb - 1)
        def _(i):
            later = jnp.minimum(i + 2, NT * nqb - 1)
            side = _Side(i >> 20, k_ref.at[later % NT], vt_ref.at[(i + 1) % NT])
            for j in range(4):
                for b in range(QB):
                    list(attend(j, b, True, ot_ref.at[i % NT, i // NT * QB + b], side))
                    q_now[b, _tile(j, DH // 2)] = qt_ref[
                        later % NT, later // NT * QB + b, _tile(j, DH // 2)]

        _run(unflip_tasks(0, rep >> 20) + nested_left_tasks(lhs_refs, 0, range(3)))
        pl.loop(0, QB)(functools.partial(output, True))
        pl.loop(QB, NR)(functools.partial(output, False))

    vmem = pltpu.VMEM
    pl.run_scoped(start_up, vmem((3 * NP, 256, D), BF16))

    @pl.loop(0, 2)
    def _(rep):
        pl.run_scoped(
            functools.partial(local_layer, rep),
            [vmem((2, R, 128), F32)] * NP,
            [vmem((2, HALO + R + PAD, 128), F32)] * NP,
            [vmem((1, WIN, R + PAD, 128), F32)] * NP,
            vmem((1, NT, R + PAD, 128), F32),
            vmem((NR, 7, 64 + PAD, D // 2), I32),
            [vmem((1, 256 + G, D), BF16)] * 2 + [vmem((1, D + G, 256), BF16)])
        pl.run_scoped(
            functools.partial(full_layer, rep),
            [vmem((1, 7, 32, D // 4), I32)] * 7,
            [[vmem((2, 64, 256), F32)] * 2] * 2,
            [vmem((1, R + PAD, D), F32)] * 2,
            vmem((NT, NR, 64, R), I32),
            vmem((NT, S // 2, 128), I32),
            vmem((NT, NR, 64, R), I32),
            vmem((NT, NR, 128 + PAD, R), F32),
            vmem((QB, 64, R), I32),
            vmem((S // 2, 128), I32),
            vmem((NR, 64, R), I32),
            vmem((2, 2, DH + 16, 128), F32),
            vmem((2, DH + 1, G * len(SIDE), 128), F32),
            vmem((1, 8 * len(SIDE), 128), I32),
            vmem((4 * QB, S, R), F32),
            vmem((4 * QB, 8, R), F32))
        pl.when(rep == 0)(lambda: _run(sum(norm_tasks(0, rep >> 20), []) + left_tasks(lhs1_ref)))

    for i in range(NR):
        out_copy(i).wait()


@jax.jit
def pallas_interleave_layers__sliding_local_dilated__softmax_full_mha__prompt_kernel(
    A_x: jax.Array,
    A_wqkv: jax.Array,
    A_wo: jax.Array,
    B_x: jax.Array,
    B_wqkv: jax.Array,
    B_wo: jax.Array,
):
    del B_x
    vmem = pltpu.VMEM
    dma = pltpu.SemaphoreType.DMA
    out = pl.pallas_call(
        _kernel,
        out_shape=jax.ShapeDtypeStruct((S, D), BF16),
        in_specs=[pl.BlockSpec(memory_space=pl.ANY)] * 5,
        out_specs=pl.BlockSpec(memory_space=pl.ANY),
        scratch_shapes=[
            vmem((S, D), BF16),
            vmem((1, R + G, D), BF16),
            vmem((1, NT, R + PAD, 128), F32),
            vmem((1, R, 128), F32),
            vmem((1, R, 128), F32),
            vmem((1, 4, 32 + G, D), BF16),
            vmem((7, 64, D // 2), I32),
            vmem((1, NT, HALO + R + PAD, 128), F32),
            vmem((1, WIN, R, 128), F32),
            vmem((3 * NP, NP, 7, 64, 128), I32),
            vmem((NP, NP, 7, 64, 128), I32),
            vmem((3, NR, 49, 16, 256), I32),
            vmem((NR, 49, 16, 256), I32),
            vmem((NP + 1, D + G, 256), BF16),
            vmem((4, 256, 3 * D), BF16),
            vmem((4, 256, D), BF16),
            dma((NR,)), dma((3 * NP,)), dma((NP,)), dma(()), dma(()),
        ],
        compiler_params=pltpu.CompilerParams(vmem_limit_bytes=120 * 2 ** 20),
        name="interleave_layers",
    )(A_x.reshape(S, D), A_wqkv, A_wo, B_wqkv.reshape(4, 256, 3 * D), B_wo.reshape(4, 256, D))
    return out.reshape(A_x.shape)
```
